```python
import jax
import jax.numpy as jnp

def _softmax(x, axis=-1):
    return jax.nn.softmax(x, axis=axis)
def _gelu(x):
    return jax.nn.gelu(x, approximate=True)
def _silu(x):
    return jax.nn.silu(x)
def _sigmoid(x):
    return jax.nn.sigmoid(x)
def _layernorm(x, axis=-1, eps=1e-5):
    m = jnp.mean(x, axis=axis, keepdims=True)
    v = jnp.var(x, axis=axis, keepdims=True)
    return (x - m) / jnp.sqrt(v + eps)
def _scatter_add(tgt, idx, src, axis=0):
    return tgt.at[idx].add(src)
def _segment_sum(src, seg, n):
    return jax.ops.segment_sum(src, seg, n)
class _Rng:
    def __init__(self, key):
        self._k = key
    def _next(self):
        self._k, sub = jax.random.split(self._k)
        return sub
    def normal(self, shape):
        return jax.random.normal(self._next(), shape, dtype=jnp.bfloat16)
    def randint(self, lo, hi, shape):
        return jax.random.randint(self._next(), shape, lo, hi, dtype=jnp.int32)
    def uniform(self, shape, lo=0.0, hi=1.0):
        return jax.random.uniform(self._next(), shape, jnp.bfloat16, lo, hi)
    def permutation(self, n):
        return jax.random.permutation(self._next(), n)


kernel_name = 'recurrent_scan__sliding_local_dilated__geglu_ffn__prompt'

def setup_inputs():
    _rng = _Rng(jax.random.key(int.from_bytes(__import__("os").urandom(4), "little")))
    _w = (lambda a: (lambda t: t.astype(jnp.bfloat16) if jnp.issubdtype(t.dtype, jnp.floating) else t)(jnp.asarray(a)))
    def _A_setup():
        B, S, D = 1, 2048, 1024
        return {
            "x": _w((lambda *s: _rng.normal(s) * 0.05)(B, S, D)),
            "wqkv": _w((lambda *s: _rng.normal(s) * 0.05)(D, 3 * D)),
            "wo": _w((lambda *s: _rng.normal(s) * 0.05)(D, D)),
        }
    _A_in = _A_setup()

    def _B_setup():
        B, S, D, F = 1, 2048, 1024, 3584
        return {
            "x": _w((lambda *s: _rng.normal(s) * 0.05)(B, S, D)),
            "w_gate": _w((lambda *s: _rng.normal(s) * 0.05)(D, F)),
            "w_up": _w((lambda *s: _rng.normal(s) * 0.05)(D, F)),
            "w_down": _w((lambda *s: _rng.normal(s) * 0.05)(F, D)),
        }
    _B_in = _B_setup()

    return {
        "A_x": _A_in["x"],
        "A_wqkv": _A_in["wqkv"],
        "A_wo": _A_in["wo"],
        "B_x": _B_in["x"],
        "B_w_gate": _B_in["w_gate"],
        "B_w_up": _B_in["w_up"],
        "B_w_down": _B_in["w_down"],
    }

def reference(A_x, A_wqkv, A_wo, B_x, B_w_gate, B_w_up, B_w_down):
    def _A_ref(x, wqkv, wo):
        B, S, D = x.shape
        H = 32; Dh = D // H
        W, dil = 8, 2
        qkv = (lambda x, *d: x.transpose(*d))((x @ wqkv).reshape(B, S, 3, H, Dh), 2, 0, 3, 1, 4)
        q, k, v = qkv[0], qkv[1], qkv[2]
        scale = Dh ** -0.5
        pos = jnp.arange(S)
        off = jnp.arange(W) * dil
        idx = pos[:, None] - off[None, :]
        mask = idx >= 0
        idx_c = jnp.where(mask, idx, 0).reshape(-1)
        kg = k[:, :, idx_c, :].reshape(B, H, S, W, Dh)
        vg = v[:, :, idx_c, :].reshape(B, H, S, W, Dh)
        logits = jnp.einsum("bhsd,bhswd->bhsw", q, kg) * scale
        logits = jnp.where(mask[None, None, :, :], logits, -1e9)
        attn = _softmax(logits, axis=-1)
        o = jnp.einsum("bhsw,bhswd->bhsd", attn, vg)
        return (lambda x, *d: x.transpose(*d))(o, 0, 2, 1, 3).reshape(B, S, D) @ wo

    def _B_ref(x, w_gate, w_up, w_down):
        return (_gelu(x @ w_gate) * (x @ w_up)) @ w_down

    x = A_x
    xn = _layernorm(x, axis=-1)
    s = _A_ref(xn, A_wqkv, A_wo)
    g = _silu(_B_ref(xn, B_w_gate, B_w_up, B_w_down))
    return x + s * g
```

```python
import functools

import jax
import jax.numpy as jnp
from jax import lax
import jax.experimental.pallas as pl
import jax.experimental.pallas.tpu as pltpu

F32 = jnp.float32
BF16 = jnp.bfloat16

S, D, F = 2048, 1024, 3584
H, DH, WIN, DIL = 32, 32, 8, 2
KH = D // 2
HALO = 16
NJ = F // 256

STRASSEN = (
    ((1, 0, 0, 1), (1, 0, 0, 1), (1, 0, 0, 1)),
    ((0, 0, 1, 1), (1, 0, 0, 0), (0, 0, 1, -1)),
    ((1, 0, 0, 0), (0, 1, 0, -1), (0, 1, 0, 1)),
    ((0, 0, 0, 1), (-1, 0, 1, 0), (1, 0, 1, 0)),
    ((1, 1, 0, 0), (0, 0, 0, 1), (-1, 1, 0, 0)),
    ((-1, 0, 1, 0), (1, 1, 0, 0), (0, 0, 0, 1)),
    ((0, 1, 0, -1), (0, 0, 1, 1), (1, 0, 0, 0)),
)
CLASSIC = (
    ((1, 0, 0, 0), (1, 0, 0, 0), (1, 0, 0, 0)),
    ((0, 1, 0, 0), (0, 0, 1, 0), (1, 0, 0, 0)),
    ((1, 0, 0, 0), (0, 1, 0, 0), (0, 1, 0, 0)),
    ((0, 1, 0, 0), (0, 0, 0, 1), (0, 1, 0, 0)),
    ((0, 0, 1, 0), (1, 0, 0, 0), (0, 0, 1, 0)),
    ((0, 0, 0, 1), (0, 0, 1, 0), (0, 0, 1, 0)),
    ((0, 0, 1, 0), (0, 1, 0, 0), (0, 0, 0, 1)),
    ((0, 0, 0, 1), (0, 0, 0, 1), (0, 0, 0, 1)),
)


def _combine(coef, quads):
    idx = [i for i, c in enumerate(coef) if c != 0]
    get = lambda i: quads[i]() if callable(quads[i]) else quads[i]
    if len(idx) == 1:
        assert coef[idx[0]] == 1
        return get(idx[0]).astype(BF16)
    idx.sort(key=lambda i: -coef[i])
    a, b = get(idx[0]).astype(F32), get(idx[1]).astype(F32)
    return ((a + b) if coef[idx[1]] == 1 else (a - b)).astype(BF16)


def _blockmm(scheme, lhs, rhs, between=None):
    c = [None] * 4
    neg = [False] * 4
    for i, (_, _, cc) in enumerate(scheme):
        m = jnp.dot(lhs(i), rhs(i), preferred_element_type=F32)
        for qd, s in enumerate(cc):
            if s == 0:
                continue
            if c[qd] is None:
                c[qd], neg[qd] = m, s < 0
            elif neg[qd]:
                assert s > 0
                c[qd], neg[qd] = m - c[qd], False
            else:
                c[qd] = c[qd] + m if s > 0 else c[qd] - m
        if between is not None:
            between(i)
    assert not any(neg)
    return c


def _gelu(g):
    hg = 0.5 * g
    t = jnp.tanh(g * (0.7978845608028654 + 0.035677408136300125 * (g * g)))
    return hg * t + hg


def _kernel(x_hbm, wqkv_hbm, wo_hbm, wg_hbm, wu_hbm, wd_hbm, out_hbm,
            xbuf, aop, wg_buf, wu_buf, wd_buf, wqkv_buf, wo_buf,
            hop, wdop, wqop, woop, q_s, k_s, v_s, oop, g_s, obuf, tmp_u, tmp_f,
            sem_x, sem_g, sem_u, sem_d, sem_w, sem_o, *, scheme, TM, M1, RB):
    MH = TM // 2
    NT = S // TM
    NP = len(scheme)

    def x_copy(t):
        rows = pl.ds(pl.multiple_of(t * TM, TM), TM)
        return pltpu.make_async_copy(x_hbm.at[rows], xbuf.at[rows], sem_x.at[t])

    def g_copy(j):
        cols = pl.ds(pl.multiple_of(j * 256, 256), 256)
        return pltpu.make_async_copy(wg_hbm.at[:, cols], wg_buf.at[j], sem_g.at[j])

    def u_copy(j):
        cols = pl.ds(pl.multiple_of(j * 256, 256), 256)
        return pltpu.make_async_copy(wu_hbm.at[:, cols], wu_buf.at[j], sem_u.at[j])

    def d_copy(j):
        rows = pl.ds(pl.multiple_of(j * 256, 256), 256)
        return pltpu.make_async_copy(wd_hbm.at[rows], wd_buf.at[rows], sem_d.at[j])

    def qkv_copy(m):
        cols = pl.ds(pl.multiple_of(m * D, D), D)
        return pltpu.make_async_copy(wqkv_hbm.at[:, cols], wqkv_buf.at[m], sem_w.at[m])

    def wo_copy(c):
        return pltpu.make_async_copy(wo_hbm.at[:, pl.ds(c * 128, 128)], wo_buf.at[c], sem_w.at[3 + c])

    def o_copy(t):
        rows = pl.ds(pl.multiple_of(t * TM, TM), TM)
        return pltpu.make_async_copy(obuf.at[rows], out_hbm.at[rows], sem_o.at[t])

    for t in range(NT):
        x_copy(t).start()
    g_copy(0).start()
    u_copy(0).start()

    def layernorm(rows):
        xv = xbuf[rows, :].astype(F32)
        xc = xv - jnp.mean(xv, axis=-1, keepdims=True)
        var = jnp.mean(xc * xc, axis=-1, keepdims=True)
        return xc * lax.rsqrt(var + 1e-5)

    LB = 64

    def ln_tile(t, carry):
        x_copy(t).wait()
        for i in range(0, MH, LB):
            top = layernorm(pl.ds(pl.multiple_of(t * TM + i, LB), LB))
            bot = layernorm(pl.ds(pl.multiple_of(t * TM + MH + i, LB), LB))
            quads = (top[:, :KH], top[:, KH:], bot[:, :KH], bot[:, KH:])
            for p, (ca, _, _) in enumerate(scheme):
                aop[p, pl.ds(pl.multiple_of(t * MH + i, LB), LB), :] = _combine(ca, quads)
        return carry

    lax.fori_loop(0, NT, ln_tile, 0)
    g_copy(1).start()
    u_copy(1).start()

    def prep_wd(j):
        r0 = pl.multiple_of(j * 256, 256)
        for i in range(0, 128, 32):
            top = wd_buf[pl.ds(r0 + i, 32), :]
            bot = wd_buf[pl.ds(r0 + 128 + i, 32), :]
            quads = (top[:, :KH], top[:, KH:], bot[:, :KH], bot[:, KH:])
            for p, (_, cb, _) in enumerate(scheme):
                wdop[p, pl.ds(pl.multiple_of(j * 128, 128) + i, 32), :] = _combine(cb, quads)

    def permute_cols(w, slot):
        tmp_u[slot] = pltpu.bitcast(w, jnp.uint32).T
        p = jnp.concatenate(
            [tmp_u[slot, pl.ds(d, H, stride=DH), :] for d in range(DH)], axis=0)
        return pltpu.bitcast(p.T, BF16)

    def prep_qkv(i):
        m, rb = i // 2, i % 2
        r0 = pl.multiple_of(rb * 256, 256)
        top = permute_cols(wqkv_buf[m, pl.ds(r0, 256), :], 0)
        bot = permute_cols(wqkv_buf[m, pl.ds(KH + r0, 256), :], 1)
        for r in range(0, 256, 32):
            quads = (top[r:r + 32, :KH], top[r:r + 32, KH:], bot[r:r + 32, :KH], bot[r:r + 32, KH:])
            for p, (_, cb, _) in enumerate(scheme):
                wqop[m, p, pl.ds(r0 + r, 32), :] = _combine(cb, quads)

    def prep_wo(c):
        tmp_f[0] = wo_buf[c].astype(F32)
        tmp_f[1] = wo_buf[c + 4].astype(F32)
        for d in range(DH // 2):
            quads = tuple(tmp_f[s, pl.ds(dd, H, stride=DH), :]
                          for dd in (d, d + DH // 2) for s in (0, 1))
            for p, (_, cb, _) in enumerate(scheme):
                woop[p, c, pl.ds(d * H, H), :] = _combine(cb, quads)

    def ffn_up(j, extra):
        g_copy(j).wait()
        u_copy(j).wait()

        def rhs(buf):
            quads = tuple(
                functools.partial(lambda r, c: buf[j, pl.ds(r, KH), pl.ds(c, 128)], r, c)
                for r in (0, KH) for c in (0, 128))
            return lambda p: _combine(scheme[p][1], quads)

        extra()
        for m0 in range(0, S // 2, M1):
            lhs = lambda p: aop[p, pl.ds(m0, M1), :]
            gate = _blockmm(scheme, lhs, rhs(wg_buf))
            act = [_gelu(g) for g in gate]
            up = _blockmm(scheme, lhs, rhs(wu_buf))
            h = [a * u for a, u in zip(act, up)]
            for p, (ca, _, _) in enumerate(scheme):
                hop[p, j, pl.ds(m0, M1), :] = _combine(ca, h)

    def prefetch(j):
        @pl.when(j + 2 < NJ)
        def _():
            g_copy(j + 2).start()
            u_copy(j + 2).start()

    def loop_a(j, carry):
        prefetch(j)

        @pl.when(j < 3)
        def _():
            qkv_copy(j).start()

        @pl.when(j == 3)
        def _():
            for c in range(8):
                wo_copy(c).start()
            d_copy(0).start()
            d_copy(1).start()

        ffn_up(j, lambda: None)
        return carry

    def loop_b(j, carry):
        i = j - 4
        prefetch(j)
        d_copy(2 * i + 2).start()
        d_copy(2 * i + 3).start()
        d_copy(i).wait()

        @pl.when(i % 2 == 0)
        def _():
            qkv_copy(i // 2).wait()

        ffn_up(j, lambda: (prep_wd(i), prep_qkv(i)))
        return carry

    def loop_c(j, carry):
        i = j - 10
        prefetch(j)
        d_copy(6 + 2 * i).wait()
        d_copy(7 + 2 * i).wait()
        ffn_up(j, lambda: (prep_wd(6 + 2 * i), prep_wd(7 + 2 * i), prep_wo(i)))
        return carry

    lax.fori_loop(0, 4, loop_a, 0)
    lax.fori_loop(4, 10, loop_b, 0)
    for c in range(8):
        wo_copy(c).wait()
    lax.fori_loop(10, NJ, loop_c, 0)

    scale = DH ** -0.5

    def attend(t, r):
        lg = [None] * WIN
        for c in range(8):
            qv = q_s[c, pl.ds(r, RB), :]
            for w in range(WIN):
                pr = qv * k_s[c, pl.ds(HALO + r - DIL * w, RB), :]
                lg[w] = pr if c == 0 else lg[w] + pr
        for w in range(WIN):
            l = lg[w] + pltpu.roll(lg[w], 64, 1)
            l = (l + pltpu.roll(l, 32, 1)) * scale
            if r < DIL * w:
                pos = t * TM + r + lax.broadcasted_iota(jnp.int32, (RB, 128), 0)
                l = jnp.where(pos >= DIL * w, l, -1e9)
            lg[w] = l
        mx = functools.reduce(jnp.maximum, lg)
        e = [jnp.exp(l - mx) for l in lg]
        inv = 1.0 / functools.reduce(jnp.add, e)
        pw = [x * inv for x in e]
        outs = []
        for c in range(8):
            acc = None
            for w in range(WIN):
                pr = pw[w] * v_s[c, pl.ds(HALO + r - DIL * w, RB), :]
                acc = pr if acc is None else acc + pr
            outs.append(acc)
        return jnp.concatenate(outs[:4], axis=1), jnp.concatenate(outs[4:], axis=1)

    def tile(t, carry):
        prow = pl.ds(pl.multiple_of(t * MH, MH), MH)
        lhs = lambda p: aop[p, prow, :]
        for c in range(8):
            k_s[c, pl.ds(0, HALO), :] = jnp.where(t > 0, k_s[c, pl.ds(TM, HALO), :], 0.0)
        v_old = [v_s[c, pl.ds(TM, HALO), :] for c in range(8)]
        for m, (dst, off) in ((2, (v_s, HALO)), (1, (k_s, HALO)), (0, (q_s, 0))):
            quads = _blockmm(scheme, lhs, lambda p: wqop[m, p])
            for qd, val in enumerate(quads):
                for c in range(4):
                    dst[(qd % 2) * 4 + c, pl.ds(off + (qd // 2) * MH, MH), :] = val[:, c * 128:(c + 1) * 128]
            if m == 2:
                for c in range(8):
                    first = jnp.broadcast_to(v_s[c, pl.ds(HALO, 1), :], (HALO, 128))
                    v_s[c, pl.ds(0, HALO), :] = jnp.where(t > 0, v_old[c], first)

        starts = list(range(0, MH, RB))

        def between(p):
            lo, hi = p * len(starts) // NP, (p + 1) * len(starts) // NP
            for r in starts[lo:hi]:
                quads = attend(t, r) + attend(t, MH + r)
                for pp, (ca, _, _) in enumerate(scheme):
                    oop[pp, pl.ds(r, RB), :] = _combine(ca, quads)

        dn = _blockmm(
            scheme,
            lambda p: jnp.concatenate([hop[p, j, prow, :] for j in range(NJ)], axis=1),
            lambda p: wdop[p], between)
        gq = [d * jax.nn.sigmoid(d) for d in dn]
        sq = _blockmm(
            scheme, lambda p: oop[p],
            lambda p: jnp.concatenate([woop[p, c] for c in range(4)], axis=1))
        for qd in range(4):
            rows = pl.ds(pl.multiple_of(t * TM + (qd // 2) * MH, MH), MH)
            cols = pl.ds((qd % 2) * KH, KH)
            obuf[rows, cols] = (xbuf[rows, cols].astype(F32) + sq[qd] * gq[qd]).astype(BF16)
        o_copy(t).start()
        return carry

    lax.fori_loop(0, NT, tile, 0)
    for t in range(NT):
        o_copy(t).wait()


def make(scheme=STRASSEN, TM=512, M1=1024, RB=16, flags=None, interpret=False):
    NP = len(scheme)
    MH = TM // 2

    def f(A_x, A_wqkv, A_wo, B_x, B_w_gate, B_w_up, B_w_down):
        del B_x
        any_spec = pl.BlockSpec(memory_space=pl.ANY)
        out = pl.pallas_call(
            functools.partial(_kernel, scheme=scheme, TM=TM, M1=M1, RB=RB),
            out_shape=jax.ShapeDtypeStruct((S, D), BF16),
            in_specs=[any_spec] * 6,
            out_specs=any_spec,
            scratch_shapes=[
                pltpu.VMEM((S, D), BF16),
                pltpu.VMEM((NP, S // 2, KH), BF16),
                pltpu.VMEM((NJ, D, 256), BF16),
                pltpu.VMEM((NJ, D, 256), BF16),
                pltpu.VMEM((F, D), BF16),
                pltpu.VMEM((3, D, D), BF16),
                pltpu.VMEM((8, D, 128), BF16),
                pltpu.VMEM((NP, NJ, S // 2, 128), BF16),
                pltpu.VMEM((NP, F // 2, KH), BF16),
                pltpu.VMEM((3, NP, KH, KH), BF16),
                pltpu.VMEM((NP, 4, KH, 128), BF16),
                pltpu.VMEM((8, TM, 128), F32),
                pltpu.VMEM((8, HALO + TM, 128), F32),
                pltpu.VMEM((8, HALO + TM, 128), F32),
                pltpu.VMEM((NP, MH, KH), BF16),
                pltpu.VMEM((8, 128), F32),
                pltpu.VMEM((S, D), BF16),
                pltpu.VMEM((2, D, 128), jnp.uint32),
                pltpu.VMEM((2, D, 128), F32),
                pltpu.SemaphoreType.DMA((S // TM,)),
                pltpu.SemaphoreType.DMA((NJ,)),
                pltpu.SemaphoreType.DMA((NJ,)),
                pltpu.SemaphoreType.DMA((NJ,)),
                pltpu.SemaphoreType.DMA((11,)),
                pltpu.SemaphoreType.DMA((S // TM,)),
            ],
            compiler_params=pltpu.CompilerParams(
                vmem_limit_bytes=126 * 2**20, **({"flags": flags} if flags else {})),
            name="fused_block",
            interpret=interpret,
        )(A_x.reshape(S, D), A_wqkv, A_wo, B_w_gate, B_w_up, B_w_down)
        return out.reshape(1, S, D)

    return f


@jax.jit
def pallas_recurrent_scan__sliding_local_dilated__geglu_ffn__prompt_kernel(
    A_x: jax.Array,
    A_wqkv: jax.Array,
    A_wo: jax.Array,
    B_x: jax.Array,
    B_w_gate: jax.Array,
    B_w_up: jax.Array,
    B_w_down: jax.Array,
):
    return make()(A_x, A_wqkv, A_wo, B_x, B_w_gate, B_w_up, B_w_down)
```

```python
import functools

import jax
import jax.numpy as jnp
from jax import lax
import jax.experimental.pallas as pl
import jax.experimental.pallas.tpu as pltpu

F32 = jnp.float32
BF16 = jnp.bfloat16
U32 = jnp.uint32

S, D, F = 2048, 1024, 3584
H, DH, WIN, DIL = 32, 32, 8, 2
HALO = 16
NJ = F // 512
NU = S // 512

LHS = ((1, 0, 0, 1), (0, 0, 1, 1), (1, 0, 0, 0), (0, 0, 0, 1),
       (1, 1, 0, 0), (-1, 0, 1, 0), (0, 1, 0, -1))
RHS = ((1, 0, 0, 1), (1, 0, 0, 0), (0, 1, 0, -1), (-1, 0, 1, 0),
       (0, 0, 0, 1), (1, 1, 0, 0), (0, 0, 1, 1))
OUT = ((1, 0, 0, 1), (0, 0, 1, -1), (0, 1, 0, 1), (1, 0, 1, 0),
       (-1, 1, 0, 0), (0, 0, 0, 1), (1, 0, 0, 0))
NP = 7
QUADS = ((0, 0), (0, 1), (1, 0), (1, 1))


def _lin(coef, quads):
    idx = sorted((i for i, c in enumerate(coef) if c), key=lambda i: -coef[i])
    get = lambda i: quads[i]() if callable(quads[i]) else quads[i]
    if len(idx) == 1:
        return get(idx[0])
    a, b = get(idx[0]).astype(F32), get(idx[1]).astype(F32)
    return a + b if coef[idx[1]] > 0 else a - b


def _strassen(product, done, order):
    acc = [None] * 4
    left = [sum(1 for p in range(NP) if OUT[p][q]) for q in range(4)]
    for p in order:
        m = product(p)
        for q in range(4):
            s = OUT[p][q]
            if s == 0:
                continue
            if acc[q] is None:
                acc[q] = (s, m)
            else:
                s0, c = acc[q]
                assert s > 0 or s0 > 0
                acc[q] = (1, [x + y if s == s0 else (x - y if s > 0 else y - x)
                              for x, y in zip(m, c)])
            left[q] -= 1
            if left[q] == 0:
                done(q, acc[q][1])


def _quadrants(product, order):
    out = [None] * 4

    def done(q, val):
        out[q] = val[0]

    _strassen(lambda p: [product(p)], done, order)
    return out


def _dot(a, b):
    return jnp.dot(a, b, preferred_element_type=F32)


def _cat(xs):
    return jnp.concatenate(list(xs), axis=1)


def _lanes(v, c):
    return v[:, c * 128:(c + 1) * 128]


def _gelu(g):
    hg = 0.5 * g
    t = jnp.tanh(g * (0.7978845608028654 + 0.035677408136300125 * (g * g)))
    return hg * t + hg


def _kernel(x_hbm, wqkv_hbm, wo_hbm, wg_hbm, wu_hbm, wd_hbm, out_hbm,
            xbuf, aop, wqop, woop, sem_x, sem_g, sem_u, sem_d, sem_w, sem_o, *, cfg):
    RB = cfg["RB"]
    orders = {k: [int(c) for c in v] for k, v in cfg.items() if k.startswith("o_")}

    def operand(ref, lead, start, size):
        if cfg["cast"]:
            if not isinstance(start, int):
                start2 = pl.multiple_of(start // 2, size // 2)
            else:
                start2 = start // 2
            return pltpu.bitcast(ref.bitcast(U32)[(*lead, pl.ds(start2, size // 2))], BF16)
        return ref[(*lead, pl.ds(start, size))]

    def x_copy(u):
        rows = pl.ds(pl.multiple_of(u * 512, 512), 512)
        return pltpu.make_async_copy(x_hbm.at[rows], xbuf.at[rows], sem_x.at[u])

    def o_copy(t):
        rows = pl.ds(pl.multiple_of(t * 256, 256), 256)
        return pltpu.make_async_copy(xbuf.at[rows], out_hbm.at[rows], sem_o.at[t])

    def inner_index(a, b):
        return {(0, 0): 2, (1, 1): 3, (0, 1): 7, (1, 0): 8}[a, b] * NP

    def gate_slot(a, a2, c):
        return 4 * NP + (2 * a + a2) * 4 + c // 2, c % 2

    def ffn(hop, wdop, wg_buf, wu_buf, wd_buf, wqkv_buf, wo_buf, tmp_u, tmp_f):

        def g_copy(j):
            cols = pl.ds(pl.multiple_of(j * 512, 512), 512)
            return pltpu.make_async_copy(wg_hbm.at[:, cols], wg_buf.at[j % 2], sem_g.at[j % 2])

        def u_copy(j):
            cols = pl.ds(pl.multiple_of(j * 512, 512), 512)
            return pltpu.make_async_copy(wu_hbm.at[:, cols], wu_buf.at[j % 2], sem_u.at[j % 2])

        def d_copy(j):
            rows = pl.ds(pl.multiple_of(j * 512, 512), 512)
            return pltpu.make_async_copy(wd_hbm.at[rows], wd_buf.at[j % 2], sem_d.at[j % 2])

        def w_copies(u):
            slot = u % 2
            r0 = (u // 2) * 512 + (u % 2) * 128
            cs = [pltpu.make_async_copy(
                wqkv_hbm.at[pl.ds(pl.multiple_of(r0 + 256 * s, 128), 128)],
                wqkv_buf.at[slot, pl.ds(128 * s, 128)], sem_w.at[4 * slot + s]) for s in range(2)]
            cs += [pltpu.make_async_copy(
                wo_hbm.at[:, pl.ds(pl.multiple_of((u + 4 * s) * 128, 128), 128)],
                wo_buf.at[slot, s], sem_w.at[4 * slot + 2 + s]) for s in range(2)]
            return cs

        for u in range(NU):
            x_copy(u).start()
        g_copy(0).start()
        u_copy(0).start()
        d_copy(0).start()

        LB = 16

        def ln_chunk(u, carry):
            x_copy(u).wait()

            def stats(i, carry):
                r = pl.multiple_of(i * cfg["LS"], cfg["LS"])
                xv = xbuf[pl.ds(u * 512 + r, cfg["LS"]), :].astype(F32)
                mean = jnp.mean(xv, axis=-1, keepdims=True)
                xc = xv - mean
                var = jnp.mean(xc * xc, axis=-1, keepdims=True)
                tmp_f[0, pl.ds(r, cfg["LS"]), :] = jnp.broadcast_to(mean, (cfg["LS"], 128))
                tmp_f[1, pl.ds(r, cfg["LS"]), :] = jnp.broadcast_to(lax.rsqrt(var + 1e-5), (cfg["LS"], 128))
                return carry

            def ops(i, carry):
                r = pl.multiple_of(i * LB, LB)
                rows = pl.ds(pl.multiple_of(u * 128 + r, LB), LB)
                for c in range(2):
                    def xn(a, k):
                        xv = xbuf[pl.ds(u * 512 + a * 128 + r, LB), pl.ds((2 * k + c) * 128, 128)]
                        st = pl.ds(a * 128 + r, LB)
                        return (xv.astype(F32) - tmp_f[0, st, :]) * tmp_f[1, st, :]

                    blk = [[xn(a, k) for k in range(4)] for a in range(4)]
                    for p2 in range(NP):
                        inner = [_lin(LHS[p2], [blk[2 * a + a2][2 * b + b2] for a2, b2 in QUADS])
                                 for a, b in QUADS]
                        for a, b in ((0, 1), (1, 0)):
                            aop[inner_index(a, b) + p2, c, rows, :] = inner[2 * a + b].astype(BF16)
                        for p in range(NP):
                            aop[p * NP + p2, c, rows, :] = _lin(LHS[p], inner).astype(BF16)
                return carry

            lax.fori_loop(0, 512 // cfg["LS"], stats, 0)
            lax.fori_loop(0, 128 // LB, ops, 0)
            return carry

        with jax.named_scope("ph0"):
            lax.fori_loop(0, NU, ln_chunk, 0)

        def pinned(never, tok):
            if tok is None:
                return lambda v: v
            return lambda v: jnp.where(never, tok, v)

        def prep_wd(j, i, c, pin):
            def raw(kq, nq):
                v = wd_buf[j % 2, pl.ds((kq ^ 2) * 128 + i, 16), pl.ds((2 * nq + c) * 128, 128)]
                return pin(v.astype(F32))

            blk = [[raw(kq, nq) for nq in range(4)] for kq in range(4)]
            rows = pl.ds(pl.multiple_of(j * 128 + i, 16), 16)
            for p in range(NP):
                w = [_lin(RHS[p], [blk[2 * b + b2][2 * n + n2] for b, n in QUADS]) for b2, n2 in QUADS]
                for p2 in range(NP):
                    wdop[p * NP + p2, c, rows, :] = _lin(RHS[p2], w).astype(BF16)

        def up_step(j, carry):
            g_copy(j).wait()
            u_copy(j).wait()
            d_copy(j).wait()

            @pl.when(j + 1 < NJ)
            def _():
                g_copy(j + 1).start()
                u_copy(j + 1).start()
                d_copy(j + 1).start()

            @pl.when(j + 1 == NJ)
            def _():
                for cp in w_copies(0):
                    cp.start()

            count = [0]

            def raw(kq, cq):
                idx = (j % 2, pl.ds(kq * 256, 256), pl.ds(cq * 128, 128))
                return _cat([wg_buf[idx], wu_buf[idx]])

            def outer(p):
                w = [_lin(RHS[p], [functools.partial(raw, 2 * b + b2, 2 * c + c2) for b, c in QUADS])
                     for b2, c2 in QUADS]

                def inner(p2):
                    m = _dot(_cat(operand(aop, (p * NP + p2, c), 0, 512) for c in range(2)),
                             _lin(RHS[p2], w).astype(BF16))
                    n = count[0] - cfg["wd0"]
                    if 0 <= n < 16:
                        prep_wd(j, (n // 2) * 16, n % 2, pinned(j < 0, m[:16, :128] if cfg["pin1"] else None))
                    count[0] += 1
                    return m

                return _quadrants(inner, orders["o_up2"])

            blocks = [None] * 4

            def done(q, vals):
                h = [_gelu(_lanes(v, 0)) * _lanes(v, 1) for v in vals]
                blocks[q ^ 1] = [_lin(LHS[p2], h) for p2 in range(NP)]
                for p in range(NP):
                    used = [i for i in range(4) if LHS[p][i]]
                    if q ^ 1 in used and all(blocks[i] is not None for i in used):
                        for p2 in range(NP):
                            quads = [b and b[p2] for b in blocks]
                            hop[p * NP + p2, j] = _lin(LHS[p], quads).astype(BF16)

            _strassen(outer, done, orders["o_up"])
            return carry

        with jax.named_scope("ph1"):
            lax.fori_loop(0, NJ, up_step, 0)

        def prep_qkv(u, m, pin):
            w = pltpu.bitcast(wqkv_buf[u % 2, :, pl.ds(m * D, D)], U32)
            tmp_u[m] = pin(w).T
            w = jnp.concatenate([tmp_u[m, pl.ds(d, H, stride=DH), :] for d in range(DH)], axis=0)
            w = pltpu.bitcast(w.T, BF16)
            rows = pl.ds(pl.multiple_of(u * 128, 128), 128)
            for c in range(4):
                quads = [_lanes(w[b2 * 128:(b2 + 1) * 128], c + 4 * n) for b2, n in QUADS]
                for p in range(NP):
                    wqop[m, p, c, rows, :] = _lin(RHS[p], quads).astype(BF16)

        def prep_wo(u, pin):
            for s in range(2):
                tmp_f[s] = pin(wo_buf[u % 2, s].astype(F32))
            for d in range(DH // 2):
                quads = [tmp_f[n, pl.ds(d + b * (DH // 2), H, stride=DH), :] for b, n in QUADS]
                for p in range(NP):
                    woop[p, u, pl.ds(d * H, H), :] = _lin(RHS[p], quads).astype(BF16)

        def down_step(u, carry):
            for cp in w_copies(u):
                cp.wait()

            @pl.when(u + 1 < NU)
            def _():
                for cp in w_copies(u + 1):
                    cp.start()

            r0 = pl.multiple_of(u * 128, 128)
            count = [0]

            def outer(p):
                def inner(p2):
                    m = _dot(_cat(operand(hop, (p * NP + p2, j), r0, 128) for j in range(NJ)),
                             _cat(operand(wdop, (p * NP + p2, c), 0, F // 4) for c in range(2)))
                    n, rem = divmod(count[0], cfg["gap"])
                    if rem == 0 and n < 3:
                        tok = jnp.tile(pltpu.bitcast(m[:8, :128], U32), (16, 8))
                        prep_qkv(u, n, pinned(u < 0, tok if cfg["pin1"] else None))
                    if rem == 0 and n == 3:
                        tok = jnp.tile(m[:8, :128], (128, 1))
                        prep_wo(u, pinned(u < 0, tok if cfg["pin1"] else None))
                    count[0] += 1
                    return m

                return _quadrants(inner, orders["o_dn2"])

            def done(q, vals):
                a, n = QUADS[q]
                for (a2, n2), d in zip(QUADS, vals):
                    g = (d * jax.nn.sigmoid(d)).astype(BF16)
                    for c in range(2):
                        aop[(*gate_slot(a, a2, 4 * n + 2 * n2 + c), pl.ds(r0, 128))] = _lanes(g, c)

            _strassen(outer, done, orders["o_dn"])
            return carry

        with jax.named_scope("ph2"):
            lax.fori_loop(0, NU, down_step, 0)

    pl.run_scoped(
        ffn,
        pltpu.VMEM((NP * NP, NJ, S // 4, 128), BF16),
        pltpu.VMEM((NP * NP, 2, F // 4, 128), BF16),
        pltpu.VMEM((2, D, 512), BF16),
        pltpu.VMEM((2, D, 512), BF16),
        pltpu.VMEM((2, 512, D), BF16),
        pltpu.VMEM((2, 256, 3 * D), BF16),
        pltpu.VMEM((2, 2, D, 128), BF16),
        pltpu.VMEM((3, D, 128), U32),
        pltpu.VMEM((2, D, 128), F32),
    )

    scale = DH ** -0.5

    def attention(q_s, k_s, v_s, p_s, oop):

        def probs(u, r, pin):
            lg = [None] * WIN
            for c in range(8):
                qv = pin(q_s[c, pl.ds(r, RB), :])
                for w in range(WIN):
                    pr = qv * k_s[c, pl.ds(HALO + r - DIL * w, RB), :]
                    lg[w] = pr if c == 0 else lg[w] + pr
            lg = [l + pltpu.roll(l, 64, 1) for l in lg]
            lg = [(l + pltpu.roll(l, 32, 1)) * scale for l in lg]
            for w in range(WIN):
                if r < DIL * w:
                    pos = u * 512 + r + lax.broadcasted_iota(jnp.int32, (RB, 128), 0)
                    lg[w] = jnp.where(pos >= DIL * w, lg[w], -1e9)
            mx = functools.reduce(jnp.maximum, lg)
            e = [jnp.exp(l - mx) for l in lg]
            inv = 1.0 / functools.reduce(jnp.add, e)
            for w in range(WIN):
                p_s[w, pl.ds(r, RB), :] = e[w] * inv

        def mix(a, i, pin):
            pw = [[pin(p_s[w, pl.ds(a * 256 + a2 * 128 + i, 16), :]) for w in range(WIN)] for a2 in range(2)]

            def out(a2, c):
                r = a * 256 + a2 * 128 + i
                terms = [pw[a2][w] * v_s[c, pl.ds(HALO + r - DIL * w, 16), :] for w in range(WIN)]
                return functools.reduce(jnp.add, terms)

            for c in range(4):
                quads = [out(a2, c + 4 * b) for a2, b in QUADS]
                for p in range(NP):
                    oop[a, p, c, pl.ds(i, 16), :] = _lin(LHS[p], quads).astype(BF16)

        def chunk(u, carry):
            r0 = pl.multiple_of(u * 128, 128)
            never = u < 0
            for c in range(8):
                k_s[c, pl.ds(0, HALO), :] = jnp.where(u > 0, k_s[c, pl.ds(512, HALO), :], 0.0)
            v_old = [v_s[c, pl.ds(512, HALO), :] for c in range(8)]

            def project(m, a, dst, off):
                ms = []

                def product(p):
                    lhs = _cat(operand(aop, (inner_index(a, b) + p, c), r0, 128) for b, c in QUADS)
                    ms.append(_dot(lhs, _cat(operand(wqop, (m, p, c), 0, 512) for c in range(4))))
                    return ms[-1]

                for (a2, n), val in zip(QUADS, _quadrants(product, orders["o_at"])):
                    for c in range(4):
                        dst[4 * n + c, pl.ds(off + a * 256 + a2 * 128, 128), :] = _lanes(val, c)
                return ms

            def output(a):
                ms = []

                def product(p):
                    ms.append(_dot(_cat(operand(oop, (a, p, c), 0, 128) for c in range(4)),
                                   _cat(operand(woop, (p, c), 0, 512) for c in range(4))))
                    return ms[-1]

                for (a2, n), val in zip(QUADS, _quadrants(product, orders["o_at"])):
                    rows = pl.ds(pl.multiple_of(u * 512 + a * 256 + a2 * 128, 128), 128)
                    for c in range(4):
                        cols = pl.ds((4 * n + c) * 128, 128)
                        g = aop[(*gate_slot(a, a2, 4 * n + c), pl.ds(r0, 128))].astype(F32)
                        xbuf[rows, cols] = (xbuf[rows, cols].astype(F32) + _lanes(val, c) * g).astype(BF16)
                o_copy(2 * u + a).start()
                return ms

            def spread(ms, n, rows, span, work):
                for i in range(n):
                    pos = int(i * span * len(ms) * 4 / n) - 1
                    if pos < 0 or not cfg["pin2"]:
                        work(i, lambda v: v)
                    else:
                        tok = _lanes(ms[pos // 4], pos % 4)[128 - rows:]
                        work(i, lambda v: jnp.where(never, tok, v))

            project(1, 0, k_s, HALO)
            project(0, 0, q_s, 0)
            ms = project(1, 1, k_s, HALO) + project(0, 1, q_s, 0)
            spread(ms, 256 // RB, RB, cfg["s1"], lambda i, pin: probs(u, i * RB, pin))
            ms = project(2, 0, v_s, HALO)
            for c in range(8):
                first = jnp.broadcast_to(v_s[c, pl.ds(HALO, 1), :], (HALO, 128))
                v_s[c, pl.ds(0, HALO), :] = jnp.where(u > 0, v_old[c], first)
            spread(ms, 256 // RB, RB, cfg["s2"], lambda i, pin: probs(u, 256 + i * RB, pin))
            ms = project(2, 1, v_s, HALO)
            spread(ms, 8, 16, cfg["s3"], lambda i, pin: mix(0, i * 16, pin))
            ms = output(0)
            spread(ms, 8, 16, cfg["s3"], lambda i, pin: mix(1, i * 16, pin))
            output(1)
            return carry

        with jax.named_scope("ph3"):
            lax.fori_loop(0, NU, chunk, 0)

    pl.run_scoped(
        attention,
        pltpu.VMEM((8, 512, 128), F32),
        pltpu.VMEM((8, HALO + 512, 128), F32),
        pltpu.VMEM((8, HALO + 512, 128), F32),
        pltpu.VMEM((WIN, 512, 128), F32),
        pltpu.VMEM((2, NP, 4, 128, 128), BF16),
    )
    for t in range(2 * NU):
        o_copy(t).wait()


DEFAULT = dict(RB=8, LS=64, cast=True, pin1=True, pin2=True, wd0=1, gap=7, s1=0.95, s2=0.95, s3=0.8,
               o_up="1023456", o_up2="1023456", o_dn="0123456", o_dn2="0123456", o_at="0123456")


def make(flags=None, interpret=False, **kw):
    cfg = dict(DEFAULT, **kw)

    def f(A_x, A_wqkv, A_wo, B_x, B_w_gate, B_w_up, B_w_down):
        del B_x
        any_spec = pl.BlockSpec(memory_space=pl.ANY)
        out = pl.pallas_call(
            functools.partial(_kernel, cfg=cfg),
            out_shape=jax.ShapeDtypeStruct((S, D), BF16),
            in_specs=[any_spec] * 6,
            out_specs=any_spec,
            scratch_shapes=[
                pltpu.VMEM((S, D), BF16),
                pltpu.VMEM((NP * (NP + 2), 2, S // 4, 128), BF16),
                pltpu.VMEM((3, NP, 4, D // 2, 128), BF16),
                pltpu.VMEM((NP, 4, D // 2, 128), BF16),
                pltpu.SemaphoreType.DMA((NU,)),
                pltpu.SemaphoreType.DMA((2,)),
                pltpu.SemaphoreType.DMA((2,)),
                pltpu.SemaphoreType.DMA((2,)),
                pltpu.SemaphoreType.DMA((8,)),
                pltpu.SemaphoreType.DMA((2 * NU,)),
            ],
            compiler_params=pltpu.CompilerParams(
                vmem_limit_bytes=127 * 2**20, **({"flags": flags} if flags else {})),
            name="fused_block",
            interpret=interpret,
        )(A_x.reshape(S, D), A_wqkv, A_wo, B_w_gate, B_w_up, B_w_down)
        return out.reshape(1, S, D)

    return f


@jax.jit
def pallas_recurrent_scan__sliding_local_dilated__geglu_ffn__prompt_kernel(
    A_x: jax.Array,
    A_wqkv: jax.Array,
    A_wo: jax.Array,
    B_x: jax.Array,
    B_w_gate: jax.Array,
    B_w_up: jax.Array,
    B_w_down: jax.Array,
):
    return make()(A_x, A_wqkv, A_wo, B_x, B_w_gate, B_w_up, B_w_down)
```

```python
import functools

import jax
import jax.numpy as jnp
from jax import lax
import jax.experimental.pallas as pl
import jax.experimental.pallas.tpu as pltpu

F32 = jnp.float32
BF16 = jnp.bfloat16
U32 = jnp.uint32

S, D, F = 2048, 1024, 3584
H, DH, WIN, DIL = 32, 32, 8, 2
HALO = 16
PITCH = DH + 1
NJ = F // 512
NU = S // 512
Q = 64
NT = S // (4 * Q)

LHS = ((1, 0, 0, 1), (0, 0, 1, 1), (1, 0, 0, 0), (0, 0, 0, 1),
       (1, 1, 0, 0), (-1, 0, 1, 0), (0, 1, 0, -1))
RHS = ((1, 0, 0, 1), (1, 0, 0, 0), (0, 1, 0, -1), (-1, 0, 1, 0),
       (0, 0, 0, 1), (1, 1, 0, 0), (0, 0, 1, 1))
OUT = ((1, 0, 0, 1), (0, 0, 1, -1), (0, 1, 0, 1), (1, 0, 1, 0),
       (-1, 1, 0, 0), (0, 0, 0, 1), (1, 0, 0, 0))
NP = 7
QUADS = ((0, 0), (0, 1), (1, 0), (1, 1))


def _lin(coef, quads):
    idx = sorted((i for i, c in enumerate(coef) if c), key=lambda i: -coef[i])
    get = lambda i: quads[i]() if callable(quads[i]) else quads[i]
    if len(idx) == 1:
        return get(idx[0])
    a, b = get(idx[0]).astype(F32), get(idx[1]).astype(F32)
    return a + b if coef[idx[1]] > 0 else a - b


def _strassen(product, done, order):
    acc = [None] * 4
    left = [sum(1 for p in range(NP) if OUT[p][q]) for q in range(4)]
    for p in order:
        m = product(p)
        for q in range(4):
            s = OUT[p][q]
            if s == 0:
                continue
            if acc[q] is None:
                acc[q] = (s, m)
            else:
                s0, c = acc[q]
                assert s > 0 or s0 > 0
                acc[q] = (1, [x + y if s == s0 else (x - y if s > 0 else y - x)
                              for x, y in zip(m, c)])
            left[q] -= 1
            if left[q] == 0:
                done(q, acc[q][1])


def _quadrants(product, order):
    out = [None] * 4

    def done(q, val):
        out[q] = val[0]

    _strassen(lambda p: [product(p)], done, order)
    return out


def _dot(a, b):
    return jnp.dot(a, b, preferred_element_type=F32)


def _cat(xs):
    return jnp.concatenate(list(xs), axis=1)


def _lanes(v, c):
    return v[:, c * 128:(c + 1) * 128]


def _gelu(g):
    hg = 0.5 * g
    t = jnp.tanh(g * (0.7978845608028654 + 0.035677408136300125 * (g * g)))
    return hg * t + hg


def _silu(d):
    hd = 0.5 * d
    return hd * jnp.tanh(hd) + hd


class _Filler:
    def __init__(self, never=None, lag=0):
        self.todo, self.pos = [], 0
        self.never, self.lag, self.marks = never, lag, []

    def hold(self, a):
        rows = [a[r:r + 8] for r in range(0, a.shape[0], 8)]
        while self.marks and self.marks[0][0] < self.pos + 1:
            when, mark = self.marks.pop(0)
            r = int(max(when - self.pos, 0) * len(rows))
            rows[r] = jnp.where(self.never, mark, rows[r])
        return jnp.concatenate(rows, axis=0)

    def plan(self, first, last, pieces):
        self.todo += [(self.pos + first + i * (last - first) / len(pieces), piece)
                      for i, piece in enumerate(pieces)]

    def dot(self, a, b, rows_first=False):
        m = _dot(a, b)
        nr, nc = m.shape[0] // 8, m.shape[1] // 128
        while self.todo and self.todo[0][0] < self.pos + 1:
            when, (fence, work) = self.todo.pop(0)
            i = int(max(when - self.pos, 0) * nr * nc)
            r, c = divmod(i, nc) if rows_first else divmod(i, nr)[::-1]
            if fence is not None:
                fence(_lanes(m, c)[8 * r:8 * r + 8])
            mark = work()
            if self.lag and mark is not None:
                self.marks.append((when + self.lag, mark()))
        self.pos += 1
        return m


def _kernel(x_hbm, wqkv_hbm, wo_hbm, wg_hbm, wu_hbm, wd_hbm, out_hbm,
            xbuf, aop, wqop, woop, sem_x, sem_g, sem_u, sem_d, sem_w, sem_o, *, cfg):
    RB = cfg["RB"]
    orders = {k: [int(c) for c in v] for k, v in cfg.items() if k.startswith("o_")}

    def operand(ref, lead, start, size):
        if cfg["cast"]:
            if not isinstance(start, int):
                start2 = pl.multiple_of(start >> 1, size // 2)
            else:
                start2 = start // 2
            return pltpu.bitcast(ref.bitcast(U32)[(*lead, pl.ds(start2, size // 2))], BF16)
        return ref[(*lead, pl.ds(start, size))]

    def x_copies(u):
        rows = pl.ds(pl.multiple_of(u * 4 * Q, 4 * Q), 4 * Q)
        return [pltpu.make_async_copy(x_hbm.at[rows, pl.ds(c * 128, 128)], xbuf.at[c, rows], sem_x.at[u])
                for c in range(8)]

    def inner_index(a, b):
        return {(0, 0): 2, (1, 1): 3, (0, 1): 7, (1, 0): 8}[a, b] * NP

    def gate_slot(a, a2, c):
        return 4 * NP + (2 * a + a2) * 4 + c // 2, c % 2

    def ffn(hop, wdop, wg0, wg1, wu0, wu1, wd_buf, wqkv_buf, wo_buf, tmp_u, tmp_f, *h_s):

        def early_copies(j):
            cols = pl.ds(pl.multiple_of(j * 512, 256), 256)
            return [pltpu.make_async_copy(src.at[:, cols], dst.at[j & 1], sem_g.at[j & 1])
                    for src, dst in ((wg_hbm, wg0), (wu_hbm, wu0))]

        def late_copies(j):
            cols = pl.ds(pl.multiple_of(j * 512 + 256, 256), 256)
            rows = pl.ds(pl.multiple_of(j * 512, 512), 512)
            return [pltpu.make_async_copy(src.at[:, cols], dst.at[j & 1], sem_u.at[j & 1])
                    for src, dst in ((wg_hbm, wg1), (wu_hbm, wu1))] + [
                pltpu.make_async_copy(wd_hbm.at[rows], wd_buf.at[j & 1, pl.ds(0, 512)], sem_u.at[j & 1])]

        def w_copies(u):
            slot = u & 1
            r0 = (u >> 1) * 512 + (u & 1) * 128
            cs = [pltpu.make_async_copy(
                wqkv_hbm.at[pl.ds(pl.multiple_of(r0 + 256 * s, 128), 128)],
                wqkv_buf.at[slot, pl.ds(128 * s, 128)], sem_w.at[4 * slot + s]) for s in range(2)]
            cs += [pltpu.make_async_copy(
                wo_hbm.at[:, pl.ds(pl.multiple_of((u + 4 * s) * 128, 128), 128)],
                wo_buf.at[slot, s, pl.ds(0, D)], sem_w.at[4 * slot + 2 + s]) for s in range(2)]
            return cs

        for u in range(NT):
            for cp in x_copies(u):
                cp.start()
        for cp in early_copies(0):
            cp.start()

        LB = 16
        NL = S // (4 * LB)
        sum_s, mean_s, sq_s, rstd_s = h_s

        def x_rows(i, a, c):
            return operand(xbuf, (c,), (i >> 2) * 4 * Q + a * Q + (i & 3) * LB, LB).astype(F32)

        def lane_mean(v):
            return jnp.broadcast_to(jnp.sum(v, axis=-1, keepdims=True) * (1.0 / D), v.shape)

        def ln_sum(i, a, rows):
            sum_s[a, rows, :] = functools.reduce(jnp.add, [x_rows(i, a, c) for c in range(8)])

        def ln_mean(i, a, rows):
            mean_s[a, rows, :] = lane_mean(sum_s[a, rows, :])

        def ln_squares(i, a, rows):
            xc = [x_rows(i, a, c) - mean_s[a, rows, :] for c in range(8)]
            sq_s[a, rows, :] = functools.reduce(jnp.add, [v * v for v in xc])

        def ln_rstd(i, a, rows):
            rstd_s[a, rows, :] = lax.rsqrt(lane_mean(sq_s[a, rows, :]) + 1e-5)

        def ln_operands(i):
            rows = pl.ds(pl.multiple_of(i * LB, LB), LB)
            for c in range(2):
                blk = [[(x_rows(i, a, 2 * k + c) - mean_s[a, rows, :]) * rstd_s[a, rows, :] for k in range(4)]
                       for a in range(4)]
                for p2 in range(NP):
                    inner = [_lin(LHS[p2], [blk[2 * a + a2][2 * b + b2] for a2, b2 in QUADS])
                             for a, b in QUADS]
                    for a, b in ((0, 1), (1, 0)):
                        aop[inner_index(a, b) + p2, c, rows, :] = inner[2 * a + b].astype(BF16)
                    for p in range(NP):
                        aop[p * NP + p2, c, rows, :] = _lin(LHS[p], inner).astype(BF16)

        def ln_step(i, lo=0, hi=5):
            if lo <= 4 < hi:
                ln_operands(i - 4)
            for s, stage in ((3, ln_rstd), (2, ln_squares), (1, ln_mean), (0, ln_sum)):
                if lo <= s < hi:
                    for a in range(4):
                        stage(i - s, a, pl.ds(pl.multiple_of((i - s) * LB, LB), LB))

        def ln_chunk(u, carry):
            for cp in x_copies(u):
                cp.wait()
            lax.fori_loop(4 * u, 4 * u + 4, lambda i, c: ln_step(i) or c, 0)
            return carry

        for cp in late_copies(0):
            cp.start()
        if "0" in cfg["only"]:
          with jax.named_scope("ph0"):
            for cp in x_copies(0):
                cp.wait()
            for i in range(4):
                ln_step(i, hi=i + 1)
            lax.fori_loop(1, NT, ln_chunk, 0)
            for i in range(4):
                ln_step(NL + i, lo=i + 1)

        def prep_wd(j):
            def fence(v):
                wd_buf[j >> 3, pl.ds(512, 16), pl.ds(0, 128)] = pltpu.bitcast(v, BF16)

            def work(i, c, ps):
                def raw(kq, nq):
                    return wd_buf[j & 1, pl.ds((kq ^ 2) * 128 + i, 16), pl.ds((2 * nq + c) * 128, 128)]

                rows = pl.ds(pl.multiple_of(j * 128 + i, 16), 16)
                for p in ps:
                    w = [_lin(RHS[p], [functools.partial(raw, 2 * b + b2, 2 * n + n2) for b, n in QUADS])
                         for b2, n2 in QUADS]
                    for p2 in range(NP):
                        wdop[p * NP + p2, c, rows, :] = _lin(RHS[p2], w).astype(BF16)
                return lambda: wdop.bitcast(U32)[j >> 3, 0, pl.ds(0, 8), :]

            return [(fence, functools.partial(work, i, c, ps))
                    for i in range(0, 128, 16) for c in range(2) for ps in cfg["wdp"]]

        def prep_h(j, ps):
            def fence(p, v):
                q = max(q for q in range(4) if LHS[p][q])
                h_s[q][j >> 3, pl.ds(512, 8), :] = v

            def work(i, p):
                rows = pl.ds(i, 16)
                w = [_lin(LHS[p], [functools.partial(lambda q: h_s[q][q2, rows, :], q) for q in range(4)])
                     for q2 in range(4)]
                for p2 in range(NP):
                    hop[p * NP + p2, j, rows, :] = _lin(LHS[p2], w).astype(BF16)
                return lambda: hop.bitcast(U32)[j >> 3, 0, pl.ds(0, 8), :]

            return [(functools.partial(fence, p), functools.partial(work, i, p))
                    for i in range(0, 512, 16) for p in ps]

        def up_step(j, carry):
            for cp in early_copies(j):
                cp.wait()
            if not cfg["mid"]:
                for cp in late_copies(j):
                    cp.wait()

            @pl.when(j + 1 < NJ)
            def _():
                for cp in early_copies(j + 1) + late_copies(j + 1):
                    cp.start()

            @pl.when(j + 1 == NJ)
            def _():
                for cp in w_copies(0):
                    cp.start()

            fill = _Filler(j < 0, cfg["lag"])
            fill.plan(cfg["wd0"], cfg["wd1"], prep_wd(j))
            fill.plan(cfg["hp"][0][1], cfg["hp"][0][2], prep_h(jnp.maximum(j - 1, 0), cfg["hp"][0][0]))
            for ps, first, last in cfg["hp"][1:]:
                fill.plan(first, last, prep_h(j, ps))
            fill.todo.sort(key=lambda t: t[0])

            def raw(kq, cq):
                idx = (j & 1, pl.ds(kq * 256, 256), pl.ds((cq % 2) * 128, 128))
                return _cat([wg1[idx], wu1[idx]] if cq // 2 else [wg0[idx], wu0[idx]])

            def outer(p):
                w = [_lin(RHS[p], [functools.partial(raw, 2 * b + b2, 2 * c + c2) for b, c in QUADS])
                     for b2, c2 in QUADS]

                def inner(p2):
                    if fill.pos == cfg["mid"] and cfg["mid"]:
                        for cp in late_copies(j):
                            cp.wait()
                    lhs = [aop.bitcast(U32)[p * NP + p2, c] for c in range(2)]
                    lhs[0] = fill.hold(lhs[0])
                    return fill.dot(_cat(pltpu.bitcast(x, BF16) for x in lhs),
                                    _lin(RHS[p2], w).astype(BF16), rows_first=True)

                return _quadrants(inner, orders["o_up2"])

            def done(q, vals):
                for q2, v in enumerate(vals):
                    h_s[q ^ 1][q2, pl.ds(0, 512), :] = _gelu(_lanes(v, 0)) * _lanes(v, 1)

            _strassen(outer, done, orders["o_up"])
            return carry

        if "1" in cfg["only"]:
          with jax.named_scope("ph1"):
            lax.fori_loop(0, NJ, up_step, 0)
            for _, work in prep_h(NJ - 1, cfg["hp"][0][0]):
                work()

        def prep_qkv(u):
            def fence_in(v):
                wqkv_buf[u >> 3, pl.ds(256, 16), pl.ds(0, 128)] = pltpu.bitcast(v, BF16)

            def fence_tmp(v):
                tmp_u[u >> 3, pl.ds(H * PITCH, 8), :] = pltpu.bitcast(v, U32)

            def scatter(m, c):
                w = pltpu.bitcast(wqkv_buf[u & 1, pl.ds(0, 256), pl.ds(m * D + c * 128, 128)], U32).T
                for h in range(4):
                    tmp_u[m, pl.ds((4 * c + h) * PITCH, DH), :] = w[h * DH:(h + 1) * DH]

            def gather(m, c):
                w = [jnp.concatenate([tmp_u[m, pl.ds(4 * cc + d, H, stride=PITCH), :] for d in range(4)], axis=0)
                     for cc in (c, c + 4)]
                w = [pltpu.bitcast(x.T, BF16) for x in w]
                quads = [w[n][b2 * 128:(b2 + 1) * 128] for b2, n in QUADS]
                for p in range(NP):
                    rows = pl.ds(pl.multiple_of(u * 128, 128), 128)
                    wqop[m, p, c, rows, :] = _lin(RHS[p], quads).astype(BF16)

            return ([(fence_in, functools.partial(scatter, m, c)) for m in range(3) for c in range(8)],
                    [(fence_tmp, functools.partial(gather, m, c)) for m in range(3) for c in range(4)])

        def prep_wo(u):
            def fence_in(v):
                wo_buf[u >> 3, 0, pl.ds(D, 16), :] = pltpu.bitcast(v, BF16)

            def fence_tmp(v):
                tmp_f[u >> 3, pl.ds(H * PITCH, 8), :] = v

            def scatter(h):
                for s in range(2):
                    tmp_f[s, pl.ds(h * PITCH, DH), :] = wo_buf[u & 1, s, pl.ds(h * DH, DH), :].astype(F32)

            def gather(d):
                quads = [tmp_f[n, pl.ds(d + b * (DH // 2), H, stride=PITCH), :] for b, n in QUADS]
                for p in range(NP):
                    woop[p, u, pl.ds(d * H, H), :] = _lin(RHS[p], quads).astype(BF16)

            return ([(fence_in, functools.partial(scatter, h)) for h in range(H)]
                    + [(fence_tmp, functools.partial(gather, d)) for d in range(DH // 2)])

        def down_step(u, carry):
            for cp in w_copies(u):
                cp.wait()

            @pl.when(u + 1 < NU)
            def _():
                for cp in w_copies(u + 1):
                    cp.start()

            r0 = pl.multiple_of(u * 128, 128)
            fill = _Filler()
            scatter, gather = prep_qkv(u)
            fill.plan(0, cfg["d1"], scatter)
            fill.plan(cfg["d1"], cfg["d2"], prep_wo(u))
            fill.plan(cfg["d2"], cfg["d3"], gather)

            def outer(p):
                def inner(p2):
                    return fill.dot(_cat(operand(hop, (p * NP + p2, j), r0, 128) for j in range(NJ)),
                                    _cat(operand(wdop, (p * NP + p2, c), 0, F // 4) for c in range(2)))

                return _quadrants(inner, orders["o_dn2"])

            def done(q, vals):
                a, n = QUADS[q]
                for (a2, n2), d in zip(QUADS, vals):
                    g = _silu(d).astype(BF16)
                    for c in range(2):
                        aop[(*gate_slot(a, a2, 4 * n + 2 * n2 + c), pl.ds(r0, 128))] = _lanes(g, c)

            _strassen(outer, done, orders["o_dn"])
            return carry

        if "2" in cfg["only"]:
          with jax.named_scope("ph2"):
            lax.fori_loop(0, NU, down_step, 0)

    pl.run_scoped(
        ffn,
        pltpu.VMEM((NP * NP, NJ, S // 4, 128), BF16),
        pltpu.VMEM((NP * NP, 2, F // 4, 128), BF16),
        *[pltpu.VMEM((2, D, 256), BF16)] * 4,
        pltpu.VMEM((2, 512 + 16, D), BF16),
        pltpu.VMEM((2, 256 + 16, 3 * D), BF16),
        pltpu.VMEM((2, 2, D + 16, 128), BF16),
        pltpu.VMEM((3, H * PITCH + 8, 128), U32),
        pltpu.VMEM((2, H * PITCH + 8, 128), F32),
        *[pltpu.VMEM((4, 512 + 8, 128), F32)] * 4,
    )

    scale = DH ** -0.5

    def attention(q_s, k0, k1, v0, v1, p_s, oop, obuf):
        def o_copies(t):
            rows = pl.ds(pl.multiple_of(t * 2 * Q, 2 * Q), 2 * Q)
            return [pltpu.make_async_copy(obuf.at[c, rows], out_hbm.at[rows, pl.ds(c * 128, 128)], sem_o.at[t])
                    for c in range(8)]

        k_s, v_s = (k0, k1), (v0, v1)

        def chunk(u, carry):
            r0 = pl.multiple_of(u * Q, Q)
            fill = _Filler()

            def fence(ref):
                def park(v):
                    ref[u, pl.ds(HALO + 2 * Q, 8), :] = v
                return park

            def probs(a):
                pieces = []
                for r in range(0, 2 * Q, RB):
                    lg = [None] * WIN

                    def logits(c, r=r, lg=lg):
                        qv = q_s[c, pl.ds(a * 2 * Q + r, RB), :]
                        for w in range(WIN):
                            pr = qv * k_s[a][c, pl.ds(HALO + r - DIL * w, RB), :]
                            lg[w] = pr if c == 0 else lg[w] + pr

                    def softmax(r=r, lg=lg):
                        lg = [l + pltpu.roll(l, 64, 1) for l in lg]
                        lg = [(l + pltpu.roll(l, 32, 1)) * scale for l in lg]
                        for w in range(WIN):
                            if a == 0 and r < DIL * w:
                                pos = u * 4 * Q + r + lax.broadcasted_iota(jnp.int32, (RB, 128), 0)
                                lg[w] = jnp.where(pos >= DIL * w, lg[w], -1e9)
                        mx = functools.reduce(jnp.maximum, lg)
                        e = [jnp.exp(l - mx) for l in lg]
                        inv = 1.0 / functools.reduce(jnp.add, e)
                        for w in range(WIN):
                            p_s[w, pl.ds(a * 2 * Q + r, RB), :] = e[w] * inv

                    pieces += [(fence(k_s[a]) if c % cfg["cq"] == 0 else None, functools.partial(logits, c))
                               for c in range(8)]
                    pieces.append((None, softmax))
                return pieces

            def mix(a):
                pieces = []
                for i in range(0, Q, 16):
                    for c in range(4):
                        outs = []

                        def part(r, cc, outs=outs):
                            terms = [p_s[w, pl.ds(a * 2 * Q + r, 8), :]
                                     * v_s[a][cc, pl.ds(HALO + r - DIL * w, 8), :] for w in range(WIN)]
                            outs.append(functools.reduce(jnp.add, terms))

                        def store(i=i, c=c, outs=outs):
                            quads = [jnp.concatenate(outs[2 * q:2 * q + 2], axis=0) for q in range(4)]
                            for p in range(NP):
                                oop[a, p, c, pl.ds(i, 16), :] = _lin(LHS[p], quads).astype(BF16)

                        pieces += [(fence(v_s[a]) if (4 * a2 + 2 * b + s) % cfg["cv"] == 0 else None,
                                    functools.partial(part, a2 * Q + i + 8 * s, c + 4 * b))
                                   for a2, b in QUADS for s in range(2)]
                        pieces.append((None, store))
                return pieces

            def project(m, a, dst, off):
                def product(p):
                    lhs = _cat(operand(aop, (inner_index(a, b) + p, c), r0, Q) for b, c in QUADS)
                    return [fill.dot(lhs, _cat(operand(wqop, (m, p, c), 0, 512) for c in range(4)))]

                def done(q, val):
                    a2, n = QUADS[q]
                    for c in range(4):
                        dst[4 * n + c, pl.ds(off + a2 * Q, Q), :] = _lanes(val[0], c)

                _strassen(product, done, orders["o_at"])

            def output(a):
                def product(p):
                    return [fill.dot(_cat(operand(oop, (a, p, c), 0, Q) for c in range(4)),
                                     _cat(operand(woop, (p, c), 0, 512) for c in range(4)))]

                def done(q, val):
                    a2, n = QUADS[q]
                    rows = pl.ds(pl.multiple_of((4 * u + 2 * a + a2) * Q, Q), Q)
                    for c in range(4):
                        g = operand(aop, gate_slot(a, a2, 4 * n + c), r0, Q).astype(F32)
                        xv = operand(xbuf, (4 * n + c,), rows.start, Q).astype(F32)
                        obuf[4 * n + c, rows, :] = (xv + _lanes(val[0], c) * g).astype(BF16)

                _strassen(product, done, orders["o_wo"])
                for cp in o_copies(2 * u + a):
                    cp.start()

            tail = pl.ds(2 * Q, HALO)
            head = pl.ds(0, HALO)
            k0[:, head, :] = jnp.where(u > 0, k1[:, tail, :], 0.0)
            project(1, 0, k0, HALO)
            k1[:, head, :] = k0[:, tail, :]
            project(0, 0, q_s, 0)
            fill.plan(0, cfg["e1"], probs(0))
            project(1, 1, k1, HALO)
            project(0, 1, q_s, 2 * Q)
            fill.plan(0, cfg["e2"], probs(1))
            project(2, 0, v0, HALO)
            for c in range(8):
                first = jnp.broadcast_to(v0[c, pl.ds(HALO, 1), :], (HALO, 128))
                v0[c, head, :] = jnp.where(u > 0, v1[c, tail, :], first)
            v1[:, head, :] = v0[:, tail, :]
            fill.plan(0, cfg["e3"], mix(0))
            project(2, 1, v1, HALO)
            fill.plan(0, cfg["e3"], mix(1))
            output(0)
            assert not fill.todo
            output(1)
            return carry

        if "3" in cfg["only"]:
          with jax.named_scope("ph3"):
            lax.fori_loop(0, NT, chunk, 0)
        for t in range(2 * NT):
            for cp in o_copies(t):
                cp.wait()

    kv = pltpu.VMEM((8, HALO + 2 * Q + 8, 128), F32)
    pl.run_scoped(
        attention,
        pltpu.VMEM((8, 4 * Q, 128), F32), kv, kv, kv, kv,
        pltpu.VMEM((WIN, 4 * Q, 128), F32),
        pltpu.VMEM((2, NP, 4, Q, 128), BF16),
        pltpu.VMEM((8, S, 128), BF16),
    )


DEFAULT = dict(mid=0, late=22, lag=1, b=4, only='0123', up=3, lo=True, RB=8, LS=64, cast=True, pin1=True, pin2=True, wd0=14, wd1=36, hp=(((1,5,4,6),0.5,8),((3,),14,18),((0,2),28,36)), wdp=((0,1),(2,4),(3,),(5,),(6,)), d1=12, d2=22, d3=46, e1=13.5, e2=7, e3=6.5, cq=4, cv=2, o_wo='0123456',
               o_up="1324056", o_up2="1324056", o_dn="0123456", o_dn2="0123456", o_at="0123456")


def make(flags=None, interpret=False, **kw):
    cfg = dict(DEFAULT, **kw)

    def f(A_x, A_wqkv, A_wo, B_x, B_w_gate, B_w_up, B_w_down):
        del B_x
        any_spec = pl.BlockSpec(memory_space=pl.ANY)
        out = pl.pallas_call(
            functools.partial(_kernel, cfg=cfg),
            out_shape=jax.ShapeDtypeStruct((S, D), BF16),
            in_specs=[any_spec] * 6,
            out_specs=any_spec,
            scratch_shapes=[
                pltpu.VMEM((8, S, 128), BF16),
                pltpu.VMEM((NP * (NP + 2), 2, S // 4, 128), BF16),
                pltpu.VMEM((3, NP, 4, D // 2, 128), BF16),
                pltpu.VMEM((NP, 4, D // 2, 128), BF16),
                pltpu.SemaphoreType.DMA((NT,)),
                pltpu.SemaphoreType.DMA((2,)),
                pltpu.SemaphoreType.DMA((2,)),
                pltpu.SemaphoreType.DMA((2,)),
                pltpu.SemaphoreType.DMA((8,)),
                pltpu.SemaphoreType.DMA((2 * NT,)),
            ],
            compiler_params=pltpu.CompilerParams(
                vmem_limit_bytes=127 * 2**20, **({"flags": flags} if flags else {})),
            name="fused_block",
            interpret=interpret,
        )(A_x.reshape(S, D), A_wqkv, A_wo, B_w_gate, B_w_up, B_w_down)
        return out.reshape(1, S, D)

    return f


@jax.jit
def pallas_recurrent_scan__sliding_local_dilated__geglu_ffn__prompt_kernel(
    A_x: jax.Array,
    A_wqkv: jax.Array,
    A_wo: jax.Array,
    B_x: jax.Array,
    B_w_gate: jax.Array,
    B_w_up: jax.Array,
    B_w_down: jax.Array,
):
    return make()(A_x, A_wqkv, A_wo, B_x, B_w_gate, B_w_up, B_w_down)
```

```python
import functools

import jax
import jax.numpy as jnp
from jax import lax
import jax.experimental.pallas as pl
import jax.experimental.pallas.tpu as pltpu

F32 = jnp.float32
BF16 = jnp.bfloat16
U32 = jnp.uint32

S, D, F = 2048, 1024, 3584
H, DH, WIN, DIL = 32, 32, 8, 2
HALO = 16
PITCH = DH + 1
Q = 64
NT = S // (4 * Q)
NJ = F // 512
NU = S // 512

LHS = ((1, 0, 0, 1), (0, 0, 1, 1), (1, 0, 0, 0), (0, 0, 0, 1),
       (1, 1, 0, 0), (-1, 0, 1, 0), (0, 1, 0, -1))
RHS = ((1, 0, 0, 1), (1, 0, 0, 0), (0, 1, 0, -1), (-1, 0, 1, 0),
       (0, 0, 0, 1), (1, 1, 0, 0), (0, 0, 1, 1))
OUT = ((1, 0, 0, 1), (0, 0, 1, -1), (0, 1, 0, 1), (1, 0, 1, 0),
       (-1, 1, 0, 0), (0, 0, 0, 1), (1, 0, 0, 0))
NP = 7
QUADS = ((0, 0), (0, 1), (1, 0), (1, 1))


def _lin(coef, quad):
    idx = sorted((q for q, c in enumerate(coef) if c), key=lambda q: -coef[q])
    if len(idx) == 1:
        return quad(idx[0])
    a, b = quad(idx[0]).astype(F32), quad(idx[1]).astype(F32)
    return a + b if coef[idx[1]] > 0 else a - b


def _operands(coefs, p, block):
    w = [_lin(coefs[p], lambda q: block(q, q2)) for q2 in range(4)]
    return lambda p2: _lin(coefs[p2], w.__getitem__).astype(BF16)


def _quarter(q, q2):
    return 2 * (q // 2) + q2 // 2, 2 * (q % 2) + q2 % 2


def _strassen(product, done, order):
    acc = [None] * 4
    left = [sum(1 for p in range(NP) if OUT[p][q]) for q in range(4)]
    for p in order:
        m = product(p)
        for q in range(4):
            s = OUT[p][q]
            if s == 0:
                continue
            if acc[q] is None:
                acc[q] = (s, m)
            else:
                s0, c = acc[q]
                assert s > 0 or s0 > 0
                acc[q] = (1, [x + y if s == s0 else (x - y if s > 0 else y - x)
                              for x, y in zip(m, c)])
            left[q] -= 1
            if left[q] == 0:
                done(q, acc[q][1])


def _quadrants(product, order):
    out = [None] * 4

    def done(q, val):
        out[q] = val[0]

    _strassen(lambda p: [product(p)], done, order)
    return out


def _cat(xs):
    return jnp.concatenate(list(xs), axis=1)


def _lanes(v, c):
    return v[:, c * 128:(c + 1) * 128]


def _gelu(g):
    hg = 0.5 * g
    t = jnp.tanh(g * (0.7978845608028654 + 0.035677408136300125 * (g * g)))
    return hg * t + hg


def _silu(d):
    hd = 0.5 * d
    return hd * jnp.tanh(hd) + hd


def _rows(start, size):
    return pl.ds(start if isinstance(start, int) else pl.multiple_of(start, size), size)


def _words(ref, lead, start, size):
    return ref.bitcast(U32)[(*lead, _rows(start >> 1, size // 2))]


def _load(ref, lead, start, size):
    return pltpu.bitcast(_words(ref, lead, start, size), BF16)


class _Filler:
    def __init__(self, never=None, lag=0):
        self.todo, self.pos = [], 0
        self.never, self.lag, self.marks = never, lag, []

    def plan(self, first, last, pieces):
        self.todo += [(self.pos + first + i * (last - first) / len(pieces), piece)
                      for i, piece in enumerate(pieces)]
        self.todo.sort(key=lambda t: t[0])

    def hold(self, a):
        rows = [a[r:r + 8] for r in range(0, a.shape[0], 8)]
        while self.marks and self.marks[0][0] < self.pos + 1:
            when, mark = self.marks.pop(0)
            r = int(max(when - self.pos, 0) * len(rows))
            rows[r] = jnp.where(self.never, mark, rows[r])
        return jnp.concatenate(rows, axis=0)

    def dot(self, a, b):
        m = jnp.dot(a, b, preferred_element_type=F32)
        nr, nc = m.shape[0] // 8, m.shape[1] // 128
        while self.todo and self.todo[0][0] < self.pos + 1:
            when, (fence, work) = self.todo.pop(0)
            i = int(max(when - self.pos, 0) * nr * nc)
            r, c = divmod(i, nc) if a.shape[1] == 256 else divmod(i, nr)[::-1]
            if fence is not None:
                fence(_lanes(m, c)[8 * r:8 * r + 8])
            mark = work()
            if self.lag and mark is not None:
                self.marks.append((when + self.lag, mark()))
        self.pos += 1
        return m


def _kernel(x_hbm, wqkv_hbm, wo_hbm, wg_hbm, wu_hbm, wd_hbm, out_hbm,
            xbuf, ybuf, aop, wqk_op, wv_op, wo_op, sem_x, sem_e, sem_l, sem_w, sem_o, *, cfg):
    orders = {k: [int(c) for c in v] for k, v in cfg.items() if k.startswith("o_")}

    def chunk_cols(c):
        return _rows(c * 128, 128)

    def x_copies(t):
        rows = _rows(t * 4 * Q, 4 * Q)
        return [pltpu.make_async_copy(x_hbm.at[rows], xbuf.at[rows], sem_x.at[t])]

    def half_index(a, b):
        return {(0, 0): 2, (1, 1): 3, (0, 1): 7, (1, 0): 8}[a, b] * NP

    def ffn(hop, wd_op, wo_buf):

        def qkv_row(u, m):
            return 512 + ((u & 1) * 3 + m) * 256

        def qkv_copies(u):
            return [pltpu.make_async_copy(wqkv_hbm.at[_rows(kq * 256 + u * 64, 64), pl.ds(m * D, D)],
                                          xbuf.at[_rows(qkv_row(u, m) + kq * 64, 64)], sem_w.at[u & 1])
                    for m in range(3) for kq in range(4)]

        def wo_copies():
            return [pltpu.make_async_copy(wo_hbm.at[:, chunk_cols(c)], wo_buf.at[c, pl.ds(0, D)], sem_w.at[2])
                    for c in range(8)]

        def expand(wd_buf, *h_s):

            def up_copies(j, c, sem):
                return [pltpu.make_async_copy(src.at[:, chunk_cols(4 * j + cq)],
                                              ybuf.at[(j & 1) * 4 + cq, pl.ds(r, D)], sem.at[j & 1])
                        for cq in (2 * c, 2 * c + 1) for src, r in ((wg_hbm, 0), (wu_hbm, D))]

            def early_copies(j):
                return up_copies(j, 0, sem_e)

            def late_copies(j):
                return up_copies(j, 1, sem_l) + [pltpu.make_async_copy(
                    wd_hbm.at[_rows(j * 512, 512)], wd_buf.at[j & 1, pl.ds(0, 512)], sem_l.at[j & 1])]

            for cp in sum((x_copies(t) for t in range(cfg["ahead"])), []):
                cp.start()

            LB = 16
            NL = S // (4 * LB)
            sum_s, mean_s, sq_s, rstd_s = h_s

            def x_rows(i, a, c):
                return xbuf[_rows((i >> 2) * 4 * Q + a * Q + (i & 3) * LB, LB), chunk_cols(c)].astype(F32)

            def lane_mean(v):
                return jnp.broadcast_to(jnp.sum(v, axis=-1, keepdims=True) * (1.0 / D), v.shape)

            def ln_sum(i, a, rows):
                sum_s[a, rows, :] = functools.reduce(jnp.add, [x_rows(i, a, c) for c in range(8)])

            def ln_mean(i, a, rows):
                mean_s[a, rows, :] = lane_mean(sum_s[a, rows, :])

            def ln_squares(i, a, rows):
                xc = [x_rows(i, a, c) - mean_s[a, rows, :] for c in range(8)]
                sq_s[a, rows, :] = functools.reduce(jnp.add, [v * v for v in xc])

            def ln_rstd(i, a, rows):
                rstd_s[a, rows, :] = lax.rsqrt(lane_mean(sq_s[a, rows, :]) + 1e-5)

            def ln_operands(i):
                rows = _rows(i * LB, LB)
                for c in range(2):
                    xn = {(a, k): (x_rows(i, a, 2 * k + c) - mean_s[a, rows, :]) * rstd_s[a, rows, :]
                          for a in range(4) for k in range(4)}
                    for p2 in range(NP):
                        inner = [_lin(LHS[p2], lambda q2: xn[_quarter(q, q2)]) for q in range(4)]
                        for q in (1, 2):
                            aop[half_index(*QUADS[q]) + p2, c, rows, :] = inner[q].astype(BF16)
                        for p in range(NP):
                            aop[p * NP + p2, c, rows, :] = _lin(LHS[p], inner.__getitem__).astype(BF16)

            def ln_step(i, lo=0, hi=5):
                if lo <= 4 < hi:
                    ln_operands(i - 4)
                for s, stage in ((3, ln_rstd), (2, ln_squares), (1, ln_mean), (0, ln_sum)):
                    if lo <= s < hi:
                        for a in range(4):
                            stage(i - s, a, _rows((i - s) * LB, LB))

            def ln_tile(t, carry):
                for cp in x_copies(t):
                    cp.wait()
                nxt = t + cfg["ahead"]

                @pl.when(nxt < NT)
                def _():
                    for cp in x_copies(nxt):
                        cp.start()

                @pl.when(nxt == NT)
                def _():
                    for cp in early_copies(0):
                        cp.start()

                lax.fori_loop(4 * t, 4 * t + 4, lambda i, c: ln_step(i) or c, 0)
                return carry

            if "0" in cfg["only"]:
              with jax.named_scope("ph0"):
                for cp in x_copies(0):
                    cp.wait()
                for cp in x_copies(cfg["ahead"]):
                    cp.start()
                for i in range(4):
                    ln_step(i, hi=i + 1)
                lax.fori_loop(1, NT, ln_tile, 0)
                for cp in late_copies(0):
                    cp.start()
                for i in range(4):
                    ln_step(NL + i, lo=i + 1)

            def prep_wd(j):
                def fence(v):
                    wd_buf[j >> 3, pl.ds(512, 16), pl.ds(0, 128)] = pltpu.bitcast(v, BF16)

                def work(i, c, ps):
                    def block(q, q2):
                        kq, nq = _quarter(q, q2)
                        return wd_buf[j & 1, pl.ds((kq ^ 2) * 128 + i, 16), chunk_cols(2 * nq + c)]

                    for p in ps:
                        op = _operands(RHS, p, block)
                        for p2 in range(NP):
                            wd_op[p * NP + p2, c, _rows(j * 128 + i, 16), :] = op(p2)
                    return lambda: _words(wd_op, (j >> 3, 0), 0, 16)

                return [(fence, functools.partial(work, i, c, ps))
                        for i in range(0, 128, 16) for c in range(2) for ps in cfg["wdp"]]

            def prep_h(j, ps):
                def fence(p, v):
                    h_s[max(q for q in range(4) if LHS[p][q])][j >> 3, pl.ds(512, 8), :] = v

                def work(i, p):
                    op = _operands(LHS, p, lambda q, q2: h_s[q][q2, pl.ds(i, 16), :])
                    for p2 in range(NP):
                        hop[p * NP + p2, j, pl.ds(i, 16), :] = op(p2)
                    return lambda: _words(hop, (j >> 3, 0), 0, 16)

                return [(functools.partial(fence, p), functools.partial(work, i, p))
                        for i in range(0, 512, 16) for p in ps]

            def up_step(j, carry):
                for cp in early_copies(j):
                    cp.wait()

                @pl.when(j + 1 < NJ)
                def _():
                    for cp in early_copies(j + 1) + late_copies(j + 1):
                        cp.start()

                @pl.when(j + 1 == NJ)
                def _():
                    for cp in qkv_copies(0) + wo_copies():
                        cp.start()

                fill = _Filler(j < 0, cfg["lag"])
                fill.plan(cfg["wd0"], cfg["wd1"], prep_wd(j))
                fill.plan(cfg["hp"][0][1], cfg["hp"][0][2], prep_h(jnp.maximum(j - 1, 0), cfg["hp"][0][0]))
                for ps, first, last in cfg["hp"][1:]:
                    fill.plan(first, last, prep_h(j, ps))

                def block(q, q2):
                    kq, cq = _quarter(q, q2)
                    return _cat(_load(ybuf, ((j & 1) * 4 + cq,), r + kq * 256, 256) for r in (0, D))

                def outer(p):
                    if fill.pos == cfg["mid"]:
                        for cp in late_copies(j):
                            cp.wait()
                    rhs = _operands(RHS, p, block)

                    def inner(p2):
                        lhs = [_words(aop, (p * NP + p2, c), 0, 512) for c in range(2)]
                        lhs[0] = fill.hold(lhs[0])
                        return fill.dot(_cat(pltpu.bitcast(x, BF16) for x in lhs), rhs(p2))

                    return _quadrants(inner, orders["o_up2"])

                def done(q, vals):
                    for q2, v in enumerate(vals):
                        h_s[q ^ 1][q2, pl.ds(0, 512), :] = _gelu(_lanes(v, 0)) * _lanes(v, 1)

                _strassen(outer, done, orders["o_up"])
                assert not fill.todo
                return carry

            if "1" in cfg["only"]:
              with jax.named_scope("ph1"):
                lax.fori_loop(0, NJ, up_step, 0)
                for _, work in prep_h(NJ - 1, cfg["hp"][0][0]):
                    work()

        pl.run_scoped(expand, pltpu.VMEM((2, 512 + 16, D), BF16),
                      *[pltpu.VMEM((4, 512 + 8, 128), F32)] * 4)

        def contract(tmp_u, tmp_v, tmp_f):

            def prep_qkv(u):
                def fence_in(v):
                    xbuf[_rows(496 - 16 * (u >> 3), 16), pl.ds(0, 128)] = pltpu.bitcast(v, BF16)

                def fence_u(v):
                    tmp_u[u >> 3, pl.ds(H * PITCH, 8), :] = pltpu.bitcast(v, U32)

                def fence_v(v):
                    tmp_v[u >> 3, pl.ds(128, 8), :] = pltpu.bitcast(v, U32)

                def scatter(m, c):
                    w = pltpu.bitcast(xbuf[_rows(qkv_row(u, m), 256), chunk_cols(c)], U32).T
                    for h in range(4):
                        tmp_u[m, pl.ds((4 * c + h) * PITCH, DH), :] = w[h * DH:(h + 1) * DH]

                def gather(m, c):
                    w = [tmp_u[m, pl.ds(4 * c + d, H, stride=PITCH), :] for d in range(4)]
                    tmp_v[8 * m + c, pl.ds(0, 128), :] = jnp.concatenate(w, axis=0).T

                def rows(m, c, kq, i):
                    return pltpu.bitcast(tmp_v[8 * m + c, pl.ds((kq * 64 + i) // 2, 8), :], BF16)

                def one_level(m, c, b):
                    for i in range(0, 64, 16):
                        for p in range(NP):
                            op = _lin(RHS[p], lambda q: rows(m, c + 4 * (q % 2), 2 * b + q // 2, i))
                            wqk_op[m, p, c, _rows(b * 256 + u * 64 + i, 16), :] = op.astype(BF16)

                def two_level(c, i, ps):
                    def block(q, q2):
                        kq, nq = _quarter(q, q2)
                        return rows(2, 2 * nq + c, kq, i)

                    for p in ps:
                        op = _operands(RHS, p, block)
                        for p2 in range(NP):
                            wv_op[p * NP + p2, c, _rows(u * 64 + i, 16), :] = op(p2)

                return ([(fence_in, functools.partial(scatter, m, c)) for m in range(3) for c in range(8)],
                        [(fence_u, functools.partial(gather, m, c)) for m in range(3) for c in range(8)],
                        [(fence_v, functools.partial(one_level, m, c, b))
                         for m in range(2) for c in range(4) for b in range(2)]
                        + [(fence_v, functools.partial(two_level, c, i, ps))
                           for c in range(2) for i in range(0, 64, 16) for ps in cfg["wdp"]])

            def prep_wo(u):
                def fence_in(v):
                    wo_buf[u >> 3, pl.ds(D, 16), :] = pltpu.bitcast(v, BF16)

                def fence_f(v):
                    tmp_f[u >> 3, pl.ds(H * PITCH, 8), :] = v

                def scatter(h):
                    for nq in range(4):
                        w = _load(wo_buf, (2 * nq + (u & 1),), h * DH, DH)
                        tmp_f[nq, pl.ds(h * PITCH, DH), :] = w.astype(F32)

                def gather(d, h, ps):
                    d = (u >> 1) * 4 + d

                    def block(q, q2):
                        kq, nq = _quarter(q, q2)
                        return tmp_f[nq ^ 3, pl.ds(h * PITCH + (kq ^ 2) * 8 + d, 16, stride=PITCH), :]

                    for p in ps:
                        op = _operands(RHS, p, block)
                        for p2 in range(NP):
                            wo_op[p * NP + p2, u & 1, _rows(d * H + h, 16), :] = op(p2)

                return ([(fence_in, functools.partial(scatter, h)) for h in range(H)]
                        + [(fence_f, functools.partial(gather, d, h, ps))
                           for d in range(4) for h in (0, 16) for ps in cfg["wdp"]])

            def down_step(u, carry):
                for cp in qkv_copies(u):
                    cp.wait()

                @pl.when(u + 1 < NU)
                def _():
                    for cp in qkv_copies(u + 1):
                        cp.start()

                fill = _Filler()
                scatter, gather, combine = prep_qkv(u)
                t0, t1, t2, t3 = cfg["dn"]
                fill.plan(0, t0, scatter)
                fill.plan(t0, t1, gather)
                fill.plan(t1, t2, prep_wo(u))
                fill.plan(t2, t3, combine)

                def outer(p):
                    def inner(p2):
                        lhs = _cat(_load(hop, (p * NP + p2, j), u * 128, 128) for j in range(NJ))
                        return fill.dot(lhs, _cat(_load(wd_op, (p * NP + p2, c), 0, F // 4) for c in range(2)))

                    return _quadrants(inner, orders["o_dn2"])

                def done(q, vals):
                    for q2, d in enumerate(vals):
                        a, nq = _quarter(q, q2)
                        g = _silu(d).astype(BF16)
                        for s in range(2):
                            for c in range(2):
                                rows = _rows(((2 * u + s) * 4 + a) * Q, Q)
                                ybuf[2 * nq + c, rows, :] = _lanes(g, c)[s * Q:(s + 1) * Q]

                _strassen(outer, done, orders["o_dn"])
                assert not fill.todo
                return carry

            if "2" in cfg["only"]:
              with jax.named_scope("ph2"):
                for cp in wo_copies():
                    cp.wait()
                lax.fori_loop(0, NU, down_step, 0)

        pl.run_scoped(contract, pltpu.VMEM((3, H * PITCH + 8, 128), U32),
                      pltpu.VMEM((24, 128 + 8, 128), U32), pltpu.VMEM((4, H * PITCH + 8, 128), F32))

    pl.run_scoped(
        ffn,
        pltpu.VMEM((NP * NP, NJ, S // 4, 128), BF16),
        pltpu.VMEM((NP * NP, 2, F // 4, 128), BF16),
        pltpu.VMEM((8, D + 16, 128), BF16),
    )

    def attention(q_s, p_s, oop, obuf, k0, k1, *bufs):
        k_s, v_s, o_s = (k0, k1), bufs[:4], bufs[4:]

        def out_copies(t):
            rows = _rows(t * 2 * Q, 2 * Q)
            return [pltpu.make_async_copy(obuf.at[c, rows], out_hbm.at[rows, chunk_cols(c)], sem_o.at[t])
                    for c in range(8)]

        refetch = 1

        def tile(t, carry):
            @pl.when(t >= refetch)
            def _():
                for cp in x_copies(t):
                    cp.wait()

            fill = _Filler()
            tail, head = pl.ds(2 * Q, HALO), pl.ds(0, HALO)

            def fence(ref):
                def park(v):
                    ref[t >> 3, pl.ds(ref.shape[1] - 8, 8), :] = v
                return park

            def probs(a):
                pieces = []
                for r in range(0, 2 * Q, 8):
                    lg = [None] * WIN

                    def logits(c, r=r, lg=lg):
                        qv = q_s[c, pl.ds(a * 2 * Q + r, 8), :]
                        for w in range(WIN):
                            pr = qv * k_s[a][c, pl.ds(HALO + r - DIL * w, 8), :]
                            lg[w] = pr if c == 0 else lg[w] + pr

                    def softmax(r=r, lg=lg):
                        lg = [l + pltpu.roll(l, 64, 1) for l in lg]
                        lg = [(l + pltpu.roll(l, 32, 1)) * DH ** -0.5 for l in lg]
                        for w in range(WIN):
                            if a == 0 and r < DIL * w:
                                pos = t * 4 * Q + r + lax.broadcasted_iota(jnp.int32, (8, 128), 0)
                                lg[w] = jnp.where(pos >= DIL * w, lg[w], -1e9)
                        mx = functools.reduce(jnp.maximum, lg)
                        e = [jnp.exp(l - mx) for l in lg]
                        inv = 1.0 / functools.reduce(jnp.add, e)
                        for w in range(WIN):
                            p_s[w, pl.ds(a * 2 * Q + r, 8), :] = e[w] * inv

                    pieces += [(fence(k_s[a]) if c % cfg["cq"] == 0 else None, functools.partial(logits, c))
                               for c in range(8)]
                    pieces.append((None, softmax))
                return pieces

            def mix(q, first=0, last=2 * Q):
                def work(r, c):
                    terms = [p_s[w, pl.ds((q // 2) * 2 * Q + r, 8), :]
                             * v_s[q][c, pl.ds(HALO + r - DIL * w, 8), :] for w in range(WIN)]
                    o_s[q ^ 1][c, pl.ds(r, 8), :] = functools.reduce(jnp.add, terms)

                return [(fence(v_s[q]) if c % cfg["cv"] == 0 else None, functools.partial(work, r, c))
                        for r in range(first, last, 8) for c in range(4)]

            def prep_o(ps):
                def work(i, c, p):
                    op = _operands(LHS, p, lambda q, q2: o_s[q][2 * (q2 % 2) + c, pl.ds((q2 // 2) * Q + i, 16), :])
                    for p2 in range(NP):
                        oop[p * NP + p2, c, pl.ds(i, 16), :] = op(p2)

                return [(fence(o_s[max(q for q in range(4) if LHS[p][q])]), functools.partial(work, i, c, p))
                        for p in ps for i in range(0, Q, 16) for c in range(2)]

            def project(m, a, dst, off):
                def product(p):
                    lhs = _cat(_load(aop, (half_index(a, b) + p, c), t * Q, Q) for b, c in QUADS)
                    return [fill.dot(lhs, _cat(_load(wqk_op, (m, p, c), 0, 512) for c in range(4)))]

                def done(q, val):
                    for c in range(4):
                        dst[4 * (q % 2) + c, pl.ds(off + (q // 2) * Q, Q), :] = _lanes(val[0], c)

                _strassen(product, done, orders["o_qk"])

            def two_level(lhs, start, rhs, done, order):
                def outer(p):
                    return _quadrants(
                        lambda p2: fill.dot(_cat(_load(lhs, (p * NP + p2, c), start, Q) for c in range(2)),
                                            _cat(_load(rhs, (p * NP + p2, c), 0, 256) for c in range(2))),
                        orders["o_at2"])

                _strassen(outer, done, order)

            def values(q, vals):
                for q2, v in enumerate(vals):
                    for c in range(2):
                        v_s[q][2 * (q2 % 2) + c, pl.ds(HALO + (q2 // 2) * Q, Q), :] = _lanes(v, c)
                if q < 2:
                    for c in range(4):
                        first = jnp.broadcast_to(v_s[q][c, pl.ds(HALO, 1), :], (HALO, 128))
                        v_s[q][c, head, :] = jnp.where(t > 0, v_s[q][c, head, :], first)
                    v_s[q + 2][:, head, :] = v_s[q][:, tail, :]

            finished = []

            def output(q, vals):
                for q2, v in enumerate(vals):
                    a, nq = _quarter(q, q2)
                    for c in range(2):
                        lead, start = (2 * (nq ^ 3) + c,), (4 * t + a) * Q
                        g = _load(ybuf, lead, start, Q).astype(F32)
                        xv = xbuf[_rows(start, Q), chunk_cols(lead[0])].astype(F32)
                        obuf[(*lead, _rows(start, Q))] = (xv + _lanes(v, c) * g).astype(BF16)
                finished.append(q)
                if q ^ 1 in finished:
                    for cp in out_copies(2 * t + q // 2):
                        cp.start()

            k0[:, head, :] = jnp.where(t > 0, k1[:, tail, :], 0.0)
            for q in range(2):
                v_s[q][:, head, :] = v_s[q + 2][:, tail, :]
            project(1, 0, k0, HALO)
            k1[:, head, :] = k0[:, tail, :]
            project(0, 0, q_s, 0)
            fill.plan(0, cfg["e1"], probs(0))
            project(1, 1, k1, HALO)
            project(0, 1, q_s, 2 * Q)
            w = cfg["w"]
            fill.plan(0, w[0], probs(1))
            fill.plan(w[0], w[1], mix(1) + prep_o((2,)))
            fill.plan(w[1], w[2], mix(2, HALO) + mix(2, 0, HALO) + prep_o((3, 0)))
            fill.plan(w[2], w[3], mix(0) + prep_o((4, 6)))
            fill.plan(w[3], w[4], mix(3) + prep_o((1, 5)))
            two_level(aop, t * Q, wv_op, values, (2, 4, 3, 1, 0, 6, 5))
            two_level(oop, 0, wo_op, output, (2, 3, 0, 4, 6, 1, 5))
            assert not fill.todo
            return carry

        if "3" in cfg["only"]:
          with jax.named_scope("ph3"):
            for t in range(refetch, NT):
                for cp in x_copies(t):
                    cp.start()
            lax.fori_loop(0, NT, tile, 0)
        for t in range(2 * NT):
            for cp in out_copies(t):
                cp.wait()

    pl.run_scoped(
        attention,
        pltpu.VMEM((8, 4 * Q, 128), F32),
        pltpu.VMEM((WIN, 4 * Q, 128), F32),
        pltpu.VMEM((NP * NP, 2, Q, 128), BF16),
        pltpu.VMEM((8, S, 128), BF16),
        *[pltpu.VMEM((8, HALO + 2 * Q + 8, 128), F32)] * 2,
        *[pltpu.VMEM((4, HALO + 2 * Q + 8, 128), F32)] * 4,
        *[pltpu.VMEM((4, 2 * Q + 8, 128), F32)] * 4,
    )


DEFAULT = dict(only="0123", ahead=3, mid=14, lag=1, wd0=14, wd1=36,
               hp=(((1, 5, 4, 6), 0.5, 8), ((3,), 14, 18), ((0, 2), 28, 36)),
               wdp=((0, 1), (2, 4), (3,), (5,), (6,)), dn=(10, 20, 32, 46),
               cq=4, cv=2, e1=13.5, w=(24, 36, 52, 66, 80),
               o_up="1342056", o_up2="1324056", o_dn="0123456", o_dn2="0123456",
               o_qk="1324056", o_at2="1324056")


def make(flags=None, interpret=False, **kw):
    cfg = dict(DEFAULT, **kw)

    def f(A_x, A_wqkv, A_wo, B_x, B_w_gate, B_w_up, B_w_down):
        del B_x
        any_spec = pl.BlockSpec(memory_space=pl.ANY)
        out = pl.pallas_call(
            functools.partial(_kernel, cfg=cfg),
            out_shape=jax.ShapeDtypeStruct((S, D), BF16),
            in_specs=[any_spec] * 6,
            out_specs=any_spec,
            scratch_shapes=[
                pltpu.VMEM((S, D), BF16),
                pltpu.VMEM((8, S, 128), BF16),
                pltpu.VMEM((NP * (NP + 2), 2, S // 4, 128), BF16),
                pltpu.VMEM((2, NP, 4, D // 2, 128), BF16),
                pltpu.VMEM((NP * NP, 2, D // 4, 128), BF16),
                pltpu.VMEM((NP * NP, 2, D // 4, 128), BF16),
                pltpu.SemaphoreType.DMA((NT,)),
                pltpu.SemaphoreType.DMA((2,)),
                pltpu.SemaphoreType.DMA((2,)),
                pltpu.SemaphoreType.DMA((3,)),
                pltpu.SemaphoreType.DMA((2 * NT,)),
            ],
            compiler_params=pltpu.CompilerParams(
                vmem_limit_bytes=127 * 2**20, **({"flags": flags} if flags else {})),
            name="fused_block",
            interpret=interpret,
        )(A_x.reshape(S, D), A_wqkv, A_wo, B_w_gate, B_w_up, B_w_down)
        return out.reshape(1, S, D)

    return f


@jax.jit
def pallas_recurrent_scan__sliding_local_dilated__geglu_ffn__prompt_kernel(
    A_x: jax.Array,
    A_wqkv: jax.Array,
    A_wo: jax.Array,
    B_x: jax.Array,
    B_w_gate: jax.Array,
    B_w_up: jax.Array,
    B_w_down: jax.Array,
):
    return make()(A_x, A_wqkv, A_wo, B_x, B_w_gate, B_w_up, B_w_down)
```

```python
import functools

import jax
import jax.numpy as jnp
from jax import lax
import jax.experimental.pallas as pl
import jax.experimental.pallas.tpu as pltpu

F32 = jnp.float32
BF16 = jnp.bfloat16
U32 = jnp.uint32

S, D, F = 2048, 1024, 3584
H, DH, WIN, DIL = 32, 32, 8, 2
HALO = 16
PITCH = DH + 1
Q = 64
NT = S // (4 * Q)
NJ = F // 512
NU = S // 512

LHS = ((1, 0, 0, 1), (0, 0, 1, 1), (1, 0, 0, 0), (0, 0, 0, 1),
       (1, 1, 0, 0), (-1, 0, 1, 0), (0, 1, 0, -1))
RHS = ((1, 0, 0, 1), (1, 0, 0, 0), (0, 1, 0, -1), (-1, 0, 1, 0),
       (0, 0, 0, 1), (1, 1, 0, 0), (0, 0, 1, 1))
OUT = ((1, 0, 0, 1), (0, 0, 1, -1), (0, 1, 0, 1), (1, 0, 1, 0),
       (-1, 1, 0, 0), (0, 0, 0, 1), (1, 0, 0, 0))
NP = 7
QUADS = ((0, 0), (0, 1), (1, 0), (1, 1))


def _lin(coef, quad):
    idx = sorted((q for q, c in enumerate(coef) if c), key=lambda q: -coef[q])
    if len(idx) == 1:
        return quad(idx[0])
    a, b = quad(idx[0]).astype(F32), quad(idx[1]).astype(F32)
    return a + b if coef[idx[1]] > 0 else a - b


def _operands(coefs, p, block):
    w = [_lin(coefs[p], lambda q: block(q, q2)) for q2 in range(4)]
    return lambda p2: _lin(coefs[p2], w.__getitem__).astype(BF16)


def _quarter(q, q2):
    return 2 * (q // 2) + q2 // 2, 2 * (q % 2) + q2 % 2


def _strassen(product, done, order):
    acc = [None] * 4
    left = [sum(1 for p in range(NP) if OUT[p][q]) for q in range(4)]
    for p in order:
        m = product(p)
        for q in range(4):
            s = OUT[p][q]
            if s == 0:
                continue
            if acc[q] is None:
                acc[q] = (s, m)
            else:
                s0, c = acc[q]
                assert s > 0 or s0 > 0
                acc[q] = (1, [x + y if s == s0 else (x - y if s > 0 else y - x)
                              for x, y in zip(m, c)])
            left[q] -= 1
            if left[q] == 0:
                done(q, acc[q][1])


def _quadrants(product, order):
    out = [None] * 4

    def done(q, val):
        out[q] = val[0]

    _strassen(lambda p: [product(p)], done, order)
    return out


def _cat(xs):
    return jnp.concatenate(list(xs), axis=1)


def _lanes(v, c):
    return v[:, c * 128:(c + 1) * 128]


def _gelu(g):
    hg = 0.5 * g
    t = jnp.tanh(g * (0.7978845608028654 + 0.035677408136300125 * (g * g)))
    return hg * t + hg


def _silu(d):
    hd = 0.5 * d
    return hd * jnp.tanh(hd) + hd


def _rows(start, size):
    return pl.ds(start if isinstance(start, int) else pl.multiple_of(start, size), size)


def _words(ref, lead, start, size):
    return ref.bitcast(U32)[(*lead, _rows(start >> 1, size // 2))]


def _load(ref, lead, start, size):
    return pltpu.bitcast(_words(ref, lead, start, size), BF16)


class _Filler:
    def __init__(self, never=None, lag=0):
        self.todo, self.pos = [], 0
        self.never, self.lag, self.marks = never, lag, []

    def plan(self, first, last, pieces):
        self.todo += [(self.pos + first + i * (last - first) / len(pieces), piece)
                      for i, piece in enumerate(pieces)]
        self.todo.sort(key=lambda t: t[0])

    def hold(self, a, span):
        rows = [a[r:r + 8] for r in range(0, a.shape[0], 8)]
        while self.marks and self.marks[0][0] < self.pos + span:
            when, mark = self.marks.pop(0)
            r = int(max(when - self.pos, 0) / span * len(rows))
            rows[r] = jnp.where(self.never, mark, rows[r])
        return jnp.concatenate(rows, axis=0)

    def dot(self, words, b, span=1):
        words = list(words)
        a = _cat(pltpu.bitcast(x, BF16) for x in [self.hold(words[0], span)] + words[1:])
        m = jnp.dot(a, b, preferred_element_type=F32)
        nr, nc = m.shape[0] // 8, m.shape[1] // 128
        while self.todo and self.todo[0][0] < self.pos + span:
            when, (fence, work) = self.todo.pop(0)
            i = int(max(when - self.pos, 0) / span * nr * nc)
            r, c = divmod(i, nc) if a.shape[1] == 256 else divmod(i, nr)[::-1]
            if fence is not None:
                fence(_lanes(m, c)[8 * r:8 * r + 8])
            mark = work()
            if self.lag and mark is not None:
                self.marks.append((when + self.lag, mark()))
        self.pos += span
        return m


def _kernel(x_hbm, wqkv_hbm, wo_hbm, wg_hbm, wu_hbm, wd_hbm, out_hbm,
            xbuf, ybuf, aop, wqk_op, wv_op, wo_op, sem_x, sem_e, sem_l, sem_w, sem_o, *, cfg):
    orders = {k: [int(c) for c in v] for k, v in cfg.items() if k.startswith("o_")}

    def chunk_cols(c):
        return _rows(c * 128, 128)

    def x_copies(t):
        rows = pl.ds(4 * t, 4)
        return [pltpu.make_async_copy(x_hbm.at[rows], xbuf.at[rows], sem_x.at[t])]

    def half_index(a, b):
        return {(0, 0): 2, (1, 1): 3, (0, 1): 7, (1, 0): 8}[a, b] * NP

    def ffn(hop, wd_op, wo_buf):

        def qkv_row(u, m):
            return 8 + ((u & 1) * 3 + m) * 4

        def qkv_copies(u):
            return [pltpu.make_async_copy(wqkv_hbm.at[:, _rows(u * Q, Q), pl.ds(m * D, D)],
                                          xbuf.at[pl.ds(qkv_row(u, m), 4)], sem_w.at[u & 1])
                    for m in range(3)]

        def wo_copies():
            return [pltpu.make_async_copy(wo_hbm.at[:, chunk_cols(c)], wo_buf.at[c, pl.ds(0, D)], sem_w.at[2])
                    for c in range(8)]

        def expand(wd_buf, *h_s):

            def block(j):
                return min(j, NJ - 1) if isinstance(j, int) else jnp.minimum(j, NJ - 1)

            def up_copies(j, c, sem):
                return [pltpu.make_async_copy(src.at[:, chunk_cols(4 * block(j) + cq)],
                                              ybuf.at[(j & 1) * 4 + cq, pl.ds(r, D)], sem.at[j & 1])
                        for cq in (2 * c, 2 * c + 1) for src, r in ((wg_hbm, 0), (wu_hbm, D))]

            def early_copies(j):
                return up_copies(j, 0, sem_e)

            def late_copies(j):
                return up_copies(j, 1, sem_l) + [pltpu.make_async_copy(
                    wd_hbm.at[_rows(block(j) * 512, 512)], wd_buf.at[j & 1, pl.ds(0, 512)], sem_l.at[j & 1])]

            for cp in sum((x_copies(t) for t in range(cfg["ahead"])), []):
                cp.start()

            LB = 16
            NL = S // (4 * LB)
            sum_s, mean_s, sq_s, rstd_s = h_s

            def x_rows(i, a, c):
                return xbuf[(i >> 2) * 4 + a, _rows((i & 3) * LB, LB), chunk_cols(c)].astype(F32)

            def lane_mean(v):
                return jnp.broadcast_to(jnp.sum(v, axis=-1, keepdims=True) * (1.0 / D), v.shape)

            def ln_sum(i, a, rows):
                sum_s[a, rows, :] = functools.reduce(jnp.add, [x_rows(i, a, c) for c in range(8)])

            def ln_mean(i, a, rows):
                mean_s[a, rows, :] = lane_mean(sum_s[a, rows, :])

            def ln_squares(i, a, rows):
                xc = [x_rows(i, a, c) - mean_s[a, rows, :] for c in range(8)]
                sq_s[a, rows, :] = functools.reduce(jnp.add, [v * v for v in xc])

            def ln_rstd(i, a, rows):
                rstd_s[a, rows, :] = lax.rsqrt(lane_mean(sq_s[a, rows, :]) + 1e-5)

            def ln_operands(i):
                rows = _rows(i * LB, LB)
                for c in range(2):
                    xn = {(a, k): (x_rows(i, a, 2 * k + c) - mean_s[a, rows, :]) * rstd_s[a, rows, :]
                          for a in range(4) for k in range(4)}
                    for p2 in range(NP):
                        inner = [_lin(LHS[p2], lambda q2: xn[_quarter(q, q2)]) for q in range(4)]
                        for q in (1, 2):
                            aop[half_index(*QUADS[q]) + p2, c, rows, :] = inner[q].astype(BF16)
                        for p in range(NP):
                            aop[p * NP + p2, c, rows, :] = _lin(LHS[p], inner.__getitem__).astype(BF16)

            def ln_step(i, lo=0, hi=5):
                if lo <= 4 < hi:
                    ln_operands(i - 4)
                for s, stage in ((3, ln_rstd), (2, ln_squares), (1, ln_mean), (0, ln_sum)):
                    if lo <= s < hi:
                        for a in range(4):
                            stage(i - s, a, _rows((i - s) * LB, LB))

            def ln_tile(t, carry):
                for cp in x_copies(t):
                    cp.wait()
                nxt = t + cfg["ahead"]

                @pl.when(nxt < NT)
                def _():
                    for cp in x_copies(nxt):
                        cp.start()

                @pl.when(nxt == NT)
                def _():
                    for cp in early_copies(0):
                        cp.start()

                lax.fori_loop(4 * t, 4 * t + 4, lambda i, c: ln_step(i) or c, 0)
                return carry

            if "0" in cfg["only"]:
              with jax.named_scope("ph0"):
                for cp in x_copies(0):
                    cp.wait()
                for cp in x_copies(cfg["ahead"]):
                    cp.start()
                for i in range(4):
                    ln_step(i, hi=i + 1)
                lax.fori_loop(1, NT, ln_tile, 0)
                for cp in late_copies(0):
                    cp.start()
                for i in range(4):
                    ln_step(NL + i, lo=i + 1)
                for cp in qkv_copies(0) + qkv_copies(1) + wo_copies():
                    cp.start()

            def prep_wd(j):
                def fence(v):
                    wd_buf[j >> 3, pl.ds(512, 16), pl.ds(0, 128)] = pltpu.bitcast(v, BF16)

                def work(i, c, ps):
                    def block(q, q2):
                        kq, nq = _quarter(q, q2)
                        return wd_buf[j & 1, pl.ds((kq ^ 2) * 128 + i, 16), chunk_cols(2 * nq + c)]

                    for p in ps:
                        op = _operands(RHS, p, block)
                        for p2 in range(NP):
                            wd_op[p * NP + p2, c, _rows(j * 128 + i, 16), :] = op(p2)
                    return lambda: _words(wd_op, (j >> 3, 0), 0, 16)

                return [(fence, functools.partial(work, i, c, ps))
                        for i in range(0, 128, 16) for c in range(2) for ps in cfg["wdp"]]

            def prep_h(j, ps):
                def fence(p, v):
                    h_s[max(q for q in range(4) if LHS[p][q])][j >> 3, pl.ds(512, 8), :] = v

                def work(i, p):
                    op = _operands(LHS, p, lambda q, q2: h_s[q][q2, pl.ds(i, 16), :])
                    for p2 in range(NP):
                        hop[p * NP + p2, j, pl.ds(i, 16), :] = op(p2)
                    return lambda: _words(hop, (j >> 3, 0), 0, 16)

                return [(functools.partial(fence, p), functools.partial(work, i, p))
                        for i in range(0, 512, 16) for p in ps]

            def up_step(j, carry):
                for cp in early_copies(j):
                    cp.wait()

                fill = _Filler(j < 0, cfg["lag"])
                pieces = prep_wd(j)
                fill.plan(*cfg["wd0"], pieces[:cfg["wds"]])
                fill.plan(*cfg["wd1"], pieces[cfg["wds"]:])
                fill.plan(cfg["hp"][0][1], cfg["hp"][0][2], prep_h(jnp.maximum(j - 1, 0), cfg["hp"][0][0]))
                for ps, first, last in cfg["hp"][1:]:
                    fill.plan(first, last, prep_h(j, ps))

                def block(q, q2):
                    kq, cq = _quarter(q, q2)
                    return _cat(_load(ybuf, ((j & 1) * 4 + cq,), r + kq * 256, 256) for r in (0, D))

                def outer(p):
                    if fill.pos == cfg["mid"]:
                        for cp in early_copies(j + 1) + late_copies(j + 1):
                            cp.start()
                        for cp in late_copies(j):
                            cp.wait()
                    rhs = _operands(RHS, p, block)

                    def inner(p2):
                        return fill.dot([_words(aop, (p * NP + p2, c), 0, 512) for c in range(2)], rhs(p2))

                    return _quadrants(inner, orders["o_up2"])

                def done(q, vals):
                    for q2, v in enumerate(vals):
                        h_s[q ^ 1][q2, pl.ds(0, 512), :] = _gelu(_lanes(v, 0)) * _lanes(v, 1)

                _strassen(outer, done, orders["o_up"])
                assert not fill.todo
                return carry

            if "1" in cfg["only"]:
              with jax.named_scope("ph1"):
                lax.fori_loop(0, NJ, up_step, 0)
                for _, work in prep_h(NJ - 1, cfg["hp"][0][0]):
                    work()
                for cp in early_copies(NJ) + late_copies(NJ):
                    cp.wait()

        pl.run_scoped(expand, pltpu.VMEM((2, 512 + 16, D), BF16),
                      *[pltpu.VMEM((4, 512 + 8, 128), F32)] * 4)

        def contract(tmp_u, tmp_v, tmp_f):

            def prep_qkv(u):
                def fence_in(v):
                    xbuf[7 - (u >> 3), pl.ds(0, 16), pl.ds(0, 128)] = pltpu.bitcast(v, BF16)

                def fence_u(v):
                    tmp_u[u >> 3, pl.ds(H * PITCH, 8), :] = pltpu.bitcast(v, U32)

                def fence_v(v):
                    tmp_v[u >> 3, pl.ds(128, 8), :] = pltpu.bitcast(v, U32)

                def scatter(m, c):
                    w = pltpu.bitcast(jnp.concatenate(
                        [xbuf[qkv_row(u, m) + kq, :, chunk_cols(c)] for kq in range(4)], axis=0), U32).T
                    for h in range(4):
                        tmp_u[m, pl.ds((4 * c + h) * PITCH, DH), :] = w[h * DH:(h + 1) * DH]

                def gather(m, c):
                    w = [tmp_u[m, pl.ds(4 * c + d, H, stride=PITCH), :] for d in range(4)]
                    tmp_v[8 * m + c, pl.ds(0, 128), :] = jnp.concatenate(w, axis=0).T

                def rows(m, c, kq, i):
                    return pltpu.bitcast(tmp_v[8 * m + c, pl.ds((kq * 64 + i) // 2, 8), :], BF16)

                def one_level(m, c, b):
                    for i in range(0, 64, 16):
                        for p in range(NP):
                            op = _lin(RHS[p], lambda q: rows(m, c + 4 * (q % 2), 2 * b + q // 2, i))
                            wqk_op[m, p, c, _rows(b * 256 + u * 64 + i, 16), :] = op.astype(BF16)
                    return lambda: _words(wqk_op, (u >> 3, 0, 0), 0, 16)

                def two_level(c, i, ps):
                    def block(q, q2):
                        kq, nq = _quarter(q, q2)
                        return rows(2, 2 * nq + c, kq, i)

                    for p in ps:
                        op = _operands(RHS, p, block)
                        for p2 in range(NP):
                            wv_op[p * NP + p2, c, _rows(u * 64 + i, 16), :] = op(p2)
                    return lambda: _words(wv_op, (u >> 3, 0), 0, 16)

                return ([(fence_in, functools.partial(scatter, m, c)) for m in range(3) for c in range(8)],
                        [(fence_u, functools.partial(gather, m, c)) for m in range(3) for c in range(8)],
                        [(fence_v, functools.partial(one_level, m, c, b))
                         for m in range(2) for c in range(4) for b in range(2)]
                        + [(fence_v, functools.partial(two_level, c, i, ps))
                           for c in range(2) for i in range(0, 64, 16) for ps in cfg["wdp"]])

            def prep_wo(u):
                def fence_in(v):
                    wo_buf[u >> 3, pl.ds(D, 16), :] = pltpu.bitcast(v, BF16)

                def fence_f(v):
                    tmp_f[u >> 3, pl.ds(H * PITCH, 8), :] = v

                def scatter(h):
                    for nq in range(4):
                        w = _load(wo_buf, (2 * nq + (u & 1),), h * DH, DH)
                        tmp_f[nq, pl.ds(h * PITCH, DH), :] = w.astype(F32)
                    return lambda: pltpu.bitcast(tmp_f[u >> 3, pl.ds(0, 8), :], U32)

                def gather(d, h, ps):
                    d = (u >> 1) * 4 + d

                    def block(q, q2):
                        kq, nq = _quarter(q, q2)
                        return tmp_f[nq ^ 3, pl.ds(h * PITCH + (kq ^ 2) * 8 + d, 16, stride=PITCH), :]

                    for p in ps:
                        op = _operands(RHS, p, block)
                        for p2 in range(NP):
                            wo_op[p * NP + p2, u & 1, _rows(d * H + h, 16), :] = op(p2)
                    return lambda: _words(wo_op, (u >> 3, 0), 0, 16)

                return ([(fence_in, functools.partial(scatter, h)) for h in range(H)]
                        + [(fence_f, functools.partial(gather, d, h, ps))
                           for d in range(4) for h in (0, 16) for ps in cfg["wdp"]])

            def down_step(u, carry):
                for cp in qkv_copies(u):
                    cp.wait()

                fill = _Filler(u < 0, cfg['lag2'])
                scatter, gather, combine = prep_qkv(u)
                t0, t1, t2, t3 = cfg["dn"]
                fill.plan(0, t0, scatter)
                fill.plan(t0, t1, gather)
                fill.plan(t1, t2, prep_wo(u))
                fill.plan(t2, t3, combine)

                def outer(p):
                    def inner(p2):
                        lhs = [_words(hop, (p * NP + p2, j), u * 128, 128) for j in range(NJ)]
                        return fill.dot(lhs, _cat(_load(wd_op, (p * NP + p2, c), 0, F // 4) for c in range(2)))

                    return _quadrants(inner, orders["o_dn2"])

                def done(q, vals):
                    for q2, d in enumerate(vals):
                        a, nq = _quarter(q, q2)
                        g = _silu(d).astype(BF16)
                        for s in range(2):
                            for c in range(2):
                                rows = _rows(((2 * u + s) * 4 + a) * Q, Q)
                                ybuf[2 * nq + c, rows, :] = _lanes(g, c)[s * Q:(s + 1) * Q]

                _strassen(outer, done, orders["o_dn"])

                @pl.when(u + 2 < NU)
                def _():
                    for cp in qkv_copies(u + 2):
                        cp.start()

                assert not fill.todo
                return carry

            if "2" in cfg["only"]:
              with jax.named_scope("ph2"):
                for cp in wo_copies():
                    cp.wait()
                lax.fori_loop(0, NU, down_step, 0)

        pl.run_scoped(contract, pltpu.VMEM((3, H * PITCH + 8, 128), U32),
                      pltpu.VMEM((24, 128 + 8, 128), U32), pltpu.VMEM((4, H * PITCH + 8, 128), F32))

    pl.run_scoped(
        ffn,
        pltpu.VMEM((NP * NP, NJ, S // 4, 128), BF16),
        pltpu.VMEM((NP * NP, 2, F // 4, 128), BF16),
        pltpu.VMEM((8, D + 16, 128), BF16),
    )

    def attention(q_s, p0, p1, obuf, k0, k1, *bufs):
        p_s = (p0, p1)
        k_s, v_s, o_s, oop = (k0, k1), bufs[:4], bufs[4:8], bufs[8:]

        def out_copies(t):
            rows = _rows(t * 4 * Q, 4 * Q)
            return [pltpu.make_async_copy(obuf.at[rows], out_hbm.at[rows], sem_o.at[t])]

        refetch = 1

        def tile(t, carry):
            @pl.when(t >= refetch)
            def _():
                for cp in x_copies(t):
                    cp.wait()

            fill = _Filler(t < 0, cfg['lag3'])
            tail, head = pl.ds(2 * Q, HALO), pl.ds(0, HALO)

            def fence(ref):
                def park(v):
                    ref[t >> 3, pl.ds(ref.shape[1] - 8, 8), :] = v
                return park

            def probs(a):
                pieces = []
                for r in range(0, 2 * Q, 8):
                    lg = [None] * WIN

                    def logits(c, r=r, lg=lg):
                        qv = q_s[c, pl.ds(a * 2 * Q + r, 8), :]
                        for w in range(WIN):
                            pr = qv * k_s[a][c, pl.ds(HALO + r - DIL * w, 8), :]
                            lg[w] = pr if c == 0 else lg[w] + pr

                    def softmax(r=r, lg=lg):
                        lg = [l + pltpu.roll(l, 64, 1) for l in lg]
                        lg = [(l + pltpu.roll(l, 32, 1)) * DH ** -0.5 for l in lg]
                        for w in range(WIN):
                            if a == 0 and r < DIL * w:
                                pos = t * 4 * Q + r + lax.broadcasted_iota(jnp.int32, (8, 128), 0)
                                lg[w] = jnp.where(pos >= DIL * w, lg[w], -1e9)
                        mx = functools.reduce(jnp.maximum, lg)
                        e = [jnp.exp(l - mx) for l in lg]
                        inv = 1.0 / functools.reduce(jnp.add, e)
                        for w in range(WIN):
                            p_s[a][w, pl.ds(r, 8), :] = e[w] * inv
                        return lambda: pltpu.bitcast(p_s[a][t >> 3, pl.ds(r, 8), :], U32)

                    pieces += [(fence(k_s[a]) if c % cfg["cq"] == 0 else None, functools.partial(logits, c))
                               for c in range(8)]
                    pieces.append((None, softmax))
                return pieces

            def mix(q, first=0, last=2 * Q):
                def work(r, c):
                    terms = [p_s[q // 2][w, _rows(r + (8 * (t >> (3 + q % 2)) if cfg['dynp'] else 0), 8), :]
                             * v_s[q][c, pl.ds(HALO + r - DIL * w, 8), :] for w in range(WIN)]
                    o_s[q ^ 1][c, pl.ds(r, 8), :] = functools.reduce(jnp.add, terms)

                return [(fence(v_s[q]) if c % cfg["cv"] == 0 else None, functools.partial(work, r, c))
                        for r in range(first, last, 8) for c in range(4)]

            def prep_o(ps):
                def work(i, c, p):
                    op = _operands(LHS, p, lambda q, q2: o_s[q][2 * (q2 % 2) + c, pl.ds((q2 // 2) * Q + i, 16), :])
                    for p2 in range(NP):
                        oop[p][p2, c, pl.ds(i, 16), :] = op(p2)

                return [(fence(o_s[max(q for q in range(4) if LHS[p][q])]), functools.partial(work, i, c, p))
                        for p in ps for i in range(0, Q, 16) for c in range(2)]

            def project(m, a, dst, off):
                def product(p):
                    lhs = [_words(aop, (half_index(a, b) + p, c), t * Q, Q) for b, c in QUADS]
                    return [fill.dot(lhs, _cat(_load(wqk_op, (m, p, c), 0, 512) for c in range(4)), 4)]

                def done(q, val):
                    for c in range(4):
                        dst[4 * (q % 2) + c, pl.ds(off + (q // 2) * Q, Q), :] = _lanes(val[0], c)

                _strassen(product, done, orders["o_qk"])

            def two_level(lhs, rhs, done, order, before={}):
                def outer(p):
                    before.get(p, lambda: None)()
                    return _quadrants(
                        lambda p2: fill.dot([lhs(p, p2, c) for c in range(2)],
                                            _cat(_load(rhs, (p * NP + p2, c), 0, 256) for c in range(2))),
                        orders["o_at2"])

                _strassen(outer, done, order)

            def values(q, vals):
                for q2, v in enumerate(vals):
                    for c in range(2):
                        v_s[q][2 * (q2 % 2) + c, pl.ds(HALO + (q2 // 2) * Q, Q), :] = _lanes(v, c)
                if q < 2:
                    for c in range(4):
                        first = jnp.broadcast_to(v_s[q][c, pl.ds(HALO, 1), :], (HALO, 128))
                        v_s[q][c, head, :] = jnp.where(t > 0, v_s[q][c, head, :], first)
                    v_s[q + 2][:, head, :] = v_s[q][:, tail, :]

            def output(q, vals):
                for q2, v in enumerate(vals):
                    a, nq = _quarter(q, q2)
                    for c in range(2):
                        lead, start = (2 * (nq ^ 3) + c,), (4 * t + a) * Q
                        g = _load(ybuf, lead, start, Q).astype(F32)
                        xv = xbuf[4 * t + a, :, chunk_cols(lead[0])].astype(F32)
                        obuf[_rows(start, Q), chunk_cols(lead[0])] = (xv + _lanes(v, c) * g).astype(BF16)

            k0[:, head, :] = jnp.where(t > 0, k1[:, tail, :], 0.0)
            for q in range(2):
                v_s[q][:, head, :] = v_s[q + 2][:, tail, :]
            project(1, 0, k0, HALO)
            k1[:, head, :] = k0[:, tail, :]
            project(0, 0, q_s, 0)
            w = cfg["w"]
            fill.plan(*w[0], probs(0))
            fill.plan(*w[1], probs(1))
            fill.plan(*w[2], mix(1) + prep_o((2,)))
            fill.plan(*w[3], mix(2, HALO) + mix(2, 0, HALO) + prep_o((3, 0)))
            fill.plan(*w[4], mix(0) + prep_o((4, 6)))
            fill.plan(*w[5], mix(3) + prep_o((1, 5)))
            two_level(lambda p, p2, c: _words(aop, (p * NP + p2, c), t * Q, Q), wv_op, values, (2, 4, 3, 1, 0, 6, 5),
                      {cfg["kb"]: lambda: (project(1, 1, k1, HALO), project(0, 1, q_s, 2 * Q))})
            two_level(lambda p, p2, c: _words(oop[p], (p2, c), (t >> 3) * Q, Q), wo_op, output, (2, 3, 0, 4, 6, 1, 5))
            assert not fill.todo
            for cp in out_copies(t):
                cp.start()
            return carry

        if "3" in cfg["only"]:
          with jax.named_scope("ph3"):
            for t in range(refetch, NT):
                for cp in x_copies(t):
                    cp.start()
            lax.fori_loop(0, NT, tile, 0)
        for t in range(NT):
            for cp in out_copies(t):
                cp.wait()

    pl.run_scoped(
        attention,
        pltpu.VMEM((8, 4 * Q, 128), F32),
        *[pltpu.VMEM((WIN, 2 * Q, 128), F32)] * 2,
        pltpu.VMEM((S, D), BF16),
        *[pltpu.VMEM((8, HALO + 2 * Q + 8, 128), F32)] * 2,
        *[pltpu.VMEM((4, HALO + 2 * Q + 8, 128), F32)] * 4,
        *[pltpu.VMEM((4, 2 * Q + 8, 128), F32)] * 4,
        *[pltpu.VMEM((NP, 2, Q, 128), BF16)] * NP,
    )


DEFAULT = dict(sw=0, lag2=1.5, only="0123", ahead=3, mid=14, lag=1, wd0=(14, 21), wd1=(28, 35), wds=55,
               hp=(((4, 6), 0.5, 6.5), ((3,), 14, 21), ((0, 2), 28, 35.5), ((1, 5), 42, 47.5)),
               wdp=((0, 1), (2, 4), (3,), (5,), (6,)), dn=(10, 20, 32, 46),
               cq=4, cv=2, lag3=16, dynp=True, kb=2, w=((0, 50), (56, 84), (84, 95), (95, 108), (108, 120), (120, 132)),
               o_up="1342056", o_up2="1342056", o_dn="0123456", o_dn2="1324056",
               o_qk="1324056", o_at2="1324056")


def make(flags=None, interpret=False, **kw):
    cfg = dict(DEFAULT, **kw)

    def f(A_x, A_wqkv, A_wo, B_x, B_w_gate, B_w_up, B_w_down):
        del B_x
        any_spec = pl.BlockSpec(memory_space=pl.ANY)
        out = pl.pallas_call(
            functools.partial(_kernel, cfg=cfg),
            out_shape=jax.ShapeDtypeStruct((S, D), BF16),
            in_specs=[any_spec] * 6,
            out_specs=any_spec,
            scratch_shapes=[
                pltpu.VMEM((S // Q, Q, D), BF16),
                pltpu.VMEM((8, S, 128), BF16),
                pltpu.VMEM((NP * (NP + 2), 2, S // 4, 128), BF16),
                pltpu.VMEM((2, NP, 4, D // 2, 128), BF16),
                pltpu.VMEM((NP * NP, 2, D // 4, 128), BF16),
                pltpu.VMEM((NP * NP, 2, D // 4, 128), BF16),
                pltpu.SemaphoreType.DMA((NT,)),
                pltpu.SemaphoreType.DMA((2,)),
                pltpu.SemaphoreType.DMA((2,)),
                pltpu.SemaphoreType.DMA((3,)),
                pltpu.SemaphoreType.DMA((NT,)),
            ],
            compiler_params=pltpu.CompilerParams(
                vmem_limit_bytes=127 * 2**20, **({"flags": flags} if flags else {})),
            name="fused_block",
            interpret=interpret,
        )(A_x.reshape(S // Q, Q, D), A_wqkv.reshape(4, D // 4, 3 * D), A_wo, B_w_gate, B_w_up, B_w_down)
        return out.reshape(1, S, D)

    return f


@jax.jit
def pallas_recurrent_scan__sliding_local_dilated__geglu_ffn__prompt_kernel(
    A_x: jax.Array,
    A_wqkv: jax.Array,
    A_wo: jax.Array,
    B_x: jax.Array,
    B_w_gate: jax.Array,
    B_w_up: jax.Array,
    B_w_down: jax.Array,
):
    return make()(A_x, A_wqkv, A_wo, B_x, B_w_gate, B_w_up, B_w_down)
```

```python
import functools

import jax
import jax.numpy as jnp
from jax import lax
import jax.experimental.pallas as pl
import jax.experimental.pallas.tpu as pltpu

F32 = jnp.float32
BF16 = jnp.bfloat16
U32 = jnp.uint32

S, D, F = 2048, 1024, 3584
H, DH, WIN, DIL = 32, 32, 8, 2
HALO = 16
PITCH = DH + 1
Q = 64
NT = S // (4 * Q)
NJ = F // 512
NU = S // 512

LHS = ((1, 0, 0, 1), (0, 0, 1, 1), (1, 0, 0, 0), (0, 0, 0, 1),
       (1, 1, 0, 0), (-1, 0, 1, 0), (0, 1, 0, -1))
RHS = ((1, 0, 0, 1), (1, 0, 0, 0), (0, 1, 0, -1), (-1, 0, 1, 0),
       (0, 0, 0, 1), (1, 1, 0, 0), (0, 0, 1, 1))
OUT = ((1, 0, 0, 1), (0, 0, 1, -1), (0, 1, 0, 1), (1, 0, 1, 0),
       (-1, 1, 0, 0), (0, 0, 0, 1), (1, 0, 0, 0))
NP = 7
QUADS = ((0, 0), (0, 1), (1, 0), (1, 1))
GROUPS = ((0, 1), (2, 4), (3,), (5,), (6,))


def _lin(coef, quad):
    idx = sorted((q for q, c in enumerate(coef) if c), key=lambda q: -coef[q])
    if len(idx) == 1:
        return quad(idx[0])
    a, b = quad(idx[0]).astype(F32), quad(idx[1]).astype(F32)
    return a + b if coef[idx[1]] > 0 else a - b


def _operands(coefs, p, block):
    w = [_lin(coefs[p], lambda q: block(q, q2)) for q2 in range(4)]
    return lambda p2: _lin(coefs[p2], lambda q2: w[q2]).astype(BF16)


def _quarter(q, q2):
    return 2 * (q // 2) + q2 // 2, 2 * (q % 2) + q2 % 2


def _last_quadrant(p):
    return max(q for q in range(4) if LHS[p][q])


def _strassen(product, done, order):
    acc = [None] * 4
    left = [sum(1 for p in range(NP) if OUT[p][q]) for q in range(4)]
    for p in order:
        m = product(p)
        for q in range(4):
            s = OUT[p][q]
            if s == 0:
                continue
            if acc[q] is None:
                acc[q] = (s, m)
            else:
                s0, c = acc[q]
                assert s > 0 or s0 > 0
                acc[q] = (1, [x + y if s == s0 else (x - y if s > 0 else y - x)
                              for x, y in zip(m, c)])
            left[q] -= 1
            if left[q] == 0:
                done(q, acc[q][1])


def _quadrants(product, order):
    out = [None] * 4

    def done(q, val):
        out[q] = val[0]

    _strassen(lambda p: [product(p)], done, order)
    return out


def _cat(xs):
    return jnp.concatenate(list(xs), axis=1)


def _lanes(v, c):
    return v[:, c * 128:(c + 1) * 128]


def _gelu(g):
    half = 0.5 * g
    t = jnp.tanh(g * (0.7978845608028654 + 0.7978845608028654 * 0.044715 * (g * g)))
    return half * t + half


def _silu(d):
    half = 0.5 * d
    return half * jnp.tanh(half) + half


def _rows(start, size):
    return pl.ds(start if isinstance(start, int) else pl.multiple_of(start, size), size)


def _chunk(c):
    return _rows(c * 128, 128)


def _words(ref, lead, start, size):
    if ref.dtype == U32:
        return ref[(*lead, _rows(start >> 1, size // 2))]
    return pltpu.bitcast(ref[(*lead, _rows(start, size))], U32)


def _load(ref, lead, start, size):
    return pltpu.bitcast(_words(ref, lead, start, size), BF16)


def _store(ref, lead, start, val):
    size = val.shape[0]
    if ref.dtype == U32:
        ref[(*lead, _rows(start >> 1, size // 2))] = pltpu.bitcast(val, U32)
    else:
        ref[(*lead, _rows(start, size))] = val


class _Filler:
    def __init__(self, never, lag):
        self.never, self.lag = never, lag
        self.todo, self.marks, self.pos = [], [], 0

    def plan(self, first, last, pieces):
        self.todo += [(self.pos + first + i * (last - first) / len(pieces), piece)
                      for i, piece in enumerate(pieces)]
        self.todo.sort(key=lambda t: t[0])

    def dot(self, words, b, span=1):
        rows = [words[0][r:r + 8] for r in range(0, words[0].shape[0], 8)]
        while self.marks and self.marks[0][0] < self.pos + span:
            when, mark = self.marks.pop(0)
            r = int(max(when - self.pos, 0) / span * len(rows))
            rows[r] = jnp.where(self.never, mark, rows[r])
        a = _cat(pltpu.bitcast(x, BF16) for x in [jnp.concatenate(rows, axis=0)] + words[1:])
        m = jnp.dot(a, b, preferred_element_type=F32)
        nr, nc = m.shape[0] // 8, m.shape[1] // 128
        while self.todo and self.todo[0][0] < self.pos + span:
            when, (fence, work) = self.todo.pop(0)
            i = int(max(when - self.pos, 0) / span * nr * nc)
            r, c = divmod(i, nc) if a.shape[1] == 256 else divmod(i, nr)[::-1]
            if fence is not None:
                fence(_lanes(m, c)[8 * r:8 * r + 8])
            mark = work()
            if mark is not None:
                self.marks.append((when + self.lag, mark))
        self.pos += span
        return m


def _start(copies):
    for copy in copies:
        copy.start()


def _wait(copies):
    for copy in copies:
        copy.wait()


def _kernel(x_hbm, wqkv_hbm, wo_hbm, wg_hbm, wu_hbm, wd_hbm, out_hbm,
            xbuf, ybuf, aop, wqk_op, wv_op, wo_op, sem_x, sem_e, sem_l, sem_w, sem_o):

    def x_copy(t):
        rows = pl.ds(4 * t, 4)
        return pltpu.make_async_copy(x_hbm.at[rows], xbuf.at[rows], sem_x.at[t])

    def half_index(a, b):
        return {(0, 0): 2, (1, 1): 3, (0, 1): 7, (1, 0): 8}[a, b] * NP

    def ffn(hop, wd_op, wo_buf):

        def qkv_slab(u, m):
            return 8 + ((u & 1) * 3 + m) * 4

        def qkv_copies(u):
            return [pltpu.make_async_copy(wqkv_hbm.at[:, _rows(u * Q, Q), pl.ds(m * D, D)],
                                          xbuf.at[pl.ds(qkv_slab(u, m), 4)], sem_w.at[u & 1])
                    for m in range(3)]

        def wo_copies():
            return [pltpu.make_async_copy(wo_hbm.at[:, _chunk(c)], wo_buf.at[c, pl.ds(0, D)],
                                          sem_w.at[2]) for c in range(8)]

        def expand(wd_buf, *h_s):

            def clamp(j):
                return min(j, NJ - 1) if isinstance(j, int) else jnp.minimum(j, NJ - 1)

            def up_copies(j, c, sem):
                return [pltpu.make_async_copy(src.at[:, _chunk(4 * clamp(j) + cq)],
                                              ybuf.at[(j & 1) * 4 + cq, pl.ds(r, D)], sem.at[j & 1])
                        for cq in (2 * c, 2 * c + 1) for src, r in ((wg_hbm, 0), (wu_hbm, D))]

            def early_copies(j):
                return up_copies(j, 0, sem_e)

            def late_copies(j):
                return up_copies(j, 1, sem_l) + [pltpu.make_async_copy(
                    wd_hbm.at[_rows(clamp(j) * 512, 512)], wd_buf.at[j & 1, pl.ds(0, 512)],
                    sem_l.at[j & 1])]

            sum_s, mean_s, sq_s, rstd_s = h_s
            ahead = 3

            def x_rows(i, a, c):
                return xbuf[(i >> 2) * 4 + a, _rows((i & 3) * 16, 16), _chunk(c)].astype(F32)

            def lane_mean(v):
                return jnp.broadcast_to(jnp.sum(v, axis=-1, keepdims=True) * (1.0 / D), v.shape)

            def ln_sum(i, a, rows):
                sum_s[a, rows, :] = functools.reduce(jnp.add, [x_rows(i, a, c) for c in range(8)])

            def ln_mean(i, a, rows):
                mean_s[a, rows, :] = lane_mean(sum_s[a, rows, :])

            def ln_squares(i, a, rows):
                xc = [x_rows(i, a, c) - mean_s[a, rows, :] for c in range(8)]
                sq_s[a, rows, :] = functools.reduce(jnp.add, [v * v for v in xc])

            def ln_rstd(i, a, rows):
                rstd_s[a, rows, :] = lax.rsqrt(lane_mean(sq_s[a, rows, :]) + 1e-5)

            def ln_operands(i):
                rows = _rows(i * 16, 16)
                for c in range(2):
                    xn = {(a, k): (x_rows(i, a, 2 * k + c) - mean_s[a, rows, :]) * rstd_s[a, rows, :]
                          for a in range(4) for k in range(4)}
                    for p2 in range(NP):
                        inner = [_lin(LHS[p2], lambda q2: xn[_quarter(q, q2)]) for q in range(4)]
                        for q in (1, 2):
                            aop[half_index(*QUADS[q]) + p2, c, rows, :] = inner[q].astype(BF16)
                        for p in range(NP):
                            aop[p * NP + p2, c, rows, :] = _lin(LHS[p], lambda q: inner[q]).astype(BF16)

            def ln_step(i, lo=0, hi=5):
                if lo <= 4 < hi:
                    ln_operands(i - 4)
                for s, stage in ((3, ln_rstd), (2, ln_squares), (1, ln_mean), (0, ln_sum)):
                    if lo <= s < hi:
                        for a in range(4):
                            stage(i - s, a, _rows((i - s) * 16, 16))

            def ln_tile(t, carry):
                x_copy(t).wait()
                pl.when(t + ahead < NT)(lambda: x_copy(t + ahead).start())
                pl.when(t + ahead == NT)(lambda: _start(early_copies(0)))

                def step(i, carry):
                    ln_step(i)
                    return carry

                return lax.fori_loop(4 * t, 4 * t + 4, step, carry)

            _start(x_copy(t) for t in range(ahead))
            x_copy(0).wait()
            x_copy(ahead).start()
            for i in range(4):
                ln_step(i, hi=i + 1)
            lax.fori_loop(1, NT, ln_tile, 0)
            _start(late_copies(0))
            for i in range(4):
                ln_step(4 * NT + i, lo=i + 1)
            _start(qkv_copies(0) + qkv_copies(1) + wo_copies())

            def prep_wd(j):
                def fence(v):
                    wd_buf[j >> 3, pl.ds(512, 16), pl.ds(0, 128)] = pltpu.bitcast(v, BF16)

                def work(i, c, ps):
                    def block(q, q2):
                        kq, nq = _quarter(q, q2)
                        return wd_buf[j & 1, pl.ds((kq ^ 2) * 128 + i, 16), _chunk(2 * nq + c)]

                    for p in ps:
                        op = _operands(RHS, p, block)
                        for p2 in range(NP):
                            _store(wd_op, (p * NP + p2, c), j * 128 + i, op(p2))
                    return _words(wd_op, (j >> 3, 0), 0, 16)

                return [(fence, functools.partial(work, i, c, ps))
                        for i in range(0, 128, 16) for c in range(2) for ps in GROUPS]

            def prep_h(j, ps, ready):
                def fence(p, v):
                    h_s[_last_quadrant(p)][j >> 3, pl.ds(512, 8), :] = v

                def work(i, p):
                    assert ready(p)
                    op = _operands(LHS, p, lambda q, q2: h_s[q][q2, pl.ds(i, 16), :])
                    for p2 in range(NP):
                        hop[p * NP + p2, j, pl.ds(i, 16), :] = op(p2)
                    return _words(hop, (p * NP, j >> 3), 0, 16)

                return [(functools.partial(fence, p), functools.partial(work, i, p))
                        for i in range(0, 512, 16) for p in ps]

            def up_step(j, carry):
                _wait(early_copies(j))
                written = []

                def fresh(p):
                    return all(q in written for q in range(4) if LHS[p][q])

                fill = _Filler(j < 0, 1)
                pieces = prep_wd(j)
                fill.plan(14.6, 21.5, pieces[:55])
                fill.plan(26.5, 36.0, pieces[55:])
                fill.plan(0.5, 6.5, prep_h(jnp.maximum(j - 1, 0), (4, 6), lambda p: not written))
                fill.plan(14.3, 22, prep_h(j, (3,), fresh))
                fill.plan(28.3, 36.5, prep_h(j, (0, 2), fresh))
                fill.plan(42, 47.5, prep_h(j, (1, 5), fresh))

                def block(q, q2):
                    kq, cq = _quarter(q, q2)
                    return _cat(_load(ybuf, ((j & 1) * 4 + cq,), r + kq * 256, 256) for r in (0, D))

                def outer(p):
                    if p == 4:
                        _start(early_copies(j + 1) + late_copies(j + 1))
                        _wait(late_copies(j))
                    rhs = _operands(RHS, p, block)

                    def inner(p2):
                        lhs = [_words(aop, (p * NP + p2, c), 0, 512) for c in range(2)]
                        return fill.dot(lhs, rhs(p2))

                    return _quadrants(inner, (1, 3, 4, 2, 0, 5, 6))

                def done(q, vals):
                    for q2, v in enumerate(vals):
                        h_s[q ^ 1][q2, pl.ds(0, 512), :] = _gelu(_lanes(v, 0)) * _lanes(v, 1)
                    written.append(q ^ 1)

                _strassen(outer, done, (1, 3, 4, 2, 0, 5, 6))
                assert not fill.todo
                return carry

            lax.fori_loop(0, NJ, up_step, 0)
            for _, work in prep_h(NJ - 1, (4, 6), lambda p: True):
                work()
            _wait(early_copies(NJ) + late_copies(NJ))

        pl.run_scoped(expand, pltpu.VMEM((2, 512 + 16, D), BF16),
                      *[pltpu.VMEM((4, 512 + 8, 128), F32)] * 4)

        def contract(tmp_u, tmp_v, tmp_f):

            def prep_qkv(u):
                def fence_in(v):
                    xbuf[7 - (u >> 3), pl.ds(0, 16), pl.ds(0, 128)] = pltpu.bitcast(v, BF16)

                def fence_u(v):
                    tmp_u[u >> 3, pl.ds(H * PITCH, 8), :] = pltpu.bitcast(v, U32)

                def fence_v(v):
                    tmp_v[u >> 3, pl.ds(128, 8), :] = pltpu.bitcast(v, U32)

                def scatter(m, c):
                    w = [xbuf[qkv_slab(u, m) + kq, :, _chunk(c)] for kq in range(4)]
                    w = pltpu.bitcast(jnp.concatenate(w, axis=0), U32).T
                    for h in range(4):
                        tmp_u[m, pl.ds((4 * c + h) * PITCH, DH), :] = w[h * DH:(h + 1) * DH]

                def gather(m, c):
                    w = [tmp_u[m, pl.ds(4 * c + d, H, stride=PITCH), :] for d in range(4)]
                    tmp_v[8 * m + c, pl.ds(0, 128), :] = jnp.concatenate(w, axis=0).T

                def rows(m, c, kq, i):
                    return _load(tmp_v, (8 * m + c,), kq * Q + i, 16)

                def one_level(m, c, b):
                    for i in range(0, Q, 16):
                        for p in range(NP):
                            op = _lin(RHS[p], lambda q: rows(m, c + 4 * (q % 2), 2 * b + q // 2, i))
                            _store(wqk_op, (m, p, c), b * 256 + u * Q + i, op.astype(BF16))
                    return _words(wqk_op, (u >> 3, 0, 0), 0, 16)

                def two_level(c, i, ps):
                    def block(q, q2):
                        kq, nq = _quarter(q, q2)
                        return rows(2, 2 * nq + c, kq, i)

                    for p in ps:
                        op = _operands(RHS, p, block)
                        for p2 in range(NP):
                            _store(wv_op, (p * NP + p2, c), u * Q + i, op(p2))
                    return _words(wv_op, (u >> 3, 0), 0, 16)

                every = [(m, c) for m in range(3) for c in range(8)]
                return ([(fence_in, functools.partial(scatter, m, c)) for m, c in every],
                        [(fence_u, functools.partial(gather, m, c)) for m, c in every],
                        [(fence_v, functools.partial(one_level, m, c, b))
                         for m in range(2) for c in range(4) for b in range(2)]
                        + [(fence_v, functools.partial(two_level, c, i, ps))
                           for c in range(2) for i in range(0, Q, 16) for ps in GROUPS])

            def prep_wo(u):
                def fence_in(v):
                    wo_buf[u >> 3, pl.ds(D, 16), :] = pltpu.bitcast(v, BF16)

                def fence_f(v):
                    tmp_f[u >> 3, pl.ds(H * PITCH, 8), :] = v

                def scatter(h):
                    for nq in range(4):
                        w = _load(wo_buf, (2 * nq + (u & 1),), h * DH, DH)
                        tmp_f[nq, pl.ds(h * PITCH, DH), :] = w.astype(F32)
                    return pltpu.bitcast(tmp_f[u >> 3, pl.ds(0, 8), :], U32)

                def gather(d, h, ps):
                    d = (u >> 1) * 4 + d

                    def block(q, q2):
                        kq, nq = _quarter(q, q2)
                        first = h * PITCH + (kq ^ 2) * 8 + d
                        return tmp_f[nq ^ 3, pl.ds(first, 16, stride=PITCH), :]

                    for p in ps:
                        op = _operands(RHS, p, block)
                        for p2 in range(NP):
                            _store(wo_op, (p * NP + p2, u & 1), d * H + h, op(p2))
                    return _words(wo_op, (u >> 3, 0), 0, 16)

                return ([(fence_in, functools.partial(scatter, h)) for h in range(H)]
                        + [(fence_f, functools.partial(gather, d, h, ps))
                           for d in range(4) for h in (0, 16) for ps in GROUPS])

            def down_step(u, carry):
                _wait(qkv_copies(u))
                fill = _Filler(u < 0, 2.25)
                scatter, gather, combine = prep_qkv(u)
                fill.plan(0, 10, scatter)
                fill.plan(10, 20, gather)
                fill.plan(20, 32, prep_wo(u))
                fill.plan(32, 47, combine)

                def outer(p):
                    def inner(p2):
                        lhs = [_words(hop, (p * NP + p2, j), u * 128, 128) for j in range(NJ)]
                        rhs = _cat(_load(wd_op, (p * NP + p2, c), 0, F // 4) for c in range(2))
                        return fill.dot(lhs, rhs)

                    return _quadrants(inner, (1, 4, 3, 2, 0, 5, 6))

                def done(q, vals):
                    for q2, d in enumerate(vals):
                        a, nq = _quarter(q, q2)
                        g = _silu(d).astype(BF16)
                        for s in range(2):
                            for c in range(2):
                                rows = _rows(((2 * u + s) * 4 + a) * Q, Q)
                                ybuf[2 * nq + c, rows, :] = _lanes(g, c)[s * Q:(s + 1) * Q]

                _strassen(outer, done, range(NP))
                assert not fill.todo
                pl.when(u + 2 < NU)(lambda: _start(qkv_copies(u + 2)))
                return carry

            _wait(wo_copies())
            lax.fori_loop(0, NU, down_step, 0)

        pl.run_scoped(contract, pltpu.VMEM((3, (H + 1) * PITCH + 7, 128), U32),
                      pltpu.VMEM((24, 128 + 8, 128), U32),
                      pltpu.VMEM((4, (H + 1) * PITCH + 7, 128), F32))

    pl.run_scoped(ffn, pltpu.VMEM((NP * NP, NJ, S // 4, 128), BF16),
                  pltpu.VMEM((NP * NP, 2, F // 4, 128), BF16), pltpu.VMEM((8, D + 16, 128), BF16))

    def attention(q_s, obuf, *bufs):
        p_s, k_s, v_s, o_s, oop = bufs[:2], bufs[2:4], bufs[4:8], bufs[8:12], bufs[12:]

        def out_copy(t):
            rows = _rows(t * 4 * Q, 4 * Q)
            return pltpu.make_async_copy(obuf.at[rows], out_hbm.at[rows], sem_o.at[t])

        def tile(t, carry):
            pl.when(t >= 1)(lambda: x_copy(t).wait())
            fill = _Filler(t < 0, 14)
            tail, head = pl.ds(2 * Q, HALO), pl.ds(0, HALO)
            known = set()

            def fence(ref):
                def park(v):
                    ref[t >> 3, pl.ds(ref.shape[1] - 8, 8), :] = v
                return park

            def probs(a):
                pieces = []
                for r in range(0, 2 * Q, 8):
                    lg = [None] * WIN

                    def logits(c, r=r, lg=lg):
                        assert ("qk", a) in known
                        qv = q_s[c, pl.ds(a * 2 * Q + r, 8), :]
                        for w in range(WIN):
                            pr = qv * k_s[a][c, pl.ds(HALO + r - DIL * w, 8), :]
                            lg[w] = pr if c == 0 else lg[w] + pr

                    def softmax(r=r, lg=lg):
                        lg = [l + pltpu.roll(l, 64, 1) for l in lg]
                        lg = [(l + pltpu.roll(l, 32, 1)) * DH ** -0.5 for l in lg]
                        for w in range(WIN):
                            if a == 0 and r < DIL * w:
                                pos = t * 4 * Q + r + lax.broadcasted_iota(jnp.int32, (8, 128), 0)
                                lg[w] = jnp.where(pos >= DIL * w, lg[w], -1e9)
                        mx = functools.reduce(jnp.maximum, lg)
                        e = [jnp.exp(l - mx) for l in lg]
                        inv = 1.0 / functools.reduce(jnp.add, e)
                        for w in range(WIN):
                            p_s[a][w, pl.ds(r, 8), :] = e[w] * inv
                        return pltpu.bitcast(p_s[a][t >> 3, pl.ds(r, 8), :], U32)

                    pieces += [(None if c % 4 else fence(k_s[a]), functools.partial(logits, c))
                               for c in range(8)]
                    pieces.append((None, softmax))
                return pieces

            def mix(q, first=0, last=2 * Q):
                def work(r, c):
                    assert ("v", q) in known and (r >= HALO or ("v", q % 2) in known)
                    prow = _rows(r + 8 * (t >> (3 + q % 2)), 8)
                    terms = [p_s[q // 2][w, prow, :] * v_s[q][c, pl.ds(HALO + r - DIL * w, 8), :]
                             for w in range(WIN)]
                    o_s[q ^ 1][c, pl.ds(r, 8), :] = functools.reduce(jnp.add, terms)

                return [(None if c % 2 else fence(v_s[q]), functools.partial(work, r, c))
                        for r in range(first, last, 8) for c in range(4)]

            def prep_o(ps):
                def work(i, c, p):
                    assert ("wo", p) not in known
                    op = _operands(LHS, p, lambda q, q2: o_s[q][
                        2 * (q2 % 2) + c, pl.ds((q2 // 2) * Q + i, 16), :])
                    for p2 in range(NP):
                        oop[p][p2, c, pl.ds(i, 16), :] = op(p2)

                return [(fence(o_s[_last_quadrant(p)]), functools.partial(work, i, c, p))
                        for p in ps for i in range(0, Q, 16) for c in range(2)]

            def project(m, a, dst, off):
                def product(p):
                    lhs = [_words(aop, (half_index(a, b) + p, c), t * Q, Q) for b, c in QUADS]
                    return [fill.dot(lhs, _cat(_load(wqk_op, (m, p, c), 0, 512) for c in range(4)), 4)]

                def done(q, val):
                    for c in range(4):
                        dst[4 * (q % 2) + c, pl.ds(off + (q // 2) * Q, Q), :] = _lanes(val[0], c)

                _strassen(product, done, (4, 2, 3, 1, 0, 5, 6))

            def two_level(lhs, rhs, done, order, order2):
                def outer(p):
                    return _quadrants(lambda p2: fill.dot(
                        [lhs(p, p2, c) for c in range(2)],
                        _cat(_load(rhs, (p * NP + p2, c), 0, 256) for c in range(2))), order2)

                _strassen(outer, done, order)

            def values(q, vals):
                for q2, v in enumerate(vals):
                    for c in range(2):
                        v_s[q][2 * (q2 % 2) + c, pl.ds(HALO + (q2 // 2) * Q, Q), :] = _lanes(v, c)
                if q < 2:
                    for c in range(4):
                        first = jnp.broadcast_to(v_s[q][c, pl.ds(HALO, 1), :], (HALO, 128))
                        v_s[q][c, head, :] = jnp.where(t > 0, v_s[q][c, head, :], first)
                    v_s[q + 2][:, head, :] = v_s[q][:, tail, :]
                known.add(("v", q))

            def mixed(p, p2, c):
                known.add(("wo", p))
                return _words(oop[p], (p2, c), (t >> 3) * Q, Q)

            def output(q, vals):
                for q2, v in enumerate(vals):
                    a, nq = _quarter(q, q2)
                    for c in range(2):
                        col, start = 2 * (nq ^ 3) + c, (4 * t + a) * Q
                        g = _load(ybuf, (col,), start, Q).astype(F32)
                        xv = xbuf[4 * t + a, :, _chunk(col)].astype(F32)
                        obuf[_rows(start, Q), _chunk(col)] = (xv + _lanes(v, c) * g).astype(BF16)

            k_s[0][:, head, :] = jnp.where(t > 0, k_s[1][:, tail, :], 0.0)
            for q in range(2):
                v_s[q][:, head, :] = v_s[q + 2][:, tail, :]
            project(1, 0, k_s[0], HALO)
            k_s[1][:, head, :] = k_s[0][:, tail, :]
            project(0, 0, q_s, 0)
            known.add(("qk", 0))
            fill.plan(0, 50, probs(0))
            fill.plan(56, 84, probs(1))
            fill.plan(84, 95, mix(1) + prep_o((2,)))
            fill.plan(95, 108, mix(2, HALO) + mix(2, 0, HALO) + prep_o((3, 0)))
            fill.plan(108, 120, mix(0) + prep_o((4, 6)))
            fill.plan(120, 132, mix(3) + prep_o((1, 5)))
            project(1, 1, k_s[1], HALO)
            project(0, 1, q_s, 2 * Q)
            known.add(("qk", 1))
            two_level(lambda p, p2, c: _words(aop, (p * NP + p2, c), t * Q, Q), wv_op, values,
                      (2, 4, 3, 1, 0, 6, 5), (1, 3, 4, 2, 0, 5, 6))
            two_level(mixed, wo_op, output, (2, 3, 0, 4, 6, 1, 5), (1, 3, 4, 2, 0, 6, 5))
            assert not fill.todo
            out_copy(t).start()
            return carry

        _start(x_copy(t) for t in range(1, NT))
        lax.fori_loop(0, NT, tile, 0)
        _wait(out_copy(t) for t in range(NT))

    pl.run_scoped(
        attention,
        pltpu.VMEM((8, 4 * Q, 128), F32),
        pltpu.VMEM((S, D), BF16),
        *[pltpu.VMEM((WIN, 2 * Q, 128), F32)] * 2,
        *[pltpu.VMEM((8, HALO + 2 * Q + 8, 128), F32)] * 2,
        *[pltpu.VMEM((4, HALO + 2 * Q + 8, 128), F32)] * 4,
        *[pltpu.VMEM((4, 2 * Q + 8, 128), F32)] * 4,
        *[pltpu.VMEM((NP, 2, Q, 128), BF16)] * NP,
    )


@jax.jit
def pallas_recurrent_scan__sliding_local_dilated__geglu_ffn__prompt_kernel(
    A_x: jax.Array,
    A_wqkv: jax.Array,
    A_wo: jax.Array,
    B_x: jax.Array,
    B_w_gate: jax.Array,
    B_w_up: jax.Array,
    B_w_down: jax.Array,
):
    del B_x
    in_hbm = pl.BlockSpec(memory_space=pl.ANY)
    out = pl.pallas_call(
        _kernel,
        out_shape=jax.ShapeDtypeStruct((S, D), BF16),
        in_specs=[in_hbm] * 6,
        out_specs=in_hbm,
        scratch_shapes=[
            pltpu.VMEM((S // Q, Q, D), BF16),
            pltpu.VMEM((8, S, 128), BF16),
            pltpu.VMEM((NP * (NP + 2), 2, S // 4, 128), BF16),
            pltpu.VMEM((2, NP, 4, D // 2, 128), BF16),
            pltpu.VMEM((NP * NP, 2, D // 8, 128), U32),
            pltpu.VMEM((NP * NP, 2, D // 8, 128), U32),
            pltpu.SemaphoreType.DMA((NT,)),
            pltpu.SemaphoreType.DMA((2,)),
            pltpu.SemaphoreType.DMA((2,)),
            pltpu.SemaphoreType.DMA((3,)),
            pltpu.SemaphoreType.DMA((NT,)),
        ],
        compiler_params=pltpu.CompilerParams(vmem_limit_bytes=127 * 2**20),
        name="fused_block",
    )(A_x.reshape(S // Q, Q, D), A_wqkv.reshape(4, D // 4, 3 * D), A_wo,
      B_w_gate, B_w_up, B_w_down)
    return out.reshape(A_x.shape)
```

```python
import functools

import jax
import jax.numpy as jnp
from jax import lax
import jax.experimental.pallas as pl
import jax.experimental.pallas.tpu as pltpu

F32 = jnp.float32
BF16 = jnp.bfloat16
U32 = jnp.uint32

S, D, F = 2048, 1024, 3584
H, DH, WIN, DIL = 32, 32, 8, 2
HALO = 16
PITCH = DH + 1
Q = 64
NT = S // (4 * Q)
NJ = F // 512
NU = S // 512

LHS = ((1, 0, 0, 1), (0, 0, 1, 1), (1, 0, 0, 0), (0, 0, 0, 1),
       (1, 1, 0, 0), (-1, 0, 1, 0), (0, 1, 0, -1))
RHS = ((1, 0, 0, 1), (1, 0, 0, 0), (0, 1, 0, -1), (-1, 0, 1, 0),
       (0, 0, 0, 1), (1, 1, 0, 0), (0, 0, 1, 1))
OUT = ((1, 0, 0, 1), (0, 0, 1, -1), (0, 1, 0, 1), (1, 0, 1, 0),
       (-1, 1, 0, 0), (0, 0, 0, 1), (1, 0, 0, 0))
NP = 7
QUADS = ((0, 0), (0, 1), (1, 0), (1, 1))
GROUPS = ((0, 1), (2, 4), (3,), (5,), (6,))


def _lin(coef, quad):
    idx = sorted((q for q, c in enumerate(coef) if c), key=lambda q: -coef[q])
    if len(idx) == 1:
        return quad(idx[0])
    a, b = quad(idx[0]).astype(F32), quad(idx[1]).astype(F32)
    return a + b if coef[idx[1]] > 0 else a - b


def _operands(coefs, p, block):
    w = [_lin(coefs[p], lambda q: block(q, q2)) for q2 in range(4)]
    return lambda p2: _lin(coefs[p2], lambda q2: w[q2]).astype(BF16)


def _quarter(q, q2):
    return 2 * (q // 2) + q2 // 2, 2 * (q % 2) + q2 % 2


def _last_quadrant(p):
    return max(q for q in range(4) if LHS[p][q])


def _strassen(product, done, order):
    acc = [None] * 4
    left = [sum(1 for p in range(NP) if OUT[p][q]) for q in range(4)]
    for p in order:
        m = product(p)
        for q in range(4):
            s = OUT[p][q]
            if s == 0:
                continue
            if acc[q] is None:
                acc[q] = (s, m)
            else:
                s0, c = acc[q]
                assert s > 0 or s0 > 0
                acc[q] = (1, [x + y if s == s0 else (x - y if s > 0 else y - x)
                              for x, y in zip(m, c)])
            left[q] -= 1
            if left[q] == 0:
                done(q, acc[q][1])


def _quadrants(product, order):
    out = [None] * 4

    def done(q, val):
        out[q] = val[0]

    _strassen(lambda p: [product(p)], done, order)
    return out


def _cat(xs):
    return jnp.concatenate(list(xs), axis=1)


def _lanes(v, c):
    return v[:, c * 128:(c + 1) * 128]


def _gelu(g):
    half = 0.5 * g
    t = jnp.tanh(g * (0.7978845608028654 + 0.7978845608028654 * 0.044715 * (g * g)))
    return half * t + half


def _silu(d):
    half = 0.5 * d
    return half * jnp.tanh(half) + half


def _rows(start, size):
    return pl.ds(start if isinstance(start, int) else pl.multiple_of(start, size), size)


def _chunk(c):
    return _rows(c * 128, 128)


def _words(ref, lead, start, size):
    if ref.dtype == U32:
        return ref[(*lead, _rows(start >> 1, size // 2))]
    return pltpu.bitcast(ref[(*lead, _rows(start, size))], U32)


def _load(ref, lead, start, size):
    return pltpu.bitcast(_words(ref, lead, start, size), BF16)


def _store(ref, lead, start, val):
    size = val.shape[0]
    if ref.dtype == U32:
        ref[(*lead, _rows(start >> 1, size // 2))] = pltpu.bitcast(val, U32)
    else:
        ref[(*lead, _rows(start, size))] = val


class _Filler:
    def __init__(self, never, lag):
        self.never, self.lag = never, lag
        self.todo, self.marks, self.pos = [], [], 0

    def plan(self, first, last, pieces):
        self.todo += [(self.pos + first + i * (last - first) / len(pieces), piece)
                      for i, piece in enumerate(pieces)]
        self.todo.sort(key=lambda t: t[0])

    def dot(self, words, b, span=1):
        rows = [words[0][r:r + 8] for r in range(0, words[0].shape[0], 8)]
        while self.marks and self.marks[0][0] < self.pos + span:
            when, mark = self.marks.pop(0)
            r = int(max(when - self.pos, 0) / span * len(rows))
            rows[r] = jnp.where(self.never, mark, rows[r])
        a = _cat(pltpu.bitcast(x, BF16) for x in [jnp.concatenate(rows, axis=0)] + words[1:])
        m = jnp.dot(a, b, preferred_element_type=F32)
        nr, nc = m.shape[0] // 8, m.shape[1] // 128
        while self.todo and self.todo[0][0] < self.pos + span:
            when, (fence, work) = self.todo.pop(0)
            i = int(max(when - self.pos, 0) / span * nr * nc)
            r, c = divmod(i, nc) if a.shape[1] == 256 else divmod(i, nr)[::-1]
            if fence is not None:
                fence(_lanes(m, c)[8 * r:8 * r + 8])
            mark = work()
            if mark is not None:
                self.marks.append((when + self.lag, mark))
        self.pos += span
        return m


def _start(copies):
    for copy in copies:
        copy.start()


def _wait(copies):
    for copy in copies:
        copy.wait()


def _kernel(x_hbm, wqkv_hbm, wo_hbm, wg_hbm, wu_hbm, wd_hbm, out_hbm,
            xbuf, ybuf, aop, wqk_op, wv_op, wo_op, sem_x, sem_e, sem_l, sem_w, sem_o):

    def x_copy(t):
        rows = pl.ds(4 * t, 4)
        return pltpu.make_async_copy(x_hbm.at[rows], xbuf.at[rows], sem_x.at[t])

    def half_index(a, b):
        return {(0, 0): 2, (1, 1): 3, (0, 1): 7, (1, 0): 8}[a, b] * NP

    def ffn(hop, wd_op, wo_buf):

        def qkv_slab(u, m):
            return 8 + ((u & 1) * 3 + m) * 4

        def qkv_copies(u):
            return [pltpu.make_async_copy(wqkv_hbm.at[:, _rows(u * Q, Q), pl.ds(m * D, D)],
                                          xbuf.at[pl.ds(qkv_slab(u, m), 4)], sem_w.at[u & 1])
                    for m in range(3)]

        def wo_copies():
            return [pltpu.make_async_copy(wo_hbm.at[:, _chunk(c)], wo_buf.at[c, pl.ds(0, D)],
                                          sem_w.at[2]) for c in range(8)]

        def expand(wd_buf, *h_s):

            def clamp(j):
                return min(j, NJ - 1) if isinstance(j, int) else jnp.minimum(j, NJ - 1)

            def up_copies(j, c, sem):
                return [pltpu.make_async_copy(src.at[:, _chunk(4 * clamp(j) + cq)],
                                              ybuf.at[(j & 1) * 4 + cq, pl.ds(r, D)], sem.at[j & 1])
                        for cq in (2 * c, 2 * c + 1) for src, r in ((wg_hbm, 0), (wu_hbm, D))]

            def early_copies(j):
                return up_copies(j, 0, sem_e)

            def late_copies(j):
                return up_copies(j, 1, sem_l) + [pltpu.make_async_copy(
                    wd_hbm.at[_rows(clamp(j) * 512, 512)], wd_buf.at[j & 1, pl.ds(0, 512)],
                    sem_l.at[j & 1])]

            sum_s, mean_s, sq_s, rstd_s = h_s
            ahead = 3

            def x_rows(i, a, c):
                return xbuf[(i >> 2) * 4 + a, _rows((i & 3) * 16, 16), _chunk(c)].astype(F32)

            def lane_mean(v):
                return jnp.broadcast_to(jnp.sum(v, axis=-1, keepdims=True) * (1.0 / D), v.shape)

            def ln_sum(i, a, rows):
                sum_s[a, rows, :] = functools.reduce(jnp.add, [x_rows(i, a, c) for c in range(8)])

            def ln_mean(i, a, rows):
                mean_s[a, rows, :] = lane_mean(sum_s[a, rows, :])

            def ln_squares(i, a, rows):
                xc = [x_rows(i, a, c) - mean_s[a, rows, :] for c in range(8)]
                sq_s[a, rows, :] = functools.reduce(jnp.add, [v * v for v in xc])

            def ln_rstd(i, a, rows):
                rstd_s[a, rows, :] = lax.rsqrt(lane_mean(sq_s[a, rows, :]) + 1e-5)

            def ln_operands(i):
                rows = _rows(i * 16, 16)
                for c in range(2):
                    xn = {(a, k): (x_rows(i, a, 2 * k + c) - mean_s[a, rows, :]) * rstd_s[a, rows, :]
                          for a in range(4) for k in range(4)}
                    for p2 in range(NP):
                        inner = [_lin(LHS[p2], lambda q2: xn[_quarter(q, q2)]) for q in range(4)]
                        for q in (1, 2):
                            aop[half_index(*QUADS[q]) + p2, c, rows, :] = inner[q].astype(BF16)
                        for p in range(NP):
                            aop[p * NP + p2, c, rows, :] = _lin(LHS[p], lambda q: inner[q]).astype(BF16)

            def ln_step(i, lo=0, hi=5):
                if lo <= 4 < hi:
                    ln_operands(i - 4)
                for s, stage in ((3, ln_rstd), (2, ln_squares), (1, ln_mean), (0, ln_sum)):
                    if lo <= s < hi:
                        for a in range(4):
                            stage(i - s, a, _rows((i - s) * 16, 16))

            def ln_tile(t, carry):
                x_copy(t).wait()
                pl.when(t + ahead < NT)(lambda: x_copy(t + ahead).start())
                pl.when(t + ahead == NT)(lambda: _start(early_copies(0)))

                def step(i, carry):
                    ln_step(i)
                    return carry

                return lax.fori_loop(4 * t, 4 * t + 4, step, carry)

            _start(x_copy(t) for t in range(ahead))
            x_copy(0).wait()
            x_copy(ahead).start()
            for i in range(4):
                ln_step(i, hi=i + 1)
            lax.fori_loop(1, NT, ln_tile, 0)
            _start(late_copies(0))
            for i in range(4):
                ln_step(4 * NT + i, lo=i + 1)
            _start(qkv_copies(0) + qkv_copies(1) + wo_copies())

            def prep_wd(j):
                def fence(v):
                    wd_buf[j >> 3, pl.ds(512, 16), pl.ds(0, 128)] = pltpu.bitcast(v, BF16)

                def work(i, c, ps):
                    def block(q, q2):
                        kq, nq = _quarter(q, q2)
                        return wd_buf[j & 1, pl.ds((kq ^ 2) * 128 + i, 16), _chunk(2 * nq + c)]

                    for p in ps:
                        op = _operands(RHS, p, block)
                        for p2 in range(NP):
                            _store(wd_op, (p * NP + p2, c), j * 128 + i, op(p2))
                    return _words(wd_op, (j >> 3, 0), 0, 16)

                return [(fence, functools.partial(work, i, c, ps))
                        for i in range(0, 128, 16) for c in range(2) for ps in GROUPS]

            def prep_h(j, ps, ready):
                def fence(p, v):
                    h_s[_last_quadrant(p)][j >> 3, pl.ds(512, 8), :] = v

                def work(i, p):
                    assert ready(p)
                    op = _operands(LHS, p, lambda q, q2: h_s[q][q2, pl.ds(i, 16), :])
                    for p2 in range(NP):
                        hop[p * NP + p2, j, pl.ds(i, 16), :] = op(p2)
                    return _words(hop, (p * NP, j >> 3), 0, 16)

                return [(functools.partial(fence, p), functools.partial(work, i, p))
                        for i in range(0, 512, 16) for p in ps]

            def up_step(j, carry):
                _wait(early_copies(j))
                written = []

                def fresh(p):
                    return all(q in written for q in range(4) if LHS[p][q])

                fill = _Filler(j < 0, 1)
                pieces = prep_wd(j)
                fill.plan(14.6, 21.5, pieces[:55])
                fill.plan(26.5, 36.0, pieces[55:])
                fill.plan(0.5, 6.5, prep_h(jnp.maximum(j - 1, 0), (4, 6), lambda p: not written))
                fill.plan(14.3, 22, prep_h(j, (3,), fresh))
                fill.plan(28.3, 36.5, prep_h(j, (0, 2), fresh))
                fill.plan(42, 47.5, prep_h(j, (1, 5), fresh))

                def block(q, q2):
                    kq, cq = _quarter(q, q2)
                    return _cat(_load(ybuf, ((j & 1) * 4 + cq,), r + kq * 256, 256) for r in (0, D))

                def outer(p):
                    if p == 4:
                        _start(early_copies(j + 1) + late_copies(j + 1))
                        _wait(late_copies(j))
                    rhs = _operands(RHS, p, block)

                    def inner(p2):
                        lhs = [_words(aop, (p * NP + p2, c), 0, 512) for c in range(2)]
                        return fill.dot(lhs, rhs(p2))

                    return _quadrants(inner, (1, 3, 4, 2, 0, 5, 6))

                def done(q, vals):
                    for q2, v in enumerate(vals):
                        h_s[q ^ 1][q2, pl.ds(0, 512), :] = _gelu(_lanes(v, 0)) * _lanes(v, 1)
                    written.append(q ^ 1)

                _strassen(outer, done, (1, 3, 4, 2, 0, 5, 6))
                assert not fill.todo
                return carry

            lax.fori_loop(0, NJ, up_step, 0)
            for _, work in prep_h(NJ - 1, (4, 6), lambda p: True):
                work()
            _wait(early_copies(NJ) + late_copies(NJ))

        pl.run_scoped(expand, pltpu.VMEM((2, 512 + 16, D), BF16),
                      *[pltpu.VMEM((4, 512 + 8, 128), F32)] * 4)

        def contract(tmp_u, tmp_v, tmp_f):

            def prep_qkv(u):
                def fence_in(v):
                    xbuf[7 - (u >> 3), pl.ds(0, 16), pl.ds(0, 128)] = pltpu.bitcast(v, BF16)

                def fence_u(v):
                    tmp_u[u >> 3, pl.ds(H * PITCH, 8), :] = pltpu.bitcast(v, U32)

                def fence_v(v):
                    tmp_v[u >> 3, pl.ds(128, 8), :] = pltpu.bitcast(v, U32)

                def scatter(m, c):
                    w = [xbuf[qkv_slab(u, m) + kq, :, _chunk(c)] for kq in range(4)]
                    w = pltpu.bitcast(jnp.concatenate(w, axis=0), U32).T
                    for h in range(4):
                        tmp_u[m, pl.ds((4 * c + h) * PITCH, DH), :] = w[h * DH:(h + 1) * DH]

                def gather(m, c):
                    w = [tmp_u[m, pl.ds(4 * c + d, H, stride=PITCH), :] for d in range(4)]
                    tmp_v[8 * m + c, pl.ds(0, 128), :] = jnp.concatenate(w, axis=0).T

                def rows(m, c, kq, i):
                    return _load(tmp_v, (8 * m + c,), kq * Q + i, 16)

                def one_level(m, c, b):
                    for i in range(0, Q, 16):
                        for p in range(NP):
                            op = _lin(RHS[p], lambda q: rows(m, c + 4 * (q % 2), 2 * b + q // 2, i))
                            _store(wqk_op, (m, p, c), b * 256 + u * Q + i, op.astype(BF16))
                    return _words(wqk_op, (u >> 3, 0, 0), 0, 16)

                def two_level(c, i, ps):
                    def block(q, q2):
                        kq, nq = _quarter(q, q2)
                        return rows(2, 2 * nq + c, kq, i)

                    for p in ps:
                        op = _operands(RHS, p, block)
                        for p2 in range(NP):
                            _store(wv_op, (p * NP + p2, c), u * Q + i, op(p2))
                    return _words(wv_op, (u >> 3, 0), 0, 16)

                every = [(m, c) for m in range(3) for c in range(8)]
                return ([(fence_in, functools.partial(scatter, m, c)) for m, c in every],
                        [(fence_u, functools.partial(gather, m, c)) for m, c in every],
                        [(fence_v, functools.partial(one_level, m, c, b))
                         for m in range(2) for c in range(4) for b in range(2)]
                        + [(fence_v, functools.partial(two_level, c, i, ps))
                           for c in range(2) for i in range(0, Q, 16) for ps in GROUPS])

            def prep_wo(u):
                def fence_in(v):
                    wo_buf[u >> 3, pl.ds(D, 16), :] = pltpu.bitcast(v, BF16)

                def fence_f(v):
                    tmp_f[u >> 3, pl.ds(H * PITCH, 8), :] = v

                def scatter(h):
                    for nq in range(4):
                        w = _load(wo_buf, (2 * nq + (u & 1),), h * DH, DH)
                        tmp_f[nq, pl.ds(h * PITCH, DH), :] = w.astype(F32)
                    return pltpu.bitcast(tmp_f[u >> 3, pl.ds(0, 8), :], U32)

                def gather(d, h, ps):
                    d = (u >> 1) * 4 + d

                    def block(q, q2):
                        kq, nq = _quarter(q, q2)
                        first = h * PITCH + (kq ^ 2) * 8 + d
                        return tmp_f[nq ^ 3, pl.ds(first, 16, stride=PITCH), :]

                    for p in ps:
                        op = _operands(RHS, p, block)
                        for p2 in range(NP):
                            _store(wo_op, (p * NP + p2, u & 1), d * H + h, op(p2))
                    return _words(wo_op, (u >> 3, 0), 0, 16)

                return ([(fence_in, functools.partial(scatter, h)) for h in range(H)]
                        + [(fence_f, functools.partial(gather, d, h, ps))
                           for d in range(4) for h in (0, 16) for ps in GROUPS])

            def down_step(u, carry):
                _wait(qkv_copies(u))
                fill = _Filler(u < 0, 2.25)
                scatter, gather, combine = prep_qkv(u)
                fill.plan(0, 10, scatter)
                fill.plan(10, 20, gather)
                fill.plan(20, 32, prep_wo(u))
                fill.plan(32, 47, combine)

                def outer(p):
                    def inner(p2):
                        lhs = [_words(hop, (p * NP + p2, j), u * 128, 128) for j in range(NJ)]
                        rhs = _cat(_load(wd_op, (p * NP + p2, c), 0, F // 4) for c in range(2))
                        return fill.dot(lhs, rhs)

                    return _quadrants(inner, (1, 4, 3, 2, 0, 5, 6))

                def done(q, vals):
                    for q2, d in enumerate(vals):
                        a, nq = _quarter(q, q2)
                        g = _silu(d).astype(BF16)
                        for s in range(2):
                            for c in range(2):
                                rows = _rows(((2 * u + s) * 4 + a) * Q, Q)
                                ybuf[2 * nq + c, rows, :] = _lanes(g, c)[s * Q:(s + 1) * Q]

                _strassen(outer, done, range(NP))
                assert not fill.todo
                pl.when(u + 2 < NU)(lambda: _start(qkv_copies(u + 2)))
                return carry

            _wait(wo_copies())
            lax.fori_loop(0, NU, down_step, 0)

        pl.run_scoped(contract, pltpu.VMEM((3, (H + 1) * PITCH + 7, 128), U32),
                      pltpu.VMEM((24, 128 + 8, 128), U32),
                      pltpu.VMEM((4, (H + 1) * PITCH + 7, 128), F32))

    pl.run_scoped(ffn, pltpu.VMEM((NP * NP, NJ, S // 4, 128), BF16),
                  pltpu.VMEM((NP * NP, 2, F // 4, 128), BF16), pltpu.VMEM((8, D + 16, 128), BF16))

    def attention(q_s, obuf, *bufs):
        p_s, k_s, v_s, o_s, oop = bufs[:2], bufs[2:4], bufs[4:8], bufs[8:12], bufs[12:]

        def out_copy(t):
            rows = _rows(t * 2 * Q, 2 * Q)
            return pltpu.make_async_copy(obuf.at[rows], out_hbm.at[rows], sem_o.at[t])

        def tile(t, carry):
            pl.when(t >= 1)(lambda: x_copy(t).wait())
            fill = _Filler(t < 0, 14)
            tail, head = pl.ds(2 * Q, HALO), pl.ds(0, HALO)
            known = set()

            def fence(ref):
                def park(v):
                    ref[t >> 3, pl.ds(ref.shape[1] - 8, 8), :] = v
                return park

            def probs(a):
                pieces = []
                for r in range(0, 2 * Q, 8):
                    lg = [None] * WIN

                    def logits(c, r=r, lg=lg):
                        assert ("qk", a) in known
                        qv = q_s[c, pl.ds(a * 2 * Q + r, 8), :]
                        for w in range(WIN):
                            pr = qv * k_s[a][c, pl.ds(HALO + r - DIL * w, 8), :]
                            lg[w] = pr if c == 0 else lg[w] + pr

                    def softmax(r=r, lg=lg):
                        lg = [l + pltpu.roll(l, 64, 1) for l in lg]
                        lg = [(l + pltpu.roll(l, 32, 1)) * DH ** -0.5 for l in lg]
                        for w in range(WIN):
                            if a == 0 and r < DIL * w:
                                pos = t * 4 * Q + r + lax.broadcasted_iota(jnp.int32, (8, 128), 0)
                                lg[w] = jnp.where(pos >= DIL * w, lg[w], -1e9)
                        mx = functools.reduce(jnp.maximum, lg)
                        e = [jnp.exp(l - mx) for l in lg]
                        inv = 1.0 / functools.reduce(jnp.add, e)
                        for w in range(WIN):
                            p_s[a][w, pl.ds(r, 8), :] = e[w] * inv
                        return pltpu.bitcast(p_s[a][t >> 3, pl.ds(r, 8), :], U32)

                    pieces += [(None if c % 4 else fence(k_s[a]), functools.partial(logits, c))
                               for c in range(8)]
                    pieces.append((None, softmax))
                return pieces

            def mix(q, first=0, last=2 * Q):
                def work(r, c):
                    assert ("v", q) in known and (r >= HALO or ("v", q % 2) in known)
                    prow = _rows(r + 8 * (t >> (3 + q % 2)), 8)
                    terms = [p_s[q // 2][w, prow, :] * v_s[q][c, pl.ds(HALO + r - DIL * w, 8), :]
                             for w in range(WIN)]
                    o_s[q ^ 1][c, pl.ds(r, 8), :] = functools.reduce(jnp.add, terms)

                return [(None if c % 2 else fence(v_s[q]), functools.partial(work, r, c))
                        for r in range(first, last, 8) for c in range(4)]

            def prep_o(ps):
                def work(i, c, p):
                    assert ("wo", p) not in known
                    op = _operands(LHS, p, lambda q, q2: o_s[q][
                        2 * (q2 % 2) + c, pl.ds((q2 // 2) * Q + i, 16), :])
                    for p2 in range(NP):
                        oop[p][p2, c, pl.ds(i, 16), :] = op(p2)

                return [(fence(o_s[_last_quadrant(p)]), functools.partial(work, i, c, p))
                        for p in ps for i in range(0, Q, 16) for c in range(2)]

            def project(m, a, dst, off):
                def product(p):
                    lhs = [_words(aop, (half_index(a, b) + p, c), t * Q, Q) for b, c in QUADS]
                    return [fill.dot(lhs, _cat(_load(wqk_op, (m, p, c), 0, 512) for c in range(4)), 4)]

                def done(q, val):
                    for c in range(4):
                        dst[4 * (q % 2) + c, pl.ds(off + (q // 2) * Q, Q), :] = _lanes(val[0], c)

                _strassen(product, done, (4, 2, 3, 1, 0, 5, 6))

            def two_level(lhs, rhs, done, order, order2):
                def outer(p):
                    return _quadrants(lambda p2: fill.dot(
                        [lhs(p, p2, c) for c in range(2)],
                        _cat(_load(rhs, (p * NP + p2, c), 0, 256) for c in range(2))), order2)

                _strassen(outer, done, order)

            def values(q, vals):
                for q2, v in enumerate(vals):
                    for c in range(2):
                        v_s[q][2 * (q2 % 2) + c, pl.ds(HALO + (q2 // 2) * Q, Q), :] = _lanes(v, c)
                if q < 2:
                    for c in range(4):
                        first = jnp.broadcast_to(v_s[q][c, pl.ds(HALO, 1), :], (HALO, 128))
                        v_s[q][c, head, :] = jnp.where(t > 0, v_s[q][c, head, :], first)
                    v_s[q + 2][:, head, :] = v_s[q][:, tail, :]
                known.add(("v", q))

            def mixed(p, p2, c):
                known.add(("wo", p))
                return _words(oop[p], (p2, c), (t >> 3) * Q, Q)

            def output(q, vals):
                for q2, v in enumerate(vals):
                    a, nq = _quarter(q, q2)
                    for c in range(2):
                        col, start = 2 * (nq ^ 3) + c, (4 * t + a) * Q
                        g = _load(ybuf, (col,), start, Q).astype(F32)
                        xv = xbuf[4 * t + a, :, _chunk(col)].astype(F32)
                        obuf[_rows(start, Q), _chunk(col)] = (xv + _lanes(v, c) * g).astype(BF16)
                known.add(("out", q))
                if ("out", q ^ 1) in known:
                    out_copy(2 * t + q // 2).start()

            k_s[0][:, head, :] = jnp.where(t > 0, k_s[1][:, tail, :], 0.0)
            for q in range(2):
                v_s[q][:, head, :] = v_s[q + 2][:, tail, :]
            project(1, 0, k_s[0], HALO)
            k_s[1][:, head, :] = k_s[0][:, tail, :]
            project(0, 0, q_s, 0)
            known.add(("qk", 0))
            fill.plan(0, 50, probs(0))
            fill.plan(56, 84, probs(1))
            fill.plan(84, 95, mix(1) + prep_o((2,)))
            fill.plan(95, 108, mix(2, HALO) + mix(2, 0, HALO) + prep_o((3, 0)))
            fill.plan(108, 120, mix(0) + prep_o((4, 6)))
            fill.plan(120, 132, mix(3) + prep_o((1, 5)))
            project(1, 1, k_s[1], HALO)
            project(0, 1, q_s, 2 * Q)
            known.add(("qk", 1))
            two_level(lambda p, p2, c: _words(aop, (p * NP + p2, c), t * Q, Q), wv_op, values,
                      (2, 4, 3, 1, 0, 6, 5), (1, 3, 4, 2, 0, 5, 6))
            two_level(mixed, wo_op, output, (2, 3, 0, 4, 6, 1, 5), (1, 3, 4, 2, 0, 6, 5))
            assert not fill.todo
            return carry

        _start(x_copy(t) for t in range(1, NT))
        lax.fori_loop(0, NT, tile, 0)
        _wait(out_copy(t) for t in range(2 * NT))

    pl.run_scoped(
        attention,
        pltpu.VMEM((8, 4 * Q, 128), F32),
        pltpu.VMEM((S, D), BF16),
        *[pltpu.VMEM((WIN, 2 * Q, 128), F32)] * 2,
        *[pltpu.VMEM((8, HALO + 2 * Q + 8, 128), F32)] * 2,
        *[pltpu.VMEM((4, HALO + 2 * Q + 8, 128), F32)] * 4,
        *[pltpu.VMEM((4, 2 * Q + 8, 128), F32)] * 4,
        *[pltpu.VMEM((NP, 2, Q, 128), BF16)] * NP,
    )


@jax.jit
def pallas_recurrent_scan__sliding_local_dilated__geglu_ffn__prompt_kernel(
    A_x: jax.Array,
    A_wqkv: jax.Array,
    A_wo: jax.Array,
    B_x: jax.Array,
    B_w_gate: jax.Array,
    B_w_up: jax.Array,
    B_w_down: jax.Array,
):
    del B_x
    in_hbm = pl.BlockSpec(memory_space=pl.ANY)
    out = pl.pallas_call(
        _kernel,
        out_shape=jax.ShapeDtypeStruct((S, D), BF16),
        in_specs=[in_hbm] * 6,
        out_specs=in_hbm,
        scratch_shapes=[
            pltpu.VMEM((S // Q, Q, D), BF16),
            pltpu.VMEM((8, S, 128), BF16),
            pltpu.VMEM((NP * (NP + 2), 2, S // 4, 128), BF16),
            pltpu.VMEM((2, NP, 4, D // 2, 128), BF16),
            pltpu.VMEM((NP * NP, 2, D // 8, 128), U32),
            pltpu.VMEM((NP * NP, 2, D // 8, 128), U32),
            pltpu.SemaphoreType.DMA((NT,)),
            pltpu.SemaphoreType.DMA((2,)),
            pltpu.SemaphoreType.DMA((2,)),
            pltpu.SemaphoreType.DMA((3,)),
            pltpu.SemaphoreType.DMA((2 * NT,)),
        ],
        compiler_params=pltpu.CompilerParams(vmem_limit_bytes=127 * 2**20),
        name="fused_block",
    )(A_x.reshape(S // Q, Q, D), A_wqkv.reshape(4, D // 4, 3 * D), A_wo,
      B_w_gate, B_w_up, B_w_down)
    return out.reshape(A_x.shape)
```

```python
import functools

import jax
import jax.numpy as jnp
from jax import lax
import jax.experimental.pallas as pl
import jax.experimental.pallas.tpu as pltpu

F32 = jnp.float32
BF16 = jnp.bfloat16
U32 = jnp.uint32

S, D, F = 2048, 1024, 3584
H, DH, WIN, DIL = 32, 32, 8, 2
SCALE = DH ** -0.5
LOG2E = 1.4426950408889634
HALO = 16
PITCH = DH + 1
Q = 64
NT = S // (4 * Q)
NJ = F // 512
NU = S // 512

LHS = ((1, 0, 0, 1), (0, 0, 1, 1), (1, 0, 0, 0), (0, 0, 0, 1),
       (1, 1, 0, 0), (-1, 0, 1, 0), (0, 1, 0, -1))
RHS = ((1, 0, 0, 1), (1, 0, 0, 0), (0, 1, 0, -1), (-1, 0, 1, 0),
       (0, 0, 0, 1), (1, 1, 0, 0), (0, 0, 1, 1))
OUT = ((1, 0, 0, 1), (0, 0, 1, -1), (0, 1, 0, 1), (1, 0, 1, 0),
       (-1, 1, 0, 0), (0, 0, 0, 1), (1, 0, 0, 0))
NP = 7
QUADS = ((0, 0), (0, 1), (1, 0), (1, 1))
GROUPS = ((0, 1), (2, 4), (3,), (5,), (6,))


def _lin(coef, quad):
    idx = sorted((q for q, c in enumerate(coef) if c), key=lambda q: -coef[q])
    if len(idx) == 1:
        return quad(idx[0])
    a, b = quad(idx[0]).astype(F32), quad(idx[1]).astype(F32)
    return a + b if coef[idx[1]] > 0 else a - b


def _operands(coefs, p, block):
    w = [_lin(coefs[p], lambda q: block(q, q2)) for q2 in range(4)]
    return lambda p2: _lin(coefs[p2], lambda q2: w[q2]).astype(BF16)


def _quarter(q, q2):
    return 2 * (q // 2) + q2 // 2, 2 * (q % 2) + q2 % 2


def _last_quadrant(p):
    return max(q for q in range(4) if LHS[p][q])


def _strassen(product, done, order):
    acc = [None] * 4
    left = [sum(1 for p in range(NP) if OUT[p][q]) for q in range(4)]
    for p in order:
        m = product(p)
        for q in range(4):
            s = OUT[p][q]
            if s == 0:
                continue
            if acc[q] is None:
                acc[q] = (s, m)
            else:
                s0, c = acc[q]
                assert s > 0 or s0 > 0
                acc[q] = (1, [x + y if s == s0 else (x - y if s > 0 else y - x)
                              for x, y in zip(m, c)])
            left[q] -= 1
            if left[q] == 0:
                done(q, acc[q][1])


def _quadrants(product, order):
    out = [None] * 4

    def done(q, val):
        out[q] = val[0]

    _strassen(lambda p: [product(p)], done, order)
    return out


def _cat(xs):
    return jnp.concatenate(list(xs), axis=1)


def _lanes(v, c):
    return v[:, c * 128:(c + 1) * 128]


def _gelu(g):
    half = 0.5 * g
    t = jnp.tanh(g * (0.7978845608028654 + 0.7978845608028654 * 0.044715 * (g * g)))
    return half * t + half


def _silu(d):
    half = 0.5 * d
    return half * jnp.tanh(half) + half


def _rows(start, size):
    return pl.ds(start if isinstance(start, int) else pl.multiple_of(start, size), size)


def _chunk(c):
    return _rows(c * 128, 128)


def _words(ref, lead, start, size):
    if ref.dtype == U32:
        return ref[(*lead, _rows(start >> 1, size // 2))]
    return pltpu.bitcast(ref[(*lead, _rows(start, size))], U32)


def _load(ref, lead, start, size):
    return pltpu.bitcast(_words(ref, lead, start, size), BF16)


def _store(ref, lead, start, val):
    size = val.shape[0]
    if ref.dtype == U32:
        ref[(*lead, _rows(start >> 1, size // 2))] = pltpu.bitcast(val, U32)
    else:
        ref[(*lead, _rows(start, size))] = val


class _Filler:
    def __init__(self, never, lag):
        self.never, self.lag = never, lag
        self.todo, self.marks, self.pos = [], [], 0

    def plan(self, first, last, pieces):
        self.todo += [(self.pos + first + i * (last - first) / len(pieces), piece)
                      for i, piece in enumerate(pieces)]
        self.todo.sort(key=lambda t: t[0])

    def dot(self, words, b, span=1):
        rows = [words[0][r:r + 8] for r in range(0, words[0].shape[0], 8)]
        while self.marks and self.marks[0][0] < self.pos + span:
            when, mark = self.marks.pop(0)
            r = int(max(when - self.pos, 0) / span * len(rows))
            rows[r] = jnp.where(self.never, mark, rows[r])
        a = _cat(pltpu.bitcast(x, BF16) for x in [jnp.concatenate(rows, axis=0)] + words[1:])
        m = jnp.dot(a, b, preferred_element_type=F32)
        nr, nc = m.shape[0] // 8, m.shape[1] // 128
        while self.todo and self.todo[0][0] < self.pos + span:
            when, (fence, work) = self.todo.pop(0)
            i = int(max(when - self.pos, 0) / span * nr * nc)
            r, c = divmod(i, nc) if a.shape[1] == 256 else divmod(i, nr)[::-1]
            if fence is not None:
                fence(_lanes(m, c)[8 * r:8 * r + 8])
            mark = work()
            if mark is not None:
                self.marks.append((when + self.lag, mark))
        self.pos += span
        return m


def _start(copies):
    for copy in copies:
        copy.start()


def _wait(copies):
    for copy in copies:
        copy.wait()


def _kernel(x_hbm, wqkv_hbm, wo_hbm, wg_hbm, wu_hbm, wd_hbm, out_hbm,
            xbuf, ybuf, kbuf, wd_buf, aop, wq_op, wv_op, wo_op, sem_x, sem_k, sem_u, sem_w, sem_o):

    def x_copy(t):
        rows = pl.ds(4 * t, 4)
        return pltpu.make_async_copy(x_hbm.at[rows], xbuf.at[rows], sem_x.at[t])

    def half_index(a, b):
        return {(0, 0): 2, (1, 1): 3, (0, 1): 7, (1, 0): 8}[a, b] * NP

    def up_copies(j, which=range(9)):
        def ends(n):
            if n == 8:
                return wd_hbm.at[_rows(j * 512, 512)], wd_buf.at[j & 1, pl.ds(0, 512)]
            return ((wg_hbm, wu_hbm)[n % 2].at[:, _chunk(4 * j + n // 2)],
                    ybuf.at[(j & 1) * 4 + n // 2, pl.ds((n % 2) * D, D)])

        return [pltpu.make_async_copy(*ends(n), sem_u.at[j & 1]) for n in which]

    def scatter(src, slab, tmp_u, m, c):
        w = [src[slab + kq, :, _chunk(c)] for kq in range(4)]
        w = pltpu.bitcast(jnp.concatenate(w, axis=0), U32).T
        for h in range(4):
            tmp_u[m, pl.ds((4 * c + h) * PITCH, DH), :] = w[h * DH:(h + 1) * DH]

    def gather(tmp_u, tmp_v, m, c):
        w = [tmp_u[m, pl.ds(4 * c + d, H, stride=PITCH), :] for d in range(4)]
        tmp_v[8 * m + c, pl.ds(0, 128), :] = jnp.concatenate(w, axis=0).T

    def one_level(tmp_v, dst, u, c, b):
        for i in range(0, Q, 16):
            for p in range(NP):
                op = _lin(RHS[p], lambda q: _load(
                    tmp_v, (c + 4 * (q % 2),), (2 * b + q // 2) * Q + i, 16))
                _store(dst, (p, c), b * 256 + u * Q + i, op.astype(BF16))
        return _words(dst, (u >> 3, 0), 0, 16)

    def keys(wk_buf, wk_op, tmp_u, tmp_v, xn_s, sum_s, mean_s, sq_s, rstd_s):

        def k_copy(u):
            return pltpu.make_async_copy(wqkv_hbm.at[:, _rows(u * Q, Q), pl.ds(D, D)],
                                         wk_buf.at[pl.ds(4 * u, 4)], sem_k.at[u])

        def layernorm(t, strips=range(0, Q, 16)):
            def x_rows(i, a, c):
                return xbuf[4 * t + a, _rows(i, 16), _chunk(c)].astype(F32)

            def lane_mean(v):
                return jnp.broadcast_to(jnp.sum(v, axis=-1, keepdims=True) * (1.0 / D), v.shape)

            def total(i, a):
                xs = [x_rows(i, a, c) for c in range(8)]
                sum_s[a, _rows(i, 16), :] = functools.reduce(jnp.add, xs)

            def mean(i, a):
                mean_s[a, _rows(i, 16), :] = lane_mean(sum_s[a, _rows(i, 16), :])

            def squares(i, a):
                xc = [x_rows(i, a, c) - mean_s[a, _rows(i, 16), :] for c in range(8)]
                sq_s[a, _rows(i, 16), :] = functools.reduce(jnp.add, [v * v for v in xc])

            def rstd(i, a):
                rstd_s[a, _rows(i, 16), :] = lax.rsqrt(lane_mean(sq_s[a, _rows(i, 16), :]) + 1e-5)

            def scale(i, a):
                rows = _rows(i, 16)
                for c in range(8):
                    xn = (x_rows(i, a, c) - mean_s[a, rows, :]) * rstd_s[a, rows, :]
                    xn_s[c, _rows(a * Q + i, 16), :] = xn

            def operands(i, c, p):
                def block(q, q2):
                    a, k = _quarter(q, q2)
                    return xn_s[2 * k + c, _rows(a * Q + i, 16), :]

                op = _operands(LHS + ((0, 1, 0, 0), (0, 0, 1, 0)), p, block)
                for p2 in range(NP):
                    aop[p * NP + p2, c, _rows(t * Q + i, 16), :] = op(p2)

            return [[functools.partial(f, i, a) for i in strips for a in range(4)]
                    for f in (total, mean, squares, rstd, scale)] + [
                [functools.partial(operands, i, c, p)
                 for i in strips for c in range(2) for p in range(NP + 2)]]

        def run(stages):
            for works in stages:
                for work in works:
                    work()

        def prep_k(u, carry):
            k_copy(u).wait()
            x_copy(u + 1).start()
            run(layernorm(0, [16 * u])[5:])
            tmp_u[u >> 3, pl.ds(H * PITCH, 8), :] = _words(aop, (u >> 3, 0), 0, 16)
            for c in range(8):
                scatter(wk_buf, 4 * u, tmp_u, 0, c)
            for c in (0, 4, 1, 5, 2, 6, 3, 7):
                gather(tmp_u, tmp_v, 0, c)
            for c in range(4):
                for b in range(2):
                    one_level(tmp_v, wk_op, u, c, b)
            return carry

        def key_tile(t, carry):
            pl.when(t + 1 < NT)(lambda: x_copy(t + 1).wait())

            def fence(v):
                xbuf[S // Q - (t >> 3), pl.ds(0, 16), pl.ds(0, 128)] = pltpu.bitcast(v, BF16)

            def fence_xn(v):
                xn_s[t >> 3, pl.ds(4 * Q, 8), :] = v

            lhs = [[jnp.concatenate([_words(aop, (half_index(a, b) + p, c), t * Q, Q)
                                     for a in range(2)], axis=0) for b, c in QUADS]
                   for p in range(NP)]
            fill = _Filler(t < 0, 0)
            stages = layernorm(jnp.minimum(t + 1, NT - 1))
            fences = (fence, None, fence, None, fence, fence_xn)
            windows = ((0, 0.45), (0.45, 0.45), (0.75, 1.95), (1.95, 1.95), (1.95, 3.2), (3.35, 6.9))
            for works, window, f in zip(stages, windows, fences):
                fill.plan(*window, [(f, work) for work in works])

            def product(p):
                return [fill.dot(lhs[p], _cat(_load(wk_op, (p, c), 0, 512) for c in range(4)))]

            def done(q, val):
                k = val[0].astype(BF16)
                for a in range(2):
                    for c in range(4):
                        rows = _rows((4 * t + 2 * a + q // 2) * Q, Q)
                        kbuf[4 * (q % 2) + c, rows, :] = _lanes(k, c)[a * Q:(a + 1) * Q]

            _strassen(product, done, (1, 3, 4, 2, 0, 5, 6))
            assert not fill.todo
            return carry

        _start([x_copy(0)] + [k_copy(u) for u in range(3)])
        x_copy(0).wait()
        k_copy(3).start()
        run(layernorm(0)[:5])
        lax.fori_loop(0, 4, prep_k, 0)
        _start([x_copy(t) for t in range(5, NT)] + up_copies(0) + up_copies(1))
        lax.fori_loop(0, NT, key_tile, 0)

    pl.run_scoped(keys, pltpu.VMEM((16, Q, D), BF16), pltpu.VMEM((NP, 4, D // 2, 128), BF16),
                  pltpu.VMEM((1, (H + 1) * PITCH + 7, 128), U32), pltpu.VMEM((8, 128 + 8, 128), U32),
                  pltpu.VMEM((8, 4 * Q + 8, 128), F32), *[pltpu.VMEM((4, Q, 128), F32)] * 4)

    def ffn(hop, wd_op):

        def qv_slab(u, m):
            return ((u & 1) * 2 + m) * 4

        def qv_copies(u):
            return [pltpu.make_async_copy(wqkv_hbm.at[:, _rows(u * Q, Q), pl.ds(2 * m * D, D)],
                                          xbuf.at[pl.ds(qv_slab(u, m), 4)], sem_w.at[u & 1])
                    for m in range(2)]

        def wo_copy():
            return pltpu.make_async_copy(wo_hbm, xbuf.at[pl.ds(16, 16)], sem_w.at[2])

        def expand(*h_s):
            _start(qv_copies(0) + qv_copies(1) + [wo_copy()])

            def prep_wd(j):
                def fence(v):
                    wd_buf[j >> 3, pl.ds(512, 16), pl.ds(0, 128)] = pltpu.bitcast(v, BF16)

                def work(i, c, ps):
                    def block(q, q2):
                        kq, nq = _quarter(q, q2)
                        return wd_buf[j & 1, pl.ds((kq ^ 2) * 128 + i, 16), _chunk(2 * nq + c)]

                    for p in ps:
                        op = _operands(RHS, p, block)
                        for p2 in range(NP):
                            _store(wd_op, (p * NP + p2, c), j * 128 + i, op(p2))
                    return _words(wd_op, (j >> 3, 0), 0, 16)

                return [(fence, functools.partial(work, i, c, ps))
                        for i in range(0, 128, 16) for c in range(2) for ps in GROUPS]

            def prep_h(j, ps, ready):
                def fence(p, v):
                    h_s[_last_quadrant(p)][j >> 3, pl.ds(512, 8), :] = v

                def work(i, p):
                    assert ready(p)
                    op = _operands(LHS, p, lambda q, q2: h_s[q][q2, pl.ds(i, 16), :])
                    for p2 in range(NP):
                        hop[p * NP + p2, j, pl.ds(i, 16), :] = op(p2)
                    return _words(hop, (j >> 3, 0), 0, 16)

                return [(functools.partial(fence, p), functools.partial(work, i, p))
                        for i in range(0, 512, 16) for p in ps]

            def up_step(j, carry):
                _wait(up_copies(j))
                written = []

                def fresh(p):
                    return all(q in written for q in range(4) if LHS[p][q])

                fill = _Filler(j < 0, 0.75)
                pieces = prep_wd(j)
                fill.plan(14.6, 21.5, pieces[:45])
                fill.plan(25.5, 37, pieces[45:])
                fill.plan(1.1, 5.5, prep_h(jnp.maximum(j - 1, 0), (4, 6), lambda p: not written))
                fill.plan(14.3, 22, prep_h(j, (3,), fresh))
                fill.plan(29.2, 36, prep_h(j, (0, 2), fresh))
                fill.plan(42, 47, prep_h(j, (1, 5), fresh))

                def block(q, q2):
                    kq, cq = _quarter(q, q2)
                    return _cat(_load(ybuf, ((j & 1) * 4 + cq,), r + kq * 256, 256) for r in (0, D))

                def outer(p):
                    rhs = _operands(RHS, p, block)

                    def inner(p2):
                        lhs = [_words(aop, (p * NP + p2, c), 0, 512) for c in range(2)]
                        return fill.dot(lhs, rhs(p2))

                    return _quadrants(inner, (4, 2, 1, 3, 0, 6, 5))

                def done(q, vals):
                    for q2, v in enumerate(vals):
                        h_s[q ^ 1][q2, pl.ds(0, 512), :] = _gelu(_lanes(v, 0)) * _lanes(v, 1)
                    written.append(q ^ 1)

                _strassen(outer, done, (1, 3, 4, 2, 0, 5, 6))
                for n in range(0, 9, 3):
                    pl.when(j + 2 < NJ)(lambda: _start(up_copies(j + 2, range(n, n + 3))))
                assert not fill.todo
                return carry

            hop[0, 0, pl.ds(0, 16), :] = jnp.zeros((16, 128), BF16)
            lax.fori_loop(0, NJ, up_step, 0)
            for _, work in prep_h(NJ - 1, (4, 6), lambda p: True):
                work()

        pl.run_scoped(expand, *[pltpu.VMEM((4, 512 + 8, 128), F32)] * 4)

        def contract(tmp_u, tmp_v, tmp_f):

            def fence_in(u, v):
                xbuf[S // Q - (u >> 3), pl.ds(0, 16), pl.ds(0, 128)] = pltpu.bitcast(v, BF16)

            def prep_qv(u):
                def fence_u(v):
                    tmp_u[u >> 3, pl.ds(H * PITCH, 8), :] = pltpu.bitcast(v, U32)

                def fence_v(v):
                    tmp_v[u >> 3, pl.ds(128, 8), :] = pltpu.bitcast(v, U32)

                def two_level(c, i, ps):
                    def block(q, q2):
                        kq, nq = _quarter(q, q2)
                        return _load(tmp_v, (8 + 2 * nq + c,), kq * Q + i, 16)

                    for p in ps:
                        op = _operands(RHS, p, block)
                        for p2 in range(NP):
                            _store(wv_op, (p * NP + p2, c), u * Q + i, op(p2))
                    return _words(wv_op, (u >> 3, 0), 0, 16)

                every = [(m, c) for m in range(2) for c in range(8)]
                return ([(functools.partial(fence_in, u),
                          functools.partial(scatter, xbuf, qv_slab(u, m), tmp_u, m, c)) for m, c in every],
                        [(fence_u, functools.partial(gather, tmp_u, tmp_v, m, c)) for m, c in every],
                        [(fence_v, functools.partial(one_level, tmp_v, wq_op, u, c, b))
                         for c in range(4) for b in range(2)]
                        + [(fence_v, functools.partial(two_level, c, i, ps))
                           for c in range(2) for i in range(0, Q, 16) for ps in GROUPS])

            def prep_wo(u):
                def fence_f(v):
                    tmp_f[u >> 3, pl.ds(16 * PITCH, 8), :] = v

                def spread(h, cs):
                    for c in cs:
                        w = xbuf[16 + (u & 1) * 8 + h // 2, pl.ds((h % 2) * DH, DH), _chunk(c)]
                        tmp_f[c, pl.ds(h * PITCH, DH), :] = w.astype(F32)
                    return pltpu.bitcast(tmp_f[u >> 3, pl.ds(0, 8), :], U32)

                def collect(d, c, ps):
                    d = (u >> 1) * 4 + d

                    def block(q, q2):
                        kq, nq = _quarter(q, q2)
                        return tmp_f[2 * (nq ^ 3) + c, pl.ds((kq ^ 2) * 8 + d, 16, stride=PITCH), :]

                    for p in ps:
                        op = _operands(RHS, p, block)
                        for p2 in range(NP):
                            _store(wo_op, (p * NP + p2, c), d * H + (u & 1) * 16, op(p2))
                    return _words(wo_op, (u >> 3, 0), 0, 16)

                return ([(functools.partial(fence_in, u), functools.partial(spread, h, cs))
                         for h in range(16) for cs in (range(4), range(4, 8))]
                        + [(fence_f, functools.partial(collect, d, c, ps))
                           for d in range(4) for c in range(2) for ps in GROUPS])

            def down_step(u, carry):
                _wait(qv_copies(u))
                fill = _Filler(u < 0, 2.75)
                scatters, gathers, combines = prep_qv(u)
                fill.plan(0, 9.5, scatters)
                fill.plan(9.5, 14.5, gathers)
                fill.plan(14.5, 38, prep_wo(u))
                fill.plan(38, 47, combines)

                def outer(p):
                    def inner(p2):
                        lhs = [_words(hop, (p * NP + p2, j), u * 128, 128) for j in range(NJ)]
                        rhs = _cat(_load(wd_op, (p * NP + p2, c), 0, F // 4) for c in range(2))
                        return fill.dot(lhs, rhs)

                    return _quadrants(inner, (1, 4, 3, 2, 0, 5, 6))

                def done(q, vals):
                    for q2, d in enumerate(vals):
                        a, nq = _quarter(q, q2)
                        g = _silu(d).astype(BF16)
                        for s in range(2):
                            for c in range(2):
                                rows = _rows(((2 * u + s) * 4 + a) * Q, Q)
                                ybuf[2 * nq + c, rows, :] = _lanes(g, c)[s * Q:(s + 1) * Q]

                _strassen(outer, done, (1, 3, 2, 4, 0, 6, 5))
                assert not fill.todo
                pl.when(u + 2 < NU)(lambda: _start(qv_copies(u + 2)))
                pl.when(u + 2 == NU)(lambda: x_copy(0).start())
                return carry

            wo_copy().wait()
            lax.fori_loop(0, NU, down_step, 0)

        pl.run_scoped(contract, pltpu.VMEM((2, (H + 1) * PITCH + 7, 128), U32),
                      pltpu.VMEM((16, 128 + 8, 128), U32), pltpu.VMEM((8, 17 * PITCH + 7, 128), F32))

    pl.run_scoped(ffn, pltpu.VMEM((NP * NP, NJ, S // 4, 128), BF16),
                  pltpu.VMEM((NP * NP, 2, F // 4, 128), BF16))

    def attention(q_s, obuf, *bufs):
        p_s, k_s, v_s, o_s, oop = bufs[:2], bufs[2:4], bufs[4:8], bufs[8:12], bufs[12:]

        def out_copy(t):
            rows = _rows(t * 2 * Q, 2 * Q)
            return pltpu.make_async_copy(obuf.at[rows], out_hbm.at[rows], sem_o.at[t])

        def tile(t, carry):
            x_copy(t).wait()
            fill = _Filler(t < 0, 20)
            tail, head = pl.ds(2 * Q, HALO), pl.ds(0, HALO)
            known = set()

            def fence(ref):
                def park(v):
                    ref[t >> 3, pl.ds(ref.shape[1] - 8, 8), :] = v
                return park

            def probs(a):
                pieces = []
                for r in range(0, 2 * Q, 8):
                    lg = [None] * WIN

                    def logits(c, r=r, lg=lg):
                        assert ("qk", a) in known
                        qv = q_s[c, pl.ds(a * 2 * Q + r, 8), :]
                        for w in range(WIN):
                            pr = qv * k_s[a][c, pl.ds(HALO + r - DIL * w, 8), :]
                            lg[w] = pr if c == 0 else lg[w] + pr

                    def softmax(r=r, lg=lg):
                        lg = [l + pltpu.roll(l, 64, 1) for l in lg]
                        lg = [l + pltpu.roll(l, 32, 1) for l in lg]
                        for w in range(WIN):
                            if a == 0 and r < DIL * w:
                                pos = t * 4 * Q + r + lax.broadcasted_iota(jnp.int32, (8, 128), 0)
                                lg[w] = jnp.where(pos >= DIL * w, lg[w], -1e9 / SCALE)
                        mx = functools.reduce(jnp.maximum, lg)
                        e = [jnp.exp2((l - mx) * (SCALE * LOG2E)) for l in lg]
                        inv = 1.0 / functools.reduce(jnp.add, e)
                        for w in range(WIN):
                            p_s[a][w, pl.ds(r, 8), :] = e[w] * inv
                        return pltpu.bitcast(p_s[a][t >> 3, pl.ds(r, 8), :], U32)

                    pieces += [(None if c % 3 else fence(k_s[a]), functools.partial(logits, c))
                               for c in range(8)]
                    pieces.append((None, softmax))
                return pieces

            def mix(q, first=0, last=2 * Q):
                def work(r, c):
                    assert ("v", q) in known and (r >= HALO or ("v", q % 2) in known)
                    prow = _rows(r + 8 * (t >> (3 + q % 2)), 8)
                    terms = [p_s[q // 2][w, prow, :] * v_s[q][c, pl.ds(HALO + r - DIL * w, 8), :]
                             for w in range(WIN)]
                    o_s[q ^ 1][c, pl.ds(r, 8), :] = functools.reduce(jnp.add, terms)

                return [(None if c % 2 else fence(v_s[q]), functools.partial(work, r, c))
                        for r in range(first, last, 8) for c in range(4)]

            def prep_o(ps):
                def work(i, c, p):
                    assert ("wo", p) not in known
                    op = _operands(LHS, p, lambda q, q2: o_s[q][
                        2 * (q2 % 2) + c, pl.ds((q2 // 2) * Q + i, 16), :])
                    for p2 in range(NP):
                        oop[p][p2, c, pl.ds(i, 16), :] = op(p2)

                return [(fence(o_s[_last_quadrant(p)]), functools.partial(work, i, c, p))
                        for p in ps for i in range(0, Q, 16) for c in range(2)]

            def widen(a):
                def work(r, c):
                    k_s[a][c, pl.ds(HALO + r, Q), :] = _load(kbuf, (c,), (4 * t + 2 * a) * Q + r, Q).astype(F32)

                def park(v):
                    kbuf[t >> 3, pl.ds(S, 16), :] = pltpu.bitcast(v, BF16)

                return [(park, functools.partial(work, r, c)) for r in (0, Q) for c in range(8)]

            def queries(a):
                def product(p):
                    lhs = [_words(aop, (half_index(a, b) + p, c), t * Q, Q) for b, c in QUADS]
                    return [fill.dot(lhs, _cat(_load(wq_op, (p, c), 0, 512) for c in range(4)), 4)]

                def done(q, val):
                    for c in range(4):
                        q_s[4 * (q % 2) + c, pl.ds((2 * a + q // 2) * Q, Q), :] = _lanes(val[0], c)

                _strassen(product, done, (1, 3, 4, 0, 2, 5, 6))
                known.add(("qk", a))

            def two_level(lhs, rhs, done, order, order2):
                def outer(p):
                    return _quadrants(lambda p2: fill.dot(
                        [lhs(p, p2, c) for c in range(2)],
                        _cat(_load(rhs, (p * NP + p2, c), 0, 256) for c in range(2))), order2)

                _strassen(outer, done, order)

            def values(q, vals):
                for q2, v in enumerate(vals):
                    for c in range(2):
                        v_s[q][2 * (q2 % 2) + c, pl.ds(HALO + (q2 // 2) * Q, Q), :] = _lanes(v, c)
                if q < 2:
                    for c in range(4):
                        first = jnp.broadcast_to(v_s[q][c, pl.ds(HALO, 1), :], (HALO, 128))
                        v_s[q][c, head, :] = jnp.where(t > 0, v_s[q][c, head, :], first)
                    v_s[q + 2][:, head, :] = v_s[q][:, tail, :]
                known.add(("v", q))

            def mixed(p, p2, c):
                known.add(("wo", p))
                return _words(oop[p], (p2, c), (t >> 3) * Q, Q)

            def output(q, vals):
                for q2, v in enumerate(vals):
                    a, nq = _quarter(q, q2)
                    for c in range(2):
                        col, start = 2 * (nq ^ 3) + c, (4 * t + a) * Q
                        g = _load(ybuf, (col,), start, Q).astype(F32)
                        xv = xbuf[4 * t + a, :, _chunk(col)].astype(F32)
                        obuf[_rows(start, Q), _chunk(col)] = (xv + _lanes(v, c) * g).astype(BF16)
                known.add(("out", q))
                if ("out", q ^ 1) in known:
                    out_copy(2 * t + q // 2).start()

            k_s[0][:, head, :] = jnp.where(t > 0, k_s[1][:, tail, :], 0.0)
            for q in range(2):
                v_s[q][:, head, :] = v_s[q + 2][:, tail, :]
            fill.plan(0, 18, widen(0) + widen(1))
            queries(0)
            assert not fill.todo
            k_s[1][:, head, :] = k_s[0][:, tail, :]
            fill.plan(0, 27, probs(0))
            fill.plan(28, 55, probs(1))
            fill.plan(55, 67, mix(1) + prep_o((2,)))
            fill.plan(67, 79, mix(2, HALO) + mix(2, 0, HALO) + prep_o((3, 0)))
            fill.plan(79, 89, mix(0) + prep_o((4, 6)))
            fill.plan(89, 102, mix(3) + prep_o((1, 5)))
            queries(1)
            two_level(lambda p, p2, c: _words(aop, (p * NP + p2, c), t * Q, Q), wv_op, values,
                      (2, 4, 3, 1, 0, 6, 5), (4, 2, 3, 1, 0, 5, 6))
            two_level(mixed, wo_op, output, (2, 3, 0, 4, 6, 1, 5), (1, 3, 2, 4, 0, 6, 5))
            assert not fill.todo
            return carry

        _start(x_copy(t) for t in range(1, NT))
        lax.fori_loop(0, NT, tile, 0)
        _wait(out_copy(t) for t in range(2 * NT))

    pl.run_scoped(
        attention,
        pltpu.VMEM((8, 4 * Q, 128), F32),
        pltpu.VMEM((S, D), BF16),
        *[pltpu.VMEM((WIN, 2 * Q, 128), F32)] * 2,
        *[pltpu.VMEM((8, HALO + 2 * Q + 8, 128), F32)] * 2,
        *[pltpu.VMEM((4, HALO + 2 * Q + 8, 128), F32)] * 4,
        *[pltpu.VMEM((4, 2 * Q + 8, 128), F32)] * 4,
        *[pltpu.VMEM((NP, 2, Q, 128), BF16)] * NP,
    )


@jax.jit
def pallas_recurrent_scan__sliding_local_dilated__geglu_ffn__prompt_kernel(
    A_x: jax.Array,
    A_wqkv: jax.Array,
    A_wo: jax.Array,
    B_x: jax.Array,
    B_w_gate: jax.Array,
    B_w_up: jax.Array,
    B_w_down: jax.Array,
):
    del B_x
    in_hbm = pl.BlockSpec(memory_space=pl.ANY)
    out = pl.pallas_call(
        _kernel,
        out_shape=jax.ShapeDtypeStruct((S, D), BF16),
        in_specs=[in_hbm] * 6,
        out_specs=in_hbm,
        scratch_shapes=[
            pltpu.VMEM((S // Q + 1, Q, D), BF16),
            pltpu.VMEM((8, S, 128), BF16),
            pltpu.VMEM((8, S + 16, 128), BF16),
            pltpu.VMEM((2, 512 + 16, D), BF16),
            pltpu.VMEM((NP * (NP + 2), 2, S // 4, 128), BF16),
            pltpu.VMEM((NP, 4, D // 4, 128), U32),
            pltpu.VMEM((NP * NP, 2, D // 8, 128), U32),
            pltpu.VMEM((NP * NP, 2, D // 8, 128), U32),
            pltpu.SemaphoreType.DMA((NT,)),
            pltpu.SemaphoreType.DMA((4,)),
            pltpu.SemaphoreType.DMA((2,)),
            pltpu.SemaphoreType.DMA((3,)),
            pltpu.SemaphoreType.DMA((2 * NT,)),
        ],
        compiler_params=pltpu.CompilerParams(vmem_limit_bytes=127 * 2**20),
        name="fused_block",
    )(A_x.reshape(S // Q, Q, D), A_wqkv.reshape(4, D // 4, 3 * D), A_wo.reshape(D // Q, Q, D),
      B_w_gate, B_w_up, B_w_down)
    return out.reshape(A_x.shape)
```

```python
import functools

import jax
import jax.numpy as jnp
from jax import lax
import jax.experimental.pallas as pl
import jax.experimental.pallas.tpu as pltpu

F32 = jnp.float32
BF16 = jnp.bfloat16
U32 = jnp.uint32

S, D, F = 2048, 1024, 3584
H, DH, WIN, DIL = 32, 32, 8, 2
SCALE = DH ** -0.5
LOG2E = 1.4426950408889634
HALO = 16
PITCH = DH + 1
Q = 64
NT = S // (4 * Q)
NJ = F // 512
NU = S // 512

LHS = ((1, 0, 0, 1), (0, 0, 1, 1), (1, 0, 0, 0), (0, 0, 0, 1),
       (1, 1, 0, 0), (-1, 0, 1, 0), (0, 1, 0, -1))
RHS = ((1, 0, 0, 1), (1, 0, 0, 0), (0, 1, 0, -1), (-1, 0, 1, 0),
       (0, 0, 0, 1), (1, 1, 0, 0), (0, 0, 1, 1))
OUT = ((1, 0, 0, 1), (0, 0, 1, -1), (0, 1, 0, 1), (1, 0, 1, 0),
       (-1, 1, 0, 0), (0, 0, 0, 1), (1, 0, 0, 0))
NP = 7
QUADS = ((0, 0), (0, 1), (1, 0), (1, 1))
GROUPS = ((0, 1), (2, 4), (3,), (5,), (6,))
XN, WK, WG, WU, WD, WQ, WV, WO, FFN = range(9)
BALANCE = 6.0


def _lin(coef, quad):
    idx = sorted((q for q, c in enumerate(coef) if c), key=lambda q: -coef[q])
    if len(idx) == 1:
        return quad(idx[0])
    a, b = quad(idx[0]).astype(F32), quad(idx[1]).astype(F32)
    return a + b if coef[idx[1]] > 0 else a - b


def _operands(coefs, p, block):
    w = [_lin(coefs[p], lambda q: block(q, q2)) for q2 in range(4)]
    return lambda p2: _lin(coefs[p2], lambda q2: w[q2]).astype(BF16)


def _quarter(q, q2):
    return 2 * (q // 2) + q2 // 2, 2 * (q % 2) + q2 % 2


def _last_quadrant(p):
    return max(q for q in range(4) if LHS[p][q])


def _strassen(product, done, order):
    acc = [None] * 4
    left = [sum(1 for p in range(NP) if OUT[p][q]) for q in range(4)]
    for p in order:
        m = product(p)
        for q in range(4):
            s = OUT[p][q]
            if s == 0:
                continue
            if acc[q] is None:
                acc[q] = (s, m)
            else:
                s0, c = acc[q]
                assert s > 0 or s0 > 0
                acc[q] = (1, [x + y if s == s0 else (x - y if s > 0 else y - x)
                              for x, y in zip(m, c)])
            left[q] -= 1
            if left[q] == 0:
                done(q, acc[q][1])


def _quadrants(product, order):
    out = [None] * 4

    def done(q, val):
        out[q] = val[0]

    _strassen(lambda p: [product(p)], done, order)
    return out


def _cat(xs):
    return jnp.concatenate(list(xs), axis=1)


def _lanes(v, c):
    return v[:, c * 128:(c + 1) * 128]


def _gelu(g):
    half = 0.5 * g
    t = jnp.tanh(g * (0.7978845608028654 + 0.7978845608028654 * 0.044715 * (g * g)))
    return half * t + half


def _silu(d):
    half = 0.5 * d
    return half * jnp.tanh(half) + half


def _rows(start, size):
    return pl.ds(start if isinstance(start, int) else pl.multiple_of(start, size), size)


def _chunk(c):
    return _rows(c * 128, 128)


def _words(ref, lead, start, size):
    if ref.dtype == U32:
        return ref[(*lead, _rows(start >> 1, size // 2))]
    return pltpu.bitcast(ref[(*lead, _rows(start, size))], U32)


def _load(ref, lead, start, size):
    return pltpu.bitcast(_words(ref, lead, start, size), BF16)


def _store(ref, lead, start, val):
    size = val.shape[0]
    if ref.dtype == U32:
        ref[(*lead, _rows(start >> 1, size // 2))] = pltpu.bitcast(val, U32)
    else:
        ref[(*lead, _rows(start, size))] = val


class _Filler:
    def __init__(self, never, lag):
        self.never, self.lag = never, lag
        self.todo, self.marks, self.pos = [], [], 0

    def plan(self, first, last, pieces):
        self.todo += [(self.pos + first + i * (last - first) / len(pieces), piece)
                      for i, piece in enumerate(pieces)]
        self.todo.sort(key=lambda t: t[0])

    def dot(self, words, b, span=1):
        rows = [words[0][r:r + 8] for r in range(0, words[0].shape[0], 8)]
        while self.marks and self.marks[0][0] < self.pos + span:
            when, mark = self.marks.pop(0)
            r = int(max(when - self.pos, 0) / span * len(rows))
            rows[r] = jnp.where(self.never, mark, rows[r])
        a = _cat(pltpu.bitcast(x, BF16) for x in [jnp.concatenate(rows, axis=0)] + words[1:])
        m = jnp.dot(a, b, preferred_element_type=F32)
        nr, nc = m.shape[0] // 8, m.shape[1] // 128
        while self.todo and self.todo[0][0] < self.pos + span:
            when, (fence, work) = self.todo.pop(0)
            i = int(max(when - self.pos, 0) / span * nr * nc)
            r, c = divmod(i, nc) if a.shape[1] == 256 else divmod(i, nr)[::-1]
            if fence is not None:
                fence(_lanes(m, c)[8 * r:8 * r + 8])
            mark = work()
            if mark is not None:
                self.marks.append((when + self.lag, mark))
        self.pos += span
        return m


class _Range:
    def __init__(self, ref, slot):
        self.ref, self.slot, self.lo, self.hi = ref, slot, None, None

    def add(self, v):
        v = jnp.broadcast_to(v, (max(v.shape[0], 8), 128))
        for r in range(0, v.shape[0], 8):
            x = v[r:r + 8]
            self.lo = x if self.lo is None else jnp.minimum(self.lo, x)
            self.hi = x if self.hi is None else jnp.maximum(self.hi, x)

    def add_rows(self, squares):
        total = jnp.sum(functools.reduce(jnp.add, squares), axis=-1, keepdims=True)
        self.add(total * (1.0 / (128 * len(squares))))

    def save(self):
        self.ref[0, self.slot] = jnp.minimum(self.ref[0, self.slot], self.lo)
        self.ref[1, self.slot] = jnp.maximum(self.ref[1, self.slot], self.hi)
        self.lo = self.hi = None

    def matrix(self, load, rows, chunks, span):
        cols = [None] * chunks

        def work(r):
            w = [load(r, c).astype(F32) for c in range(chunks)]
            squares = [x * x for x in w]
            self.add_rows(squares)
            for c, x in enumerate(squares):
                cols[c] = x[:8] + x[8:] if r % span == 0 else cols[c] + x[:8] + x[8:]
            if (r + 16) % span == 0:
                for x in cols:
                    self.add(jnp.sum(x, axis=0, keepdims=True) * (1.0 / span))
                self.save()
            return pltpu.bitcast(functools.reduce(jnp.add, cols), U32)

        return [functools.partial(work, r) for r in range(0, rows, 16)]


def _start(copies):
    for copy in copies:
        copy.start()


def _wait(copies):
    for copy in copies:
        copy.wait()


def _kernel(x_hbm, wqkv_hbm, wo_hbm, wg_hbm, wu_hbm, wd_hbm, out_hbm,
            xbuf, ybuf, kbuf, wd_buf, aop, wq_op, wv_op, wo_op, ranges, energy,
            sem_x, sem_k, sem_u, sem_w, sem_o):

    def x_copy(t):
        rows = pl.ds(4 * t, 4)
        return pltpu.make_async_copy(x_hbm.at[rows], xbuf.at[rows], sem_x.at[t])

    def half_index(a, b):
        return {(0, 0): 2, (1, 1): 3, (0, 1): 7, (1, 0): 8}[a, b] * NP

    def up_copies(j, which=range(9)):
        def ends(n):
            if n == 8:
                return wd_hbm.at[_rows(j * 512, 512)], wd_buf.at[j & 1, pl.ds(0, 512)]
            return ((wg_hbm, wu_hbm)[n % 2].at[:, _chunk(4 * j + n // 2)],
                    ybuf.at[(j & 1) * 4 + n // 2, pl.ds((n % 2) * D, D)])

        return [pltpu.make_async_copy(*ends(n), sem_u.at[j & 1]) for n in which]

    def slabs(slot, src, first):
        return _Range(ranges, slot).matrix(
            lambda r, c: src[first + r // Q, pl.ds(r % Q, 16), _chunk(c)], 4 * Q, 8, 4 * Q)

    def scatter(src, slab, tmp_u, m, c):
        w = [src[slab + kq, :, _chunk(c)] for kq in range(4)]
        w = pltpu.bitcast(jnp.concatenate(w, axis=0), U32).T
        for h in range(4):
            tmp_u[m, pl.ds((4 * c + h) * PITCH, DH), :] = w[h * DH:(h + 1) * DH]

    def gather(tmp_u, tmp_v, m, c):
        w = [tmp_u[m, pl.ds(4 * c + d, H, stride=PITCH), :] for d in range(4)]
        tmp_v[8 * m + c, pl.ds(0, 128), :] = jnp.concatenate(w, axis=0).T

    def one_level(tmp_v, dst, u, c, b):
        for i in range(0, Q, 16):
            for p in range(NP):
                op = _lin(RHS[p], lambda q: _load(
                    tmp_v, (c + 4 * (q % 2),), (2 * b + q // 2) * Q + i, 16))
                _store(dst, (p, c), b * 256 + u * Q + i, op.astype(BF16))
        return _words(dst, (u >> 3, 0), 0, 16)

    def keys(wk_buf, wk_op, tmp_u, tmp_v, xn_s, sum_s, mean_s, sq_s, rstd_s):

        def k_copy(u):
            return pltpu.make_async_copy(wqkv_hbm.at[:, _rows(u * Q, Q), pl.ds(D, D)],
                                         wk_buf.at[pl.ds(4 * u, 4)], sem_k.at[u])

        def layernorm(t, strips=range(0, Q, 16)):
            seen = _Range(ranges, XN)

            def x_rows(i, a, c):
                return xbuf[4 * t + a, _rows(i, 16), _chunk(c)].astype(F32)

            def lane_mean(v):
                return jnp.broadcast_to(jnp.sum(v, axis=-1, keepdims=True) * (1.0 / D), v.shape)

            def total(i, a):
                xs = [x_rows(i, a, c) for c in range(8)]
                sum_s[a, _rows(i, 16), :] = functools.reduce(jnp.add, xs)

            def mean(i, a):
                mean_s[a, _rows(i, 16), :] = lane_mean(sum_s[a, _rows(i, 16), :])

            def squares(i, a):
                xc = [x_rows(i, a, c) - mean_s[a, _rows(i, 16), :] for c in range(8)]
                sq_s[a, _rows(i, 16), :] = functools.reduce(jnp.add, [v * v for v in xc])

            def rstd(i, a):
                var = lane_mean(sq_s[a, _rows(i, 16), :])
                r = lax.rsqrt(var + 1e-5)
                rstd_s[a, _rows(i, 16), :] = r
                seen.add(var * r * r)
                if a == 3:
                    seen.save()

            def scale(i, a):
                rows = _rows(i, 16)
                for c in range(8):
                    xn = (x_rows(i, a, c) - mean_s[a, rows, :]) * rstd_s[a, rows, :]
                    xn_s[c, _rows(a * Q + i, 16), :] = xn

            def operands(i, c, p):
                def block(q, q2):
                    a, k = _quarter(q, q2)
                    return xn_s[2 * k + c, _rows(a * Q + i, 16), :]

                op = _operands(LHS + ((0, 1, 0, 0), (0, 0, 1, 0)), p, block)
                for p2 in range(NP):
                    aop[p * NP + p2, c, _rows(t * Q + i, 16), :] = op(p2)

            return [[functools.partial(f, i, a) for i in strips for a in range(4)]
                    for f in (total, mean, squares, rstd, scale)] + [
                [functools.partial(operands, i, c, p)
                 for i in strips for c in range(2) for p in range(NP + 2)]]

        def run(stages):
            for works in stages:
                for work in works:
                    work()

        def prep_k(u, carry):
            k_copy(u).wait()
            x_copy(u + 1).start()
            run(layernorm(0, [16 * u])[5:])
            tmp_u[u >> 3, pl.ds(H * PITCH, 8), :] = _words(aop, (u >> 3, 0), 0, 16)
            for c in range(8):
                scatter(wk_buf, 4 * u, tmp_u, 0, c)
            for c in (0, 4, 1, 5, 2, 6, 3, 7):
                gather(tmp_u, tmp_v, 0, c)
            for c in range(4):
                for b in range(2):
                    one_level(tmp_v, wk_op, u, c, b)
            return carry

        def key_tile(t, carry):
            pl.when(t + 1 < NT)(lambda: x_copy(t + 1).wait())

            def fence(v):
                xbuf[S // Q - (t >> 3), pl.ds(0, 16), pl.ds(0, 128)] = pltpu.bitcast(v, BF16)

            def fence_xn(v):
                xn_s[t >> 3, pl.ds(4 * Q, 8), :] = v

            lhs = [[jnp.concatenate([_words(aop, (half_index(a, b) + p, c), t * Q, Q)
                                     for a in range(2)], axis=0) for b, c in QUADS]
                   for p in range(NP)]
            fill = _Filler(t < 0, 0)
            stages = layernorm(jnp.minimum(t + 1, NT - 1))
            fences = (fence, None, fence, None, fence, fence_xn)
            windows = ((0, 0.45), (0.45, 0.45), (0.75, 1.95), (1.95, 1.95), (1.95, 3.2), (3.35, 6.9))
            for works, window, f in zip(stages, windows, fences):
                fill.plan(*window, [(f, work) for work in works])

            def product(p):
                return [fill.dot(lhs[p], _cat(_load(wk_op, (p, c), 0, 512) for c in range(4)))]

            def done(q, val):
                k = val[0].astype(BF16)
                for a in range(2):
                    for c in range(4):
                        rows = _rows((4 * t + 2 * a + q // 2) * Q, Q)
                        kbuf[4 * (q % 2) + c, rows, :] = _lanes(k, c)[a * Q:(a + 1) * Q]

            _strassen(product, done, (1, 3, 4, 2, 0, 5, 6))
            assert not fill.todo
            return carry

        _start([x_copy(0)] + [k_copy(u) for u in range(3)])
        ranges[0] = jnp.full(ranges.shape[1:], jnp.inf, F32)
        ranges[1] = jnp.zeros(ranges.shape[1:], F32)
        x_copy(0).wait()
        k_copy(3).start()
        run(layernorm(0)[:5])
        lax.fori_loop(0, 4, prep_k, 0)
        _start([x_copy(t) for t in range(5, NT)] + up_copies(0) + up_copies(1))
        lax.fori_loop(0, NT, key_tile, 0)

    pl.run_scoped(keys, pltpu.VMEM((16, Q, D), BF16), pltpu.VMEM((NP, 4, D // 2, 128), BF16),
                  pltpu.VMEM((1, (H + 1) * PITCH + 7, 128), U32), pltpu.VMEM((8, 128 + 8, 128), U32),
                  pltpu.VMEM((8, 4 * Q + 8, 128), F32), *[pltpu.VMEM((4, Q, 128), F32)] * 4)

    def ffn(hop, wd_op):

        def qv_slab(u, m):
            return ((u & 1) * 2 + m) * 4

        def qv_copies(u):
            return [pltpu.make_async_copy(wqkv_hbm.at[:, _rows(u * Q, Q), pl.ds(2 * m * D, D)],
                                          xbuf.at[pl.ds(qv_slab(u, m), 4)], sem_w.at[u & 1])
                    for m in range(2)]

        def wo_copy():
            return pltpu.make_async_copy(wo_hbm, xbuf.at[pl.ds(16, 16)], sem_w.at[2])

        def wk_copies(slot):
            return [pltpu.make_async_copy(wqkv_hbm.at[2 * slot + n, :, pl.ds(D, D)],
                                          wd_buf.at[slot, pl.ds(256 * n, 256)], sem_u.at[slot])
                    for n in range(2)]

        def expand(*h_s):
            _start(qv_copies(0) + qv_copies(1) + [wo_copy()])

            def prep_wd(j):
                def fence(v):
                    wd_buf[j >> 3, pl.ds(512, 16), pl.ds(0, 128)] = pltpu.bitcast(v, BF16)

                def work(i, c, ps):
                    def block(q, q2):
                        kq, nq = _quarter(q, q2)
                        return wd_buf[j & 1, pl.ds((kq ^ 2) * 128 + i, 16), _chunk(2 * nq + c)]

                    for p in ps:
                        op = _operands(RHS, p, block)
                        for p2 in range(NP):
                            _store(wd_op, (p * NP + p2, c), j * 128 + i, op(p2))
                    return _words(wd_op, (j >> 3, 0), 0, 16)

                return [(fence, functools.partial(work, i, c, ps))
                        for i in range(0, 128, 16) for c in range(2) for ps in GROUPS]

            def prep_h(j, ps, ready):
                def fence(p, v):
                    h_s[_last_quadrant(p)][j >> 3, pl.ds(512, 8), :] = v

                def work(i, p):
                    assert ready(p)
                    op = _operands(LHS, p, lambda q, q2: h_s[q][q2, pl.ds(i, 16), :])
                    for p2 in range(NP):
                        hop[p * NP + p2, j, pl.ds(i, 16), :] = op(p2)
                    return _words(hop, (j >> 3, 0), 0, 16)

                return [(functools.partial(fence, p), functools.partial(work, i, p))
                        for i in range(0, 512, 16) for p in ps]

            def balance_up(j, slot, top):
                parked = []

                def fence(v):
                    parked.append(pltpu.bitcast(v, U32))

                def load(r, c):
                    w = _words(ybuf, ((j & 1) * 4 + c + (j >> 3),), top + r, 16)
                    return pltpu.bitcast(jnp.where(j < 0, parked[-1], w), BF16)

                return [(fence, work) for work in _Range(ranges, slot).matrix(load, D, 4, D)]

            def up_step(j, carry):
                _wait(up_copies(j))
                written = []

                def fresh(p):
                    return all(q in written for q in range(4) if LHS[p][q])

                fill = _Filler(j < 0, 0.75)
                pieces = prep_wd(j)
                fill.plan(14.6, 21.5, pieces[:45])
                fill.plan(25.5, 37, pieces[45:])
                fill.plan(1.1, 5.5, prep_h(jnp.maximum(j - 1, 0), (4, 6), lambda p: not written))
                fill.plan(14.3, 22, prep_h(j, (3,), fresh))
                fill.plan(29.2, 36, prep_h(j, (0, 2), fresh))
                fill.plan(42, 47, prep_h(j, (1, 5), fresh))
                fill.plan(0.3, 10, balance_up(j, WG, 0))
                fill.plan(14, 24, balance_up(j, WU, D))
                fill.plan(28, 40, [(pieces[0][0], work) for work in _Range(ranges, WD).matrix(
                    lambda r, c: wd_buf[j & 1, pl.ds(r % 512, 16), _chunk(4 * (r // 512) + c)],
                    D, 4, 512)])

                def block(q, q2):
                    kq, cq = _quarter(q, q2)
                    return _cat(_load(ybuf, ((j & 1) * 4 + cq,), r + kq * 256, 256) for r in (0, D))

                def outer(p):
                    rhs = _operands(RHS, p, block)

                    def inner(p2):
                        lhs = [_words(aop, (p * NP + p2, c), 0, 512) for c in range(2)]
                        return fill.dot(lhs, rhs(p2))

                    return _quadrants(inner, (4, 2, 1, 3, 0, 6, 5))

                def done(q, vals):
                    for q2, v in enumerate(vals):
                        h_s[q ^ 1][q2, pl.ds(0, 512), :] = _gelu(_lanes(v, 0)) * _lanes(v, 1)
                    written.append(q ^ 1)

                _strassen(outer, done, (1, 3, 4, 2, 0, 5, 6))
                for n in range(0, 9, 3):
                    pl.when(j + 2 < NJ)(lambda: _start(up_copies(j + 2, range(n, n + 3))))
                pl.when(j + 2 >= NJ)(lambda: _start(wk_copies(j & 1)))
                assert not fill.todo
                return carry

            hop[0, 0, pl.ds(0, 16), :] = jnp.zeros((16, 128), BF16)
            lax.fori_loop(0, NJ, up_step, 0)
            for _, work in prep_h(NJ - 1, (4, 6), lambda p: True):
                work()

        pl.run_scoped(expand, *[pltpu.VMEM((4, 512 + 8, 128), F32)] * 4)

        def contract(tmp_u, tmp_v, tmp_f):

            def fence_in(u, v):
                xbuf[S // Q - (u >> 3), pl.ds(0, 16), pl.ds(0, 128)] = pltpu.bitcast(v, BF16)

            def prep_qv(u):
                def fence_u(v):
                    tmp_u[u >> 3, pl.ds(H * PITCH, 8), :] = pltpu.bitcast(v, U32)

                def fence_v(v):
                    tmp_v[u >> 3, pl.ds(128, 8), :] = pltpu.bitcast(v, U32)

                def two_level(c, i, ps):
                    def block(q, q2):
                        kq, nq = _quarter(q, q2)
                        return _load(tmp_v, (8 + 2 * nq + c,), kq * Q + i, 16)

                    for p in ps:
                        op = _operands(RHS, p, block)
                        for p2 in range(NP):
                            _store(wv_op, (p * NP + p2, c), u * Q + i, op(p2))
                    return _words(wv_op, (u >> 3, 0), 0, 16)

                every = [(m, c) for m in range(2) for c in range(8)]
                return ([(functools.partial(fence_in, u),
                          functools.partial(scatter, xbuf, qv_slab(u, m), tmp_u, m, c)) for m, c in every],
                        [(fence_u, functools.partial(gather, tmp_u, tmp_v, m, c)) for m, c in every],
                        [(fence_v, functools.partial(one_level, tmp_v, wq_op, u, c, b))
                         for c in range(4) for b in range(2)]
                        + [(fence_v, functools.partial(two_level, c, i, ps))
                           for c in range(2) for i in range(0, Q, 16) for ps in GROUPS])

            def prep_wo(u):
                def fence_f(v):
                    tmp_f[u >> 3, pl.ds(16 * PITCH, 8), :] = v

                def spread(h, cs):
                    for c in cs:
                        w = xbuf[16 + (u & 1) * 8 + h // 2, pl.ds((h % 2) * DH, DH), _chunk(c)]
                        tmp_f[c, pl.ds(h * PITCH, DH), :] = w.astype(F32)
                    return pltpu.bitcast(tmp_f[u >> 3, pl.ds(0, 8), :], U32)

                def collect(d, c, ps):
                    d = (u >> 1) * 4 + d

                    def block(q, q2):
                        kq, nq = _quarter(q, q2)
                        return tmp_f[2 * (nq ^ 3) + c, pl.ds((kq ^ 2) * 8 + d, 16, stride=PITCH), :]

                    for p in ps:
                        op = _operands(RHS, p, block)
                        for p2 in range(NP):
                            _store(wo_op, (p * NP + p2, c), d * H + (u & 1) * 16, op(p2))
                    return _words(wo_op, (u >> 3, 0), 0, 16)

                return ([(functools.partial(fence_in, u), functools.partial(spread, h, cs))
                         for h in range(16) for cs in (range(4), range(4, 8))]
                        + [(fence_f, functools.partial(collect, d, c, ps))
                           for d in range(4) for c in range(2) for ps in GROUPS])

            def down_step(u, carry):
                _wait(qv_copies(u))
                pl.when((u & 1) == 0)(lambda: _wait(wk_copies(1 - (u >> 1))))
                fill = _Filler(u < 0, 2.75)
                scatters, gathers, combines = prep_qv(u)
                fill.plan(0, 9.5, scatters)
                fill.plan(9.5, 14.5, gathers)
                fill.plan(14.5, 38, prep_wo(u))
                fill.plan(38, 47, combines)

                finished = []

                def fence_k(v):
                    wd_buf[u >> 3, pl.ds(512, 16), pl.ds(0, 128)] = pltpu.bitcast(v, BF16)

                fill.plan(0.5, 30, [(functools.partial(fence_in, u), work) for work in
                                  slabs(WQ, xbuf, qv_slab(u, 0)) + slabs(WV, xbuf, qv_slab(u, 1))
                                  + slabs(WO, xbuf, 16 + 4 * u)]
                          + [(fence_k, work) for work in _Range(ranges, WK).matrix(
                              lambda r, c: wd_buf[1 - (u >> 1), _rows((u & 1) * 256 + r, 16), _chunk(c)],
                              256, 8, 256)])

                def outer(p):
                    def inner(p2):
                        lhs = [_words(hop, (p * NP + p2, j), u * 128, 128) for j in range(NJ)]
                        rhs = _cat(_load(wd_op, (p * NP + p2, c), 0, F // 4) for c in range(2))
                        return fill.dot(lhs, rhs)

                    return _quadrants(inner, (1, 4, 3, 2, 0, 5, 6))

                def done(q, vals):
                    for q2, d in enumerate(vals):
                        a, nq = _quarter(q, q2)
                        g = _silu(d).astype(BF16)
                        for s in range(2):
                            for c in range(2):
                                rows = _rows(((2 * u + s) * 4 + a) * Q, Q)
                                ybuf[2 * nq + c, rows, :] = _lanes(g, c)[s * Q:(s + 1) * Q]
                    for a2 in range(2):
                        rows = _rows((4 * u + 2 * (q // 2) + a2) * 128, 128)
                        parts = [_lanes(d * d, c) for d in vals[2 * a2:2 * a2 + 2] for c in range(2)]
                        if q ^ 1 in finished:
                            parts.append(energy[rows, :])
                        energy[rows, :] = functools.reduce(jnp.add, parts)
                    finished.append(q)

                _strassen(outer, done, (1, 3, 2, 4, 0, 6, 5))
                assert not fill.todo
                pl.when(u + 2 < NU)(lambda: _start(qv_copies(u + 2)))
                pl.when(u + 2 == NU)(lambda: x_copy(0).start())
                return carry

            wo_copy().wait()
            lax.fori_loop(0, NU, down_step, 0)

        pl.run_scoped(contract, pltpu.VMEM((2, (H + 1) * PITCH + 7, 128), U32),
                      pltpu.VMEM((16, 128 + 8, 128), U32), pltpu.VMEM((8, 17 * PITCH + 7, 128), F32))

    pl.run_scoped(ffn, pltpu.VMEM((NP * NP, NJ, S // 4, 128), BF16),
                  pltpu.VMEM((NP * NP, 2, F // 4, 128), BF16))

    def attention(q_s, obuf, *bufs):
        p_s, k_s, v_s, o_s, oop = bufs[:2], bufs[2:4], bufs[4:8], bufs[8:12], bufs[12:]

        def out_copy(t):
            rows = _rows(t * 2 * Q, 2 * Q)
            return pltpu.make_async_copy(obuf.at[rows], out_hbm.at[rows], sem_o.at[t])

        def tile(t, carry):
            x_copy(t).wait()
            fill = _Filler(t < 0, 20)
            tail, head = pl.ds(2 * Q, HALO), pl.ds(0, HALO)
            known = set()

            def fence(ref):
                def park(v):
                    ref[t >> 3, pl.ds(ref.shape[1] - 8, 8), :] = v
                return park

            def probs(a):
                pieces = []
                for r in range(0, 2 * Q, 8):
                    lg = [None] * WIN

                    def logits(c, r=r, lg=lg):
                        assert ("qk", a) in known
                        qv = q_s[c, pl.ds(a * 2 * Q + r, 8), :]
                        for w in range(WIN):
                            pr = qv * k_s[a][c, pl.ds(HALO + r - DIL * w, 8), :]
                            lg[w] = pr if c == 0 else lg[w] + pr

                    def softmax(r=r, lg=lg):
                        lg = [l + pltpu.roll(l, 64, 1) for l in lg]
                        lg = [l + pltpu.roll(l, 32, 1) for l in lg]
                        for w in range(WIN):
                            if a == 0 and r < DIL * w:
                                pos = t * 4 * Q + r + lax.broadcasted_iota(jnp.int32, (8, 128), 0)
                                lg[w] = jnp.where(pos >= DIL * w, lg[w], -1e9 / SCALE)
                        mx = functools.reduce(jnp.maximum, lg)
                        e = [jnp.exp2((l - mx) * (SCALE * LOG2E)) for l in lg]
                        inv = 1.0 / functools.reduce(jnp.add, e)
                        for w in range(WIN):
                            p_s[a][w, pl.ds(r, 8), :] = e[w] * inv
                        return pltpu.bitcast(p_s[a][t >> 3, pl.ds(r, 8), :], U32)

                    pieces += [(None if c % 3 else fence(k_s[a]), functools.partial(logits, c))
                               for c in range(8)]
                    pieces.append((None, softmax))
                return pieces

            def mix(q, first=0, last=2 * Q):
                def work(r, c):
                    assert ("v", q) in known and (r >= HALO or ("v", q % 2) in known)
                    prow = _rows(r + 8 * (t >> (3 + q % 2)), 8)
                    terms = [p_s[q // 2][w, prow, :] * v_s[q][c, pl.ds(HALO + r - DIL * w, 8), :]
                             for w in range(WIN)]
                    o_s[q ^ 1][c, pl.ds(r, 8), :] = functools.reduce(jnp.add, terms)

                return [(None if c % 2 else fence(v_s[q]), functools.partial(work, r, c))
                        for r in range(first, last, 8) for c in range(4)]

            def prep_o(ps):
                def work(i, c, p):
                    assert ("wo", p) not in known
                    op = _operands(LHS, p, lambda q, q2: o_s[q][
                        2 * (q2 % 2) + c, pl.ds((q2 // 2) * Q + i, 16), :])
                    for p2 in range(NP):
                        oop[p][p2, c, pl.ds(i, 16), :] = op(p2)

                return [(fence(o_s[_last_quadrant(p)]), functools.partial(work, i, c, p))
                        for p in ps for i in range(0, Q, 16) for c in range(2)]

            def widen(a):
                def work(r, c):
                    k_s[a][c, pl.ds(HALO + r, Q), :] = _load(kbuf, (c,), (4 * t + 2 * a) * Q + r, Q).astype(F32)

                def park(v):
                    kbuf[t >> 3, pl.ds(S, 16), :] = pltpu.bitcast(v, BF16)

                return [(park, functools.partial(work, r, c)) for r in (0, Q) for c in range(8)]

            def queries(a):
                def product(p):
                    lhs = [_words(aop, (half_index(a, b) + p, c), t * Q, Q) for b, c in QUADS]
                    return [fill.dot(lhs, _cat(_load(wq_op, (p, c), 0, 512) for c in range(4)), 4)]

                def done(q, val):
                    for c in range(4):
                        q_s[4 * (q % 2) + c, pl.ds((2 * a + q // 2) * Q, Q), :] = _lanes(val[0], c)

                _strassen(product, done, (1, 3, 4, 0, 2, 5, 6))
                known.add(("qk", a))

            def two_level(lhs, rhs, done, order, order2):
                def outer(p):
                    return _quadrants(lambda p2: fill.dot(
                        [lhs(p, p2, c) for c in range(2)],
                        _cat(_load(rhs, (p * NP + p2, c), 0, 256) for c in range(2))), order2)

                _strassen(outer, done, order)

            def values(q, vals):
                for q2, v in enumerate(vals):
                    for c in range(2):
                        v_s[q][2 * (q2 % 2) + c, pl.ds(HALO + (q2 // 2) * Q, Q), :] = _lanes(v, c)
                if q < 2:
                    for c in range(4):
                        first = jnp.broadcast_to(v_s[q][c, pl.ds(HALO, 1), :], (HALO, 128))
                        v_s[q][c, head, :] = jnp.where(t > 0, v_s[q][c, head, :], first)
                    v_s[q + 2][:, head, :] = v_s[q][:, tail, :]
                known.add(("v", q))

            def mixed(p, p2, c):
                known.add(("wo", p))
                return _words(oop[p], (p2, c), (t >> 3) * Q, Q)

            def output(q, vals):
                for q2, v in enumerate(vals):
                    a, nq = _quarter(q, q2)
                    for c in range(2):
                        col, start = 2 * (nq ^ 3) + c, (4 * t + a) * Q
                        g = _load(ybuf, (col,), start, Q).astype(F32)
                        xv = xbuf[4 * t + a, :, _chunk(col)].astype(F32)
                        obuf[_rows(start, Q), _chunk(col)] = (xv + _lanes(v, c) * g).astype(BF16)
                known.add(("out", q))
                if ("out", q ^ 1) in known:
                    out_copy(2 * t + q // 2).start()

            k_s[0][:, head, :] = jnp.where(t > 0, k_s[1][:, tail, :], 0.0)
            for q in range(2):
                v_s[q][:, head, :] = v_s[q + 2][:, tail, :]
            fill.plan(0, 18, widen(0) + widen(1))
            queries(0)
            assert not fill.todo
            k_s[1][:, head, :] = k_s[0][:, tail, :]
            fill.plan(0, 27, probs(0))
            fill.plan(28, 55, probs(1))
            fill.plan(55, 67, mix(1) + prep_o((2,)))
            fill.plan(67, 79, mix(2, HALO) + mix(2, 0, HALO) + prep_o((3, 0)))
            fill.plan(79, 89, mix(0) + prep_o((4, 6)))
            fill.plan(89, 102, mix(3) + prep_o((1, 5)))
            queries(1)
            two_level(lambda p, p2, c: _words(aop, (p * NP + p2, c), t * Q, Q), wv_op, values,
                      (2, 4, 3, 1, 0, 6, 5), (4, 2, 3, 1, 0, 5, 6))
            two_level(mixed, wo_op, output, (2, 3, 0, 4, 6, 1, 5), (1, 3, 2, 4, 0, 6, 5))
            assert not fill.todo
            return carry

        _start(x_copy(t) for t in range(1, NT))
        lax.fori_loop(0, NT, tile, 0)
        seen = _Range(ranges, FFN)
        seen.add_rows([energy[...]])
        seen.save()
        failed = []
        for n in range(ranges.shape[1]):
            lo, hi = ranges[0, n], ranges[1, n]
            least = jnp.min(jnp.min(lo, axis=0, keepdims=True), axis=1, keepdims=True)
            balanced = (lo > 0.0) & (hi < jnp.inf) & (hi <= BALANCE * least)
            failed.append(jnp.where(balanced, 0.0, 1.0))
        unbalanced = jnp.max(functools.reduce(jnp.maximum, failed)) > 0.0
        _wait(out_copy(t) for t in range(2 * NT))
        return unbalanced

    unbalanced = pl.run_scoped(
        attention,
        pltpu.VMEM((8, 4 * Q, 128), F32),
        pltpu.VMEM((S, D), BF16),
        *[pltpu.VMEM((WIN, 2 * Q, 128), F32)] * 2,
        *[pltpu.VMEM((8, HALO + 2 * Q + 8, 128), F32)] * 2,
        *[pltpu.VMEM((4, HALO + 2 * Q + 8, 128), F32)] * 4,
        *[pltpu.VMEM((4, 2 * Q + 8, 128), F32)] * 4,
        *[pltpu.VMEM((NP, 2, Q, 128), BF16)] * NP,
    )

    def plain(xn_s, w_s, wo_s, wd_s, qkv_s, o_s, h_s):

        def repeat(n, body):
            def step(i, carry):
                body(i)
                return carry

            lax.fori_loop(0, n, step, 0)

        def fetch(src, dst):
            copy = pltpu.make_async_copy(src, dst, sem_w.at[0])
            copy.start()
            copy.wait()

        def dot(a, b):
            return jnp.dot(a, b, preferred_element_type=F32)

        def normalize(i):
            xv = xbuf[i >> 2, _rows((i & 3) * 16, 16), :].astype(F32)
            xc = xv - jnp.mean(xv, axis=-1, keepdims=True)
            var = jnp.mean(xc * xc, axis=-1, keepdims=True)
            xn_s[_rows(i * 16, 16), :] = (xc * lax.rsqrt(var + 1e-5)).astype(BF16)

        def project(m):
            def rows(i):
                first = pl.multiple_of(HALO + i * 32, 16)
                qkv_s[m, pl.ds(first, 32), :] = dot(xn_s[_rows(i * 32, 32), :], w_s[m])

            repeat(S // 32, rows)

        def attend(c):
            def rows(i):
                first = pl.multiple_of(i * 16, 16)
                pos = i * 16 + lax.broadcasted_iota(jnp.int32, (16, 128), 0)
                k, v = (qkv_s[m, pl.ds(first, HALO + 16), :] for m in (1, 2))
                qv = qkv_s[0, pl.ds(first + HALO, 16), :]
                pr = jnp.concatenate([qv * k[HALO - DIL * w:HALO - DIL * w + 16]
                                      for w in range(WIN)], axis=0)
                head = [lax.broadcasted_iota(jnp.int32, (128, 128), d) >> 5 for d in (0, 1)]
                same = jnp.where(head[0] == head[1], 1.0, 0.0).astype(BF16)
                top = pr.astype(BF16)
                lg = (dot(top, same) + dot((pr - top.astype(F32)).astype(BF16), same)) * SCALE
                lg = [jnp.where(pos >= DIL * w, lg[16 * w:16 * w + 16], -1e9) for w in range(WIN)]
                mx = functools.reduce(jnp.maximum, lg)
                e = [jnp.exp(l - mx) for l in lg]
                o = functools.reduce(jnp.add, [e[w] * v[HALO - DIL * w:HALO - DIL * w + 16]
                                               for w in range(WIN)])
                o_s[c, pl.ds(first, 16), :] = (o / functools.reduce(jnp.add, e)).astype(BF16)

            for m in (1, 2):
                qkv_s[m, pl.ds(0, HALO), :] = jnp.broadcast_to(
                    qkv_s[m, pl.ds(HALO, 1), :], (HALO, 128))
            repeat(S // 16, rows)

        def activate(f):
            def rows(i):
                g, u = (qkv_s[m, _rows(HALO + i * 16, 16), :] for m in (0, 1))
                h_s[f, _rows(i * 16, 16), :] = (_gelu(g) * u).astype(BF16)

            repeat(S // 16, rows)

        def columns(n):
            @pl.when(n < 8)
            def _():
                repeat(12, lambda i: fetch(wqkv_hbm.at[i & 3, :, _chunk(8 * (i >> 2) + n)],
                                           w_s.at[i >> 2, _rows((i & 3) * 256, 256)]))

            @pl.when(n >= 8)
            def _():
                fetch(wg_hbm.at[:, _chunk(n - 8)], w_s.at[0])
                fetch(wu_hbm.at[:, _chunk(n - 8)], w_s.at[1])

            repeat(jnp.where(n < 8, 3, 2), project)
            pl.when(n < 8)(lambda: attend(n))
            pl.when(n >= 8)(lambda: activate(n - 8))

        def finish(c):
            def rows(i):
                r = _rows(i * 16, 16)
                d = lax.fori_loop(0, NJ, lambda j, d: d + dot(
                    _cat(h_s[4 * j + n, r, :] for n in range(4)), wd_s[_rows(j * 512, 512), :]),
                    jnp.zeros((16, 128), F32))
                sv = dot(_cat(o_s[n, r, :] for n in range(8)),
                         jnp.concatenate([wo_s[n] for n in range(16)], axis=0))
                xv = wo_s[16 + (i >> 2), _rows((i & 3) * 16, 16), :].astype(F32)
                ybuf[c, r, :] = (xv + sv * _silu(d)).astype(BF16)

            fetch(wo_hbm.at[:, :, _chunk(c)], wo_s.at[pl.ds(0, 16)])
            fetch(x_hbm.at[:, :, _chunk(c)], wo_s.at[pl.ds(16, S // Q)])
            fetch(wd_hbm.at[:, _chunk(c)], wd_s)
            repeat(S // 16, rows)
            fetch(ybuf.at[c], out_hbm.at[:, _chunk(c)])

        repeat(S // 16, normalize)
        repeat(8 + F // 128, columns)
        repeat(8, finish)

    @pl.when(unbalanced)
    def _():
        pl.run_scoped(plain, pltpu.VMEM((S, D), BF16), pltpu.VMEM((3, D, 128), BF16),
                      pltpu.VMEM((16 + S // Q, Q, 128), BF16), pltpu.VMEM((F, 128), BF16),
                      pltpu.VMEM((3, HALO + S, 128), F32), pltpu.VMEM((8, S, 128), BF16),
                      pltpu.VMEM((F // 128, S, 128), BF16))


@jax.jit
def pallas_recurrent_scan__sliding_local_dilated__geglu_ffn__prompt_kernel(
    A_x: jax.Array,
    A_wqkv: jax.Array,
    A_wo: jax.Array,
    B_x: jax.Array,
    B_w_gate: jax.Array,
    B_w_up: jax.Array,
    B_w_down: jax.Array,
):
    del B_x
    in_hbm = pl.BlockSpec(memory_space=pl.ANY)
    out = pl.pallas_call(
        _kernel,
        out_shape=jax.ShapeDtypeStruct((S, D), BF16),
        in_specs=[in_hbm] * 6,
        out_specs=in_hbm,
        scratch_shapes=[
            pltpu.VMEM((S // Q + 1, Q, D), BF16),
            pltpu.VMEM((8, S, 128), BF16),
            pltpu.VMEM((8, S + 16, 128), BF16),
            pltpu.VMEM((2, 512 + 16, D), BF16),
            pltpu.VMEM((NP * (NP + 2), 2, S // 4, 128), BF16),
            pltpu.VMEM((NP, 4, D // 4, 128), U32),
            pltpu.VMEM((NP * NP, 2, D // 8, 128), U32),
            pltpu.VMEM((NP * NP, 2, D // 8, 128), U32),
            pltpu.VMEM((2, 9, 8, 128), F32),
            pltpu.VMEM((S, 128), F32),
            pltpu.SemaphoreType.DMA((NT,)),
            pltpu.SemaphoreType.DMA((4,)),
            pltpu.SemaphoreType.DMA((2,)),
            pltpu.SemaphoreType.DMA((3,)),
            pltpu.SemaphoreType.DMA((2 * NT,)),
        ],
        compiler_params=pltpu.CompilerParams(vmem_limit_bytes=127 * 2**20),
        name="fused_block",
    )(A_x.reshape(S // Q, Q, D), A_wqkv.reshape(4, D // 4, 3 * D),
      A_wo.reshape(D // Q, Q, D), B_w_gate, B_w_up, B_w_down)
    return out.reshape(A_x.shape)
```

```python
import functools

import jax
import jax.numpy as jnp
from jax import lax
import jax.experimental.pallas as pl
import jax.experimental.pallas.tpu as pltpu

F32 = jnp.float32
BF16 = jnp.bfloat16
U32 = jnp.uint32

S, D, F = 2048, 1024, 3584
H, DH, WIN, DIL = 32, 32, 8, 2
SCALE = DH ** -0.5
LOG2E = 1.4426950408889634
HALO = 16
PITCH = DH + 1
Q = 64
NT = S // (4 * Q)
NJ = F // 512
NU = S // 512

LHS = ((1, 0, 0, 1), (0, 0, 1, 1), (1, 0, 0, 0), (0, 0, 0, 1),
       (1, 1, 0, 0), (-1, 0, 1, 0), (0, 1, 0, -1))
RHS = ((1, 0, 0, 1), (1, 0, 0, 0), (0, 1, 0, -1), (-1, 0, 1, 0),
       (0, 0, 0, 1), (1, 1, 0, 0), (0, 0, 1, 1))
OUT = ((1, 0, 0, 1), (0, 0, 1, -1), (0, 1, 0, 1), (1, 0, 1, 0),
       (-1, 1, 0, 0), (0, 0, 0, 1), (1, 0, 0, 0))
NP = 7
QUADS = ((0, 0), (0, 1), (1, 0), (1, 1))
GROUPS = ((0, 1), (2, 4), (3,), (5,), (6,))
XN, WK, WG, WU, WD, WQ, WV, WO, FFN = range(9)
BALANCE = 6.0


def _lin(coef, quad):
    idx = sorted((q for q, c in enumerate(coef) if c), key=lambda q: -coef[q])
    if len(idx) == 1:
        return quad(idx[0])
    a, b = quad(idx[0]).astype(F32), quad(idx[1]).astype(F32)
    return a + b if coef[idx[1]] > 0 else a - b


def _operands(coefs, p, block):
    w = [_lin(coefs[p], lambda q: block(q, q2)) for q2 in range(4)]
    return lambda p2: _lin(coefs[p2], lambda q2: w[q2]).astype(BF16)


def _quarter(q, q2):
    return 2 * (q // 2) + q2 // 2, 2 * (q % 2) + q2 % 2


def _last_quadrant(p):
    return max(q for q in range(4) if LHS[p][q])


def _strassen(product, done, order):
    acc = [None] * 4
    left = [sum(1 for p in range(NP) if OUT[p][q]) for q in range(4)]
    for p in order:
        m = product(p)
        for q in range(4):
            s = OUT[p][q]
            if s == 0:
                continue
            if acc[q] is None:
                acc[q] = (s, m)
            else:
                s0, c = acc[q]
                assert s > 0 or s0 > 0
                acc[q] = (1, [x + y if s == s0 else (x - y if s > 0 else y - x)
                              for x, y in zip(m, c)])
            left[q] -= 1
            if left[q] == 0:
                done(q, acc[q][1])


def _quadrants(product, order):
    out = [None] * 4

    def done(q, val):
        out[q] = val[0]

    _strassen(lambda p: [product(p)], done, order)
    return out


def _cat(xs):
    return jnp.concatenate(list(xs), axis=1)


def _lanes(v, c):
    return v[:, c * 128:(c + 1) * 128]


def _gelu(g):
    half = 0.5 * g
    t = jnp.tanh(g * (0.7978845608028654 + 0.7978845608028654 * 0.044715 * (g * g)))
    return half * t + half


def _silu(d):
    half = 0.5 * d
    return half * jnp.tanh(half) + half


def _rows(start, size):
    return pl.ds(start if isinstance(start, int) else pl.multiple_of(start, size), size)


def _chunk(c):
    return _rows(c * 128, 128)


def _words(ref, lead, start, size):
    if ref.dtype == U32:
        return ref[(*lead, _rows(start >> 1, size // 2))]
    return pltpu.bitcast(ref[(*lead, _rows(start, size))], U32)


def _load(ref, lead, start, size):
    return pltpu.bitcast(_words(ref, lead, start, size), BF16)


def _store(ref, lead, start, val):
    size = val.shape[0]
    if ref.dtype == U32:
        ref[(*lead, _rows(start >> 1, size // 2))] = pltpu.bitcast(val, U32)
    else:
        ref[(*lead, _rows(start, size))] = val


class _Filler:
    def __init__(self, never, lag):
        self.never, self.lag = never, lag
        self.todo, self.marks, self.pos = [], [], 0

    def plan(self, first, last, pieces):
        self.todo += [(self.pos + first + i * (last - first) / len(pieces), piece)
                      for i, piece in enumerate(pieces)]
        self.todo.sort(key=lambda t: t[0])

    def dot(self, words, b, span=1):
        rows = [words[0][r:r + 8] for r in range(0, words[0].shape[0], 8)]
        while self.marks and self.marks[0][0] < self.pos + span:
            when, mark = self.marks.pop(0)
            r = int(max(when - self.pos, 0) / span * len(rows))
            rows[r] = jnp.where(self.never, mark, rows[r])
        a = _cat(pltpu.bitcast(x, BF16) for x in [jnp.concatenate(rows, axis=0)] + words[1:])
        m = jnp.dot(a, b, preferred_element_type=F32)
        nr, nc = m.shape[0] // 8, m.shape[1] // 128
        while self.todo and self.todo[0][0] < self.pos + span:
            when, (fence, work) = self.todo.pop(0)
            i = int(max(when - self.pos, 0) / span * nr * nc)
            r, c = divmod(i, nc) if a.shape[1] == 256 else divmod(i, nr)[::-1]
            if fence is not None:
                fence(_lanes(m, c)[8 * r:8 * r + 8])
            mark = work()
            if mark is not None:
                self.marks.append((when + self.lag, mark))
        self.pos += span
        return m


def _range_rows(slot):
    return pl.ds(S + 16 * slot, 8), pl.ds(S + 16 * slot + 8, 8)


class _Range:
    def __init__(self, ref, slot):
        self.ref, self.slot, self.lo, self.hi = ref, slot, None, None

    def add(self, v):
        v = jnp.broadcast_to(v, (max(v.shape[0], 8), 128))
        for r in range(0, v.shape[0], 8):
            x = v[r:r + 8]
            self.lo = x if self.lo is None else jnp.minimum(self.lo, x)
            self.hi = x if self.hi is None else jnp.maximum(self.hi, x)

    def add_rows(self, squares):
        total = jnp.sum(functools.reduce(jnp.add, squares), axis=-1, keepdims=True)
        self.add(total * (1.0 / (128 * len(squares))))

    def save(self):
        lo, hi = _range_rows(self.slot)
        self.ref[lo, :] = jnp.minimum(self.ref[lo, :], self.lo)
        self.ref[hi, :] = jnp.maximum(self.ref[hi, :], self.hi)
        self.lo = self.hi = None

    def matrix(self, load, rows, chunks, span):
        cols = [None] * chunks

        def work(r):
            w = [load(r, c).astype(F32) for c in range(chunks)]
            squares = [x * x for x in w]
            self.add_rows(squares)
            for c, x in enumerate(squares):
                cols[c] = x[:8] + x[8:] if r % span == 0 else cols[c] + x[:8] + x[8:]
            if (r + 16) % span == 0:
                for x in cols:
                    self.add(jnp.sum(x, axis=0, keepdims=True) * (1.0 / span))
                self.save()
            return pltpu.bitcast(functools.reduce(jnp.add, cols), U32)

        return [functools.partial(work, r) for r in range(0, rows, 16)]


def _start(copies):
    for copy in copies:
        copy.start()


def _wait(copies):
    for copy in copies:
        copy.wait()


def _kernel(x_hbm, wqkv_hbm, wo_hbm, wg_hbm, wu_hbm, wd_hbm, out_hbm,
            xbuf, ybuf, kbuf, wd_buf, aop, wq_op, wv_op, wo_op, energy,
            sem_x, sem_k, sem_u, sem_w, sem_o):

    def x_copy(t):
        rows = pl.ds(4 * t, 4)
        return pltpu.make_async_copy(x_hbm.at[rows], xbuf.at[rows], sem_x.at[t])

    def half_index(a, b):
        return {(0, 0): 2, (1, 1): 3, (0, 1): 7, (1, 0): 8}[a, b] * NP

    def up_copies(j, which=range(9)):
        def ends(n):
            if n == 8:
                return wd_hbm.at[_rows(j * 512, 512)], wd_buf.at[j & 1, pl.ds(0, 512)]
            return ((wg_hbm, wu_hbm)[n % 2].at[:, _chunk(4 * j + n // 2)],
                    ybuf.at[(j & 1) * 4 + n // 2, pl.ds((n % 2) * D, D)])

        return [pltpu.make_async_copy(*ends(n), sem_u.at[j & 1]) for n in which]

    def slabs(slot, src, first):
        return _Range(energy, slot).matrix(
            lambda r, c: src[first + r // Q, pl.ds(r % Q, 16), _chunk(c)], 4 * Q, 8, 4 * Q)

    def scatter(src, slab, tmp_u, m, c):
        w = [src[slab + kq, :, _chunk(c)] for kq in range(4)]
        w = pltpu.bitcast(jnp.concatenate(w, axis=0), U32).T
        for h in range(4):
            tmp_u[m, pl.ds((4 * c + h) * PITCH, DH), :] = w[h * DH:(h + 1) * DH]

    def gather(tmp_u, tmp_v, m, c):
        w = [tmp_u[m, pl.ds(4 * c + d, H, stride=PITCH), :] for d in range(4)]
        tmp_v[8 * m + c, pl.ds(0, 128), :] = jnp.concatenate(w, axis=0).T

    def one_level(tmp_v, dst, u, c, b):
        for i in range(0, Q, 16):
            for p in range(NP):
                op = _lin(RHS[p], lambda q: _load(
                    tmp_v, (c + 4 * (q % 2),), (2 * b + q // 2) * Q + i, 16))
                _store(dst, (p, c), b * 256 + u * Q + i, op.astype(BF16))
        return _words(dst, (u >> 3, 0), 0, 16)

    def keys(wk_buf, wk_op, tmp_u, tmp_v, xn_s, sum_s, mean_s, sq_s, rstd_s):

        def k_copy(u):
            return pltpu.make_async_copy(wqkv_hbm.at[:, _rows(u * Q, Q), pl.ds(D, D)],
                                         wk_buf.at[pl.ds(4 * u, 4)], sem_k.at[u])

        def layernorm(t, strips=range(0, Q, 16)):
            seen = _Range(energy, XN)

            def x_rows(i, a, c):
                return xbuf[4 * t + a, _rows(i, 16), _chunk(c)].astype(F32)

            def lane_mean(v):
                return jnp.broadcast_to(jnp.sum(v, axis=-1, keepdims=True) * (1.0 / D), v.shape)

            def total(i, a):
                xs = [x_rows(i, a, c) for c in range(8)]
                sum_s[a, _rows(i, 16), :] = functools.reduce(jnp.add, xs)

            def mean(i, a):
                mean_s[a, _rows(i, 16), :] = lane_mean(sum_s[a, _rows(i, 16), :])

            def squares(i, a):
                xc = [x_rows(i, a, c) - mean_s[a, _rows(i, 16), :] for c in range(8)]
                sq_s[a, _rows(i, 16), :] = functools.reduce(jnp.add, [v * v for v in xc])

            def rstd(i, a):
                var = lane_mean(sq_s[a, _rows(i, 16), :])
                r = lax.rsqrt(var + 1e-5)
                rstd_s[a, _rows(i, 16), :] = r
                seen.add(var * r * r)
                if a == 3:
                    seen.save()

            def scale(i, a):
                rows = _rows(i, 16)
                for c in range(8):
                    xn = (x_rows(i, a, c) - mean_s[a, rows, :]) * rstd_s[a, rows, :]
                    xn_s[c, _rows(a * Q + i, 16), :] = xn

            def operands(i, c, p):
                def block(q, q2):
                    a, k = _quarter(q, q2)
                    return xn_s[2 * k + c, _rows(a * Q + i, 16), :]

                op = _operands(LHS + ((0, 1, 0, 0), (0, 0, 1, 0)), p, block)
                for p2 in range(NP):
                    aop[p * NP + p2, c, _rows(t * Q + i, 16), :] = op(p2)

            return [[functools.partial(f, i, a) for i in strips for a in range(4)]
                    for f in (total, mean, squares, rstd, scale)] + [
                [functools.partial(operands, i, c, p)
                 for i in strips for c in range(2) for p in range(NP + 2)]]

        def run(stages):
            for works in stages:
                for work in works:
                    work()

        def prep_k(u, carry):
            k_copy(u).wait()
            x_copy(u + 1).start()
            run(layernorm(0, [16 * u])[5:])
            tmp_u[u >> 3, pl.ds(H * PITCH, 8), :] = _words(aop, (u >> 3, 0), 0, 16)
            for c in range(8):
                scatter(wk_buf, 4 * u, tmp_u, 0, c)
            for c in (0, 4, 1, 5, 2, 6, 3, 7):
                gather(tmp_u, tmp_v, 0, c)
            for c in range(4):
                for b in range(2):
                    one_level(tmp_v, wk_op, u, c, b)
            return carry

        def key_tile(t, carry):
            pl.when(t + 1 < NT)(lambda: x_copy(t + 1).wait())

            def fence(v):
                xbuf[S // Q - (t >> 3), pl.ds(0, 16), pl.ds(0, 128)] = pltpu.bitcast(v, BF16)

            def fence_xn(v):
                xn_s[t >> 3, pl.ds(4 * Q, 8), :] = v

            lhs = [[jnp.concatenate([_words(aop, (half_index(a, b) + p, c), t * Q, Q)
                                     for a in range(2)], axis=0) for b, c in QUADS]
                   for p in range(NP)]
            fill = _Filler(t < 0, 0)
            stages = layernorm(jnp.minimum(t + 1, NT - 1))
            fences = (fence, None, fence, None, fence, fence_xn)
            windows = ((0, 0.45), (0.45, 0.45), (0.75, 1.95), (1.95, 1.95), (1.95, 3.2), (3.35, 6.9))
            for works, window, f in zip(stages, windows, fences):
                fill.plan(*window, [(f, work) for work in works])

            def product(p):
                return [fill.dot(lhs[p], _cat(_load(wk_op, (p, c), 0, 512) for c in range(4)))]

            def done(q, val):
                k = val[0].astype(BF16)
                for a in range(2):
                    for c in range(4):
                        rows = _rows((4 * t + 2 * a + q // 2) * Q, Q)
                        kbuf[4 * (q % 2) + c, rows, :] = _lanes(k, c)[a * Q:(a + 1) * Q]

            _strassen(product, done, (1, 3, 4, 2, 0, 5, 6))
            assert not fill.todo
            return carry

        _start([x_copy(0)] + [k_copy(u) for u in range(3)])
        for lo, hi in map(_range_rows, range(9)):
            energy[lo, :] = jnp.full((8, 128), jnp.inf, F32)
            energy[hi, :] = jnp.zeros((8, 128), F32)
        x_copy(0).wait()
        k_copy(3).start()
        run(layernorm(0)[:5])
        lax.fori_loop(0, 4, prep_k, 0)
        _start([x_copy(t) for t in range(5, NT)] + up_copies(0) + up_copies(1))
        lax.fori_loop(0, NT, key_tile, 0)

    pl.run_scoped(keys, pltpu.VMEM((16, Q, D), BF16), pltpu.VMEM((NP, 4, D // 2, 128), BF16),
                  pltpu.VMEM((1, (H + 1) * PITCH + 31, 128), U32), pltpu.VMEM((8, 128 + 8, 128), U32),
                  pltpu.VMEM((8, 4 * Q + 8, 128), F32), *[pltpu.VMEM((4, Q, 128), F32)] * 4)

    def ffn(hop, wd_op):

        def qv_slab(u, m):
            return ((u & 1) * 2 + m) * 4

        def qv_copies(u):
            return [pltpu.make_async_copy(wqkv_hbm.at[:, _rows(u * Q, Q), pl.ds(2 * m * D, D)],
                                          xbuf.at[pl.ds(qv_slab(u, m), 4)], sem_w.at[u & 1])
                    for m in range(2)]

        def wo_copy():
            return pltpu.make_async_copy(wo_hbm, xbuf.at[pl.ds(16, 16)], sem_w.at[2])

        def wk_copies(slot):
            return [pltpu.make_async_copy(wqkv_hbm.at[2 * slot + n, :, pl.ds(D, D)],
                                          wd_buf.at[slot, pl.ds(256 * n, 256)], sem_u.at[slot])
                    for n in range(2)]

        def expand(*h_s):
            _start(qv_copies(0) + qv_copies(1) + [wo_copy()])

            def prep_wd(j):
                def fence(v):
                    wd_buf[j >> 3, pl.ds(512, 16), pl.ds(0, 128)] = pltpu.bitcast(v, BF16)

                def work(i, c, ps):
                    def block(q, q2):
                        kq, nq = _quarter(q, q2)
                        return wd_buf[j & 1, pl.ds((kq ^ 2) * 128 + i, 16), _chunk(2 * nq + c)]

                    for p in ps:
                        op = _operands(RHS, p, block)
                        for p2 in range(NP):
                            _store(wd_op, (p * NP + p2, c), j * 128 + i, op(p2))
                    return _words(wd_op, (j >> 3, 0), 0, 16)

                return [(fence, functools.partial(work, i, c, ps))
                        for i in range(0, 128, 16) for c in range(2) for ps in GROUPS]

            def prep_h(j, ps, ready):
                def fence(p, v):
                    h_s[_last_quadrant(p)][j >> 3, pl.ds(512, 8), :] = v

                def work(i, p):
                    assert ready(p)
                    op = _operands(LHS, p, lambda q, q2: h_s[q][q2, pl.ds(i, 16), :])
                    for p2 in range(NP):
                        hop[p * NP + p2, j, pl.ds(i, 16), :] = op(p2)
                    return _words(hop, (j >> 3, 0), 0, 16)

                return [(functools.partial(fence, p), functools.partial(work, i, p))
                        for i in range(0, 512, 16) for p in ps]

            def balance_up(j, slot, top):
                parked = []

                def fence(v):
                    parked.append(pltpu.bitcast(v, U32))

                def load(r, c):
                    w = _words(ybuf, ((j & 1) * 4 + c + (j >> 3),), top + r, 16)
                    return pltpu.bitcast(jnp.where(j < 0, parked[-1], w), BF16)

                return [(fence, work) for work in _Range(energy, slot).matrix(load, D, 4, D)]

            def up_step(j, carry):
                _wait(up_copies(j))
                written = []

                def fresh(p):
                    return all(q in written for q in range(4) if LHS[p][q])

                fill = _Filler(j < 0, 0.75)
                pieces = prep_wd(j)
                fill.plan(14.6, 21.5, pieces[:45])
                fill.plan(25.5, 37, pieces[45:])
                fill.plan(1.1, 5.5, prep_h(jnp.maximum(j - 1, 0), (4, 6), lambda p: not written))
                fill.plan(14.3, 22, prep_h(j, (3,), fresh))
                fill.plan(29.2, 36, prep_h(j, (0, 2), fresh))
                fill.plan(42, 47, prep_h(j, (1, 5), fresh))
                fill.plan(0.3, 10, balance_up(j, WG, 0))
                fill.plan(14, 24, balance_up(j, WU, D))
                fill.plan(28, 40, [(pieces[0][0], work) for work in _Range(energy, WD).matrix(
                    lambda r, c: wd_buf[j & 1, pl.ds(r % 512, 16), _chunk(4 * (r // 512) + c)],
                    D, 4, 512)])

                def block(q, q2):
                    kq, cq = _quarter(q, q2)
                    return _cat(_load(ybuf, ((j & 1) * 4 + cq,), r + kq * 256, 256) for r in (0, D))

                def outer(p):
                    rhs = _operands(RHS, p, block)

                    def inner(p2):
                        lhs = [_words(aop, (p * NP + p2, c), 0, 512) for c in range(2)]
                        return fill.dot(lhs, rhs(p2))

                    return _quadrants(inner, (4, 2, 1, 3, 0, 6, 5))

                def done(q, vals):
                    for q2, v in enumerate(vals):
                        h_s[q ^ 1][q2, pl.ds(0, 512), :] = _gelu(_lanes(v, 0)) * _lanes(v, 1)
                    written.append(q ^ 1)

                _strassen(outer, done, (1, 3, 4, 2, 0, 5, 6))
                for n in range(0, 9, 3):
                    pl.when(j + 2 < NJ)(lambda: _start(up_copies(j + 2, range(n, n + 3))))
                pl.when(j + 2 >= NJ)(lambda: _start(wk_copies(j & 1)))
                assert not fill.todo
                return carry

            hop[0, 0, pl.ds(0, 16), :] = jnp.zeros((16, 128), BF16)
            lax.fori_loop(0, NJ, up_step, 0)
            for _, work in prep_h(NJ - 1, (4, 6), lambda p: True):
                work()

        pl.run_scoped(expand, *[pltpu.VMEM((4, 512 + 8, 128), F32)] * 4)

        def contract(tmp_u, tmp_v, tmp_f):

            def fence_in(u, v):
                xbuf[S // Q - (u >> 3), pl.ds(0, 16), pl.ds(0, 128)] = pltpu.bitcast(v, BF16)

            def prep_qv(u):
                def fence_u(v):
                    tmp_u[u >> 3, pl.ds(H * PITCH, 8), :] = pltpu.bitcast(v, U32)

                def fence_v(v):
                    tmp_v[u >> 3, pl.ds(128, 8), :] = pltpu.bitcast(v, U32)

                def two_level(c, i, ps):
                    def block(q, q2):
                        kq, nq = _quarter(q, q2)
                        return _load(tmp_v, (8 + 2 * nq + c,), kq * Q + i, 16)

                    for p in ps:
                        op = _operands(RHS, p, block)
                        for p2 in range(NP):
                            _store(wv_op, (p * NP + p2, c), u * Q + i, op(p2))
                    return _words(wv_op, (u >> 3, 0), 0, 16)

                every = [(m, c) for m in range(2) for c in range(8)]
                return ([(functools.partial(fence_in, u),
                          functools.partial(scatter, xbuf, qv_slab(u, m), tmp_u, m, c)) for m, c in every],
                        [(fence_u, functools.partial(gather, tmp_u, tmp_v, m, c)) for m, c in every],
                        [(fence_v, functools.partial(one_level, tmp_v, wq_op, u, c, b))
                         for c in range(4) for b in range(2)]
                        + [(fence_v, functools.partial(two_level, c, i, ps))
                           for c in range(2) for i in range(0, Q, 16) for ps in GROUPS])

            def prep_wo(u):
                def fence_f(v):
                    tmp_f[u >> 3, pl.ds(16 * PITCH, 8), :] = v

                def spread(h, cs):
                    for c in cs:
                        w = xbuf[16 + (u & 1) * 8 + h // 2, pl.ds((h % 2) * DH, DH), _chunk(c)]
                        tmp_f[c, pl.ds(h * PITCH, DH), :] = w.astype(F32)
                    return pltpu.bitcast(tmp_f[u >> 3, pl.ds(0, 8), :], U32)

                def collect(d, c, ps):
                    d = (u >> 1) * 4 + d

                    def block(q, q2):
                        kq, nq = _quarter(q, q2)
                        return tmp_f[2 * (nq ^ 3) + c, pl.ds((kq ^ 2) * 8 + d, 16, stride=PITCH), :]

                    for p in ps:
                        op = _operands(RHS, p, block)
                        for p2 in range(NP):
                            _store(wo_op, (p * NP + p2, c), d * H + (u & 1) * 16, op(p2))
                    return _words(wo_op, (u >> 3, 0), 0, 16)

                return ([(functools.partial(fence_in, u), functools.partial(spread, h, cs))
                         for h in range(16) for cs in (range(4), range(4, 8))]
                        + [(fence_f, functools.partial(collect, d, c, ps))
                           for d in range(4) for c in range(2) for ps in GROUPS])

            def down_step(u, carry):
                _wait(qv_copies(u))
                pl.when((u & 1) == 0)(lambda: _wait(wk_copies(1 - (u >> 1))))
                fill = _Filler(u < 0, 2.75)
                scatters, gathers, combines = prep_qv(u)
                fill.plan(0, 9.5, scatters)
                fill.plan(9.5, 14.5, gathers)
                fill.plan(14.5, 38, prep_wo(u))
                fill.plan(38, 47, combines)

                finished = []

                def fence_k(v):
                    wd_buf[u >> 3, pl.ds(512, 16), pl.ds(0, 128)] = pltpu.bitcast(v, BF16)

                fill.plan(0.5, 30, [(functools.partial(fence_in, u), work) for work in
                                  slabs(WQ, xbuf, qv_slab(u, 0)) + slabs(WV, xbuf, qv_slab(u, 1))
                                  + slabs(WO, xbuf, 16 + 4 * u)]
                          + [(fence_k, work) for work in _Range(energy, WK).matrix(
                              lambda r, c: wd_buf[1 - (u >> 1), _rows((u & 1) * 256 + r, 16), _chunk(c)],
                              256, 8, 256)])

                def outer(p):
                    def inner(p2):
                        lhs = [_words(hop, (p * NP + p2, j), u * 128, 128) for j in range(NJ)]
                        rhs = _cat(_load(wd_op, (p * NP + p2, c), 0, F // 4) for c in range(2))
                        return fill.dot(lhs, rhs)

                    return _quadrants(inner, (1, 4, 3, 2, 0, 5, 6))

                def done(q, vals):
                    for q2, d in enumerate(vals):
                        a, nq = _quarter(q, q2)
                        g = _silu(d).astype(BF16)
                        for s in range(2):
                            for c in range(2):
                                rows = _rows(((2 * u + s) * 4 + a) * Q, Q)
                                ybuf[2 * nq + c, rows, :] = _lanes(g, c)[s * Q:(s + 1) * Q]
                    for a2 in range(2):
                        rows = _rows((4 * u + 2 * (q // 2) + a2) * 128, 128)
                        parts = [_lanes(d * d, c) for d in vals[2 * a2:2 * a2 + 2] for c in range(2)]
                        if q ^ 1 in finished:
                            parts.append(energy[rows, :])
                        energy[rows, :] = functools.reduce(jnp.add, parts)
                    finished.append(q)

                _strassen(outer, done, (1, 3, 2, 4, 0, 6, 5))
                assert not fill.todo
                pl.when(u + 2 < NU)(lambda: _start(qv_copies(u + 2)))
                pl.when(u + 2 == NU)(lambda: x_copy(0).start())
                return carry

            wo_copy().wait()
            lax.fori_loop(0, NU, down_step, 0)

        pl.run_scoped(contract, pltpu.VMEM((2, (H + 1) * PITCH + 31, 128), U32),
                      pltpu.VMEM((16, 128 + 8, 128), U32), pltpu.VMEM((8, 17 * PITCH + 7, 128), F32))

    pl.run_scoped(ffn, pltpu.VMEM((NP * NP, NJ, S // 4, 128), BF16),
                  pltpu.VMEM((NP * NP, 2, F // 4, 128), BF16))

    def attention(q_s, obuf, *bufs):
        p_s, k_s, v_s, o_s, oop = bufs[:2], bufs[2:4], bufs[4:8], bufs[8:12], bufs[12:]

        def out_copy(t):
            rows = _rows(t * 2 * Q, 2 * Q)
            return pltpu.make_async_copy(obuf.at[rows], out_hbm.at[rows], sem_o.at[t])

        def tile(t, carry):
            x_copy(t).wait()
            fill = _Filler(t < 0, 20)
            tail, head = pl.ds(2 * Q, HALO), pl.ds(0, HALO)
            known = set()

            def fence(ref):
                def park(v):
                    ref[t >> 3, pl.ds(ref.shape[1] - 8, 8), :] = v
                return park

            def probs(a):
                pieces = []
                for r in range(0, 2 * Q, 8):
                    lg = [None] * WIN

                    def logits(c, r=r, lg=lg):
                        assert ("qk", a) in known
                        qv = q_s[c, pl.ds(a * 2 * Q + r, 8), :]
                        for w in range(WIN):
                            pr = qv * k_s[a][c, pl.ds(HALO + r - DIL * w, 8), :]
                            lg[w] = pr if c == 0 else lg[w] + pr

                    def softmax(r=r, lg=lg):
                        lg = [l + pltpu.roll(l, 64, 1) for l in lg]
                        lg = [l + pltpu.roll(l, 32, 1) for l in lg]
                        for w in range(WIN):
                            if a == 0 and r < DIL * w:
                                pos = t * 4 * Q + r + lax.broadcasted_iota(jnp.int32, (8, 128), 0)
                                lg[w] = jnp.where(pos >= DIL * w, lg[w], -1e9 / SCALE)
                        mx = functools.reduce(jnp.maximum, lg)
                        e = [jnp.exp2((l - mx) * (SCALE * LOG2E)) for l in lg]
                        inv = 1.0 / functools.reduce(jnp.add, e)
                        for w in range(WIN):
                            p_s[a][w, pl.ds(r, 8), :] = e[w] * inv
                        return pltpu.bitcast(p_s[a][t >> 3, pl.ds(r, 8), :], U32)

                    pieces += [(None if c % 3 else fence(k_s[a]), functools.partial(logits, c))
                               for c in range(8)]
                    pieces.append((None, softmax))
                return pieces

            def mix(q, first=0, last=2 * Q):
                def work(r, c):
                    assert ("v", q) in known and (r >= HALO or ("v", q % 2) in known)
                    prow = _rows(r + 8 * (t >> (3 + q % 2)), 8)
                    terms = [p_s[q // 2][w, prow, :] * v_s[q][c, pl.ds(HALO + r - DIL * w, 8), :]
                             for w in range(WIN)]
                    o_s[q ^ 1][c, pl.ds(r, 8), :] = functools.reduce(jnp.add, terms)

                return [(None if c % 2 else fence(v_s[q]), functools.partial(work, r, c))
                        for r in range(first, last, 8) for c in range(4)]

            def prep_o(ps):
                def work(i, c, p):
                    assert ("wo", p) not in known
                    op = _operands(LHS, p, lambda q, q2: o_s[q][
                        2 * (q2 % 2) + c, pl.ds((q2 // 2) * Q + i, 16), :])
                    for p2 in range(NP):
                        oop[p][p2, c, pl.ds(i, 16), :] = op(p2)

                return [(fence(o_s[_last_quadrant(p)]), functools.partial(work, i, c, p))
                        for p in ps for i in range(0, Q, 16) for c in range(2)]

            def widen(a):
                def work(r, c):
                    k_s[a][c, pl.ds(HALO + r, Q), :] = _load(kbuf, (c,), (4 * t + 2 * a) * Q + r, Q).astype(F32)

                def park(v):
                    kbuf[t >> 3, pl.ds(S, 16), :] = pltpu.bitcast(v, BF16)

                return [(park, functools.partial(work, r, c)) for r in (0, Q) for c in range(8)]

            def queries(a):
                def product(p):
                    lhs = [_words(aop, (half_index(a, b) + p, c), t * Q, Q) for b, c in QUADS]
                    return [fill.dot(lhs, _cat(_load(wq_op, (p, c), 0, 512) for c in range(4)), 4)]

                def done(q, val):
                    for c in range(4):
                        q_s[4 * (q % 2) + c, pl.ds((2 * a + q // 2) * Q, Q), :] = _lanes(val[0], c)

                _strassen(product, done, (1, 3, 4, 0, 2, 5, 6))
                known.add(("qk", a))

            def two_level(lhs, rhs, done, order, order2):
                def outer(p):
                    return _quadrants(lambda p2: fill.dot(
                        [lhs(p, p2, c) for c in range(2)],
                        _cat(_load(rhs, (p * NP + p2, c), 0, 256) for c in range(2))), order2)

                _strassen(outer, done, order)

            def values(q, vals):
                for q2, v in enumerate(vals):
                    for c in range(2):
                        v_s[q][2 * (q2 % 2) + c, pl.ds(HALO + (q2 // 2) * Q, Q), :] = _lanes(v, c)
                if q < 2:
                    for c in range(4):
                        first = jnp.broadcast_to(v_s[q][c, pl.ds(HALO, 1), :], (HALO, 128))
                        v_s[q][c, head, :] = jnp.where(t > 0, v_s[q][c, head, :], first)
                    v_s[q + 2][:, head, :] = v_s[q][:, tail, :]
                known.add(("v", q))

            def mixed(p, p2, c):
                known.add(("wo", p))
                return _words(oop[p], (p2, c), (t >> 3) * Q, Q)

            def output(q, vals):
                for q2, v in enumerate(vals):
                    a, nq = _quarter(q, q2)
                    for c in range(2):
                        col, start = 2 * (nq ^ 3) + c, (4 * t + a) * Q
                        g = _load(ybuf, (col,), start, Q).astype(F32)
                        xv = xbuf[4 * t + a, :, _chunk(col)].astype(F32)
                        obuf[_rows(start, Q), _chunk(col)] = (xv + _lanes(v, c) * g).astype(BF16)
                known.add(("out", q))
                if ("out", q ^ 1) in known:
                    out_copy(2 * t + q // 2).start()

            k_s[0][:, head, :] = jnp.where(t > 0, k_s[1][:, tail, :], 0.0)
            for q in range(2):
                v_s[q][:, head, :] = v_s[q + 2][:, tail, :]
            fill.plan(0, 18, widen(0) + widen(1))
            queries(0)
            assert not fill.todo
            k_s[1][:, head, :] = k_s[0][:, tail, :]
            fill.plan(0, 27, probs(0))
            fill.plan(28, 55, probs(1))
            fill.plan(55, 67, mix(1) + prep_o((2,)))
            fill.plan(67, 79, mix(2, HALO) + mix(2, 0, HALO) + prep_o((3, 0)))
            fill.plan(79, 89, mix(0) + prep_o((4, 6)))
            fill.plan(89, 102, mix(3) + prep_o((1, 5)))
            queries(1)
            two_level(lambda p, p2, c: _words(aop, (p * NP + p2, c), t * Q, Q), wv_op, values,
                      (2, 4, 3, 1, 0, 6, 5), (4, 2, 3, 1, 0, 5, 6))
            two_level(mixed, wo_op, output, (2, 3, 0, 4, 6, 1, 5), (1, 3, 2, 4, 0, 6, 5))
            assert not fill.todo
            return carry

        _start(x_copy(t) for t in range(1, NT))
        lax.fori_loop(0, NT, tile, 0)
        seen = _Range(energy, FFN)
        seen.add_rows([energy[pl.ds(0, S), :]])
        seen.save()
        failed = []
        for slot in range(9):
            lo, hi = (energy[rows, :] for rows in _range_rows(slot))
            least = jnp.min(jnp.min(lo, axis=0, keepdims=True), axis=1, keepdims=True)
            balanced = (lo > 0.0) & (hi < jnp.inf) & (hi <= BALANCE * least)
            failed.append(jnp.where(balanced, 0.0, 1.0))
        unbalanced = jnp.max(functools.reduce(jnp.maximum, failed)) > 0.0
        _wait(out_copy(t) for t in range(2 * NT))
        return unbalanced

    unbalanced = pl.run_scoped(
        attention,
        pltpu.VMEM((8, 4 * Q, 128), F32),
        pltpu.VMEM((S, D), BF16),
        *[pltpu.VMEM((WIN, 2 * Q, 128), F32)] * 2,
        *[pltpu.VMEM((8, HALO + 2 * Q + 8, 128), F32)] * 2,
        *[pltpu.VMEM((4, HALO + 2 * Q + 8, 128), F32)] * 4,
        *[pltpu.VMEM((4, 2 * Q + 8, 128), F32)] * 4,
        *[pltpu.VMEM((NP, 2, Q, 128), BF16)] * NP,
    )

    def plain(xn_s, w_s, wo_s, wd_s, qkv_s, o_s, h_s):

        def repeat(n, body):
            def step(i, carry):
                body(i)
                return carry

            lax.fori_loop(0, n, step, 0)

        def fetch(src, dst):
            copy = pltpu.make_async_copy(src, dst, sem_w.at[0])
            copy.start()
            copy.wait()

        def dot(a, b):
            return jnp.dot(a, b, preferred_element_type=F32)

        def normalize(i):
            xv = xbuf[i >> 2, _rows((i & 3) * 16, 16), :].astype(F32)
            xc = xv - jnp.mean(xv, axis=-1, keepdims=True)
            var = jnp.mean(xc * xc, axis=-1, keepdims=True)
            xn_s[_rows(i * 16, 16), :] = (xc * lax.rsqrt(var + 1e-5)).astype(BF16)

        def project(m):
            def rows(i):
                first = pl.multiple_of(HALO + i * 32, 16)
                qkv_s[m, pl.ds(first, 32), :] = dot(xn_s[_rows(i * 32, 32), :], w_s[m])

            repeat(S // 32, rows)

        def attend(c):
            def rows(i):
                first = pl.multiple_of(i * 16, 16)
                pos = i * 16 + lax.broadcasted_iota(jnp.int32, (16, 128), 0)
                k, v = (qkv_s[m, pl.ds(first, HALO + 16), :] for m in (1, 2))
                qv = qkv_s[0, pl.ds(first + HALO, 16), :]
                pr = jnp.concatenate([qv * k[HALO - DIL * w:HALO - DIL * w + 16]
                                      for w in range(WIN)], axis=0)
                head = [lax.broadcasted_iota(jnp.int32, (128, 128), d) >> 5 for d in (0, 1)]
                same = jnp.where(head[0] == head[1], 1.0, 0.0).astype(BF16)
                top = pr.astype(BF16)
                lg = (dot(top, same) + dot((pr - top.astype(F32)).astype(BF16), same)) * SCALE
                lg = [jnp.where(pos >= DIL * w, lg[16 * w:16 * w + 16], -1e9) for w in range(WIN)]
                mx = functools.reduce(jnp.maximum, lg)
                e = [jnp.exp(l - mx) for l in lg]
                o = functools.reduce(jnp.add, [e[w] * v[HALO - DIL * w:HALO - DIL * w + 16]
                                               for w in range(WIN)])
                o_s[c, pl.ds(first, 16), :] = (o / functools.reduce(jnp.add, e)).astype(BF16)

            for m in (1, 2):
                qkv_s[m, pl.ds(0, HALO), :] = jnp.broadcast_to(
                    qkv_s[m, pl.ds(HALO, 1), :], (HALO, 128))
            repeat(S // 16, rows)

        def activate(f):
            def rows(i):
                g, u = (qkv_s[m, _rows(HALO + i * 16, 16), :] for m in (0, 1))
                h_s[f, _rows(i * 16, 16), :] = (_gelu(g) * u).astype(BF16)

            repeat(S // 16, rows)

        def columns(n):
            @pl.when(n < 8)
            def _():
                repeat(12, lambda i: fetch(wqkv_hbm.at[i & 3, :, _chunk(8 * (i >> 2) + n)],
                                           w_s.at[i >> 2, _rows((i & 3) * 256, 256)]))

            @pl.when(n >= 8)
            def _():
                fetch(wg_hbm.at[:, _chunk(n - 8)], w_s.at[0])
                fetch(wu_hbm.at[:, _chunk(n - 8)], w_s.at[1])

            repeat(jnp.where(n < 8, 3, 2), project)
            pl.when(n < 8)(lambda: attend(n))
            pl.when(n >= 8)(lambda: activate(n - 8))

        def finish(c):
            def rows(i):
                r = _rows(i * 16, 16)
                d = lax.fori_loop(0, NJ, lambda j, d: d + dot(
                    _cat(h_s[4 * j + n, r, :] for n in range(4)), wd_s[_rows(j * 512, 512), :]),
                    jnp.zeros((16, 128), F32))
                sv = dot(_cat(o_s[n, r, :] for n in range(8)),
                         jnp.concatenate([wo_s[n] for n in range(16)], axis=0))
                xv = wo_s[16 + (i >> 2), _rows((i & 3) * 16, 16), :].astype(F32)
                ybuf[c, r, :] = (xv + sv * _silu(d)).astype(BF16)

            fetch(wo_hbm.at[:, :, _chunk(c)], wo_s.at[pl.ds(0, 16)])
            fetch(x_hbm.at[:, :, _chunk(c)], wo_s.at[pl.ds(16, S // Q)])
            fetch(wd_hbm.at[:, _chunk(c)], wd_s)
            repeat(S // 16, rows)
            fetch(ybuf.at[c], out_hbm.at[:, _chunk(c)])

        repeat(S // 16, normalize)
        repeat(8 + F // 128, columns)
        repeat(8, finish)

    @pl.when(unbalanced)
    def _():
        pl.run_scoped(plain, pltpu.VMEM((S, D), BF16), pltpu.VMEM((3, D, 128), BF16),
                      pltpu.VMEM((16 + S // Q, Q, 128), BF16), pltpu.VMEM((F, 128), BF16),
                      pltpu.VMEM((3, HALO + S, 128), F32), pltpu.VMEM((8, S, 128), BF16),
                      pltpu.VMEM((F // 128, S, 128), BF16))


@jax.jit
def pallas_recurrent_scan__sliding_local_dilated__geglu_ffn__prompt_kernel(
    A_x: jax.Array,
    A_wqkv: jax.Array,
    A_wo: jax.Array,
    B_x: jax.Array,
    B_w_gate: jax.Array,
    B_w_up: jax.Array,
    B_w_down: jax.Array,
):
    del B_x
    in_hbm = pl.BlockSpec(memory_space=pl.ANY)
    out = pl.pallas_call(
        _kernel,
        out_shape=jax.ShapeDtypeStruct((S, D), BF16),
        in_specs=[in_hbm] * 6,
        out_specs=in_hbm,
        scratch_shapes=[
            pltpu.VMEM((S // Q + 1, Q, D), BF16),
            pltpu.VMEM((8, S, 128), BF16),
            pltpu.VMEM((8, S + 16, 128), BF16),
            pltpu.VMEM((2, 512 + 16, D), BF16),
            pltpu.VMEM((NP * (NP + 2), 2, S // 4, 128), BF16),
            pltpu.VMEM((NP, 4, D // 4, 128), U32),
            pltpu.VMEM((NP * NP, 2, D // 8, 128), U32),
            pltpu.VMEM((NP * NP, 2, D // 8, 128), U32),
            pltpu.VMEM((S + 9 * 16 + 8, 128), F32),
            pltpu.SemaphoreType.DMA((NT,)),
            pltpu.SemaphoreType.DMA((4,)),
            pltpu.SemaphoreType.DMA((2,)),
            pltpu.SemaphoreType.DMA((3,)),
            pltpu.SemaphoreType.DMA((2 * NT,)),
        ],
        compiler_params=pltpu.CompilerParams(vmem_limit_bytes=127 * 2**20),
        name="fused_block",
    )(A_x.reshape(S // Q, Q, D), A_wqkv.reshape(4, D // 4, 3 * D),
      A_wo.reshape(D // Q, Q, D), B_w_gate, B_w_up, B_w_down)
    return out.reshape(A_x.shape)
```
